```python
import jax
import jax.numpy as jnp

def _softmax(x, axis=-1):
    return jax.nn.softmax(x, axis=axis)
def _gelu(x):
    return jax.nn.gelu(x, approximate=True)
def _silu(x):
    return jax.nn.silu(x)
def _sigmoid(x):
    return jax.nn.sigmoid(x)
def _layernorm(x, axis=-1, eps=1e-5):
    m = jnp.mean(x, axis=axis, keepdims=True)
    v = jnp.var(x, axis=axis, keepdims=True)
    return (x - m) / jnp.sqrt(v + eps)
def _scatter_add(tgt, idx, src, axis=0):
    return tgt.at[idx].add(src)
def _segment_sum(src, seg, n):
    return jax.ops.segment_sum(src, seg, n)
class _Rng:
    def __init__(self, key):
        self._k = key
    def _next(self):
        self._k, sub = jax.random.split(self._k)
        return sub
    def normal(self, shape):
        return jax.random.normal(self._next(), shape, dtype=jnp.bfloat16)
    def randint(self, lo, hi, shape):
        return jax.random.randint(self._next(), shape, lo, hi, dtype=jnp.int32)
    def uniform(self, shape, lo=0.0, hi=1.0):
        return jax.random.uniform(self._next(), shape, jnp.bfloat16, lo, hi)
    def permutation(self, n):
        return jax.random.permutation(self._next(), n)


kernel_name = 'parallel_sum__linear_attn_block__moe_arch_mod__prompt'

def setup_inputs():
    _rng = _Rng(jax.random.key(int.from_bytes(__import__("os").urandom(4), "little")))
    _w = (lambda a: (lambda t: t.astype(jnp.bfloat16) if jnp.issubdtype(t.dtype, jnp.floating) else t)(jnp.asarray(a)))
    def _A_setup():
        B, S, D = 1, 2048, 1024
        return {
            "x": _w((lambda *s: _rng.normal(s) * 0.05)(B, S, D)),
            "wqkv": _w((lambda *s: _rng.normal(s) * 0.05)(D, 3 * D)),
            "wo": _w((lambda *s: _rng.normal(s) * 0.05)(D, D)),
        }
    _A_in = _A_setup()

    def _B_setup():
        B, S, D, F, C = 1, 2048, 1024, 3584, 1
        return {
            "x": _w((lambda *s: _rng.normal(s) * 0.05)(B, S, D)),
            "w_r": _w((lambda *s: _rng.normal(s) * 0.05)(D)),
            "w_gate": _w((lambda *s: _rng.normal(s) * 0.05)(D, F)),
            "w_up": _w((lambda *s: _rng.normal(s) * 0.05)(D, F)),
            "w_down": _w((lambda *s: _rng.normal(s) * 0.05)(F, D)),
        }
    _B_in = _B_setup()

    return {
        "A_x": _A_in["x"],
        "A_wqkv": _A_in["wqkv"],
        "A_wo": _A_in["wo"],
        "B_x": _B_in["x"],
        "B_w_r": _B_in["w_r"],
        "B_w_gate": _B_in["w_gate"],
        "B_w_up": _B_in["w_up"],
        "B_w_down": _B_in["w_down"],
    }

def reference(A_x, A_wqkv, A_wo, B_x, B_w_r, B_w_gate, B_w_up, B_w_down):
    def _A_ref(x, wqkv, wo):
        B, S, D = x.shape
        H = 32; Dh = D // H
        qkv = (lambda x, *d: x.transpose(*d))((x @ wqkv).reshape(B, S, 3, H, Dh), 2, 0, 3, 1, 4)
        q, k, v = qkv[0], qkv[1], qkv[2]
        phi = lambda t: jnp.where(t > 0, t + 1, jnp.exp(t)) + 1e-6
        pq, pk = phi(q), phi(k)
        kv = jnp.einsum("bhsd,bhse->bhde", pk, v)
        z = jnp.einsum("bhsd->bhd", pk)
        num = jnp.einsum("bhqd,bhde->bhqe", pq, kv)
        den = jnp.einsum("bhqd,bhd->bhq", pq, z)[..., None] + 1e-6
        o = num / den
        return (lambda x, *d: x.transpose(*d))(o, 0, 2, 1, 3).reshape(B, S, D) @ wo

    def _B_ref(x, w_r, w_gate, w_up, w_down):
        B, S, D = x.shape
        C = 1
        r = x @ w_r
        idx = jnp.argsort(-r, axis=-1)[:, :C]
        idx_e = jnp.repeat(idx.reshape(B, C, 1), D, axis=2)
        x_sel = jnp.take_along_axis(x, idx_e, axis=1)
        g = _silu(x_sel @ w_gate)
        u = x_sel @ w_up
        y = (g * u) @ w_down
        r_sel = _sigmoid(jnp.take_along_axis(r, idx, axis=1))
        y = y * r_sel.reshape(B, C, 1)
        b_off = (jnp.arange(B) * S).reshape(B, 1)
        flat_idx = (idx + b_off).reshape(B * C)
        zero = (x * 0.0).reshape(B * S, D)
        upd = _scatter_add(zero, flat_idx, y.reshape(B * C, D), axis=0)
        return x + upd.reshape(B, S, D)

    x = A_x
    xn = _layernorm(x, axis=-1)
    return x + _A_ref(xn, A_wqkv, A_wo) + _B_ref(xn, B_w_r, B_w_gate, B_w_up, B_w_down)
```

```python
import functools

import jax
import jax.numpy as jnp
from jax import lax
import jax.experimental.pallas as pl
import jax.experimental.pallas.tpu as pltpu

S = 2048
D = 1024
F = 3584
H = 32
DH = D // H
TS = 256
NS = S // TS
FC = 512
NF = F // FC
G128 = D // 128

_LN_EPS = 1.0013580322265625e-05
_EPS = 1e-6

f32 = jnp.float32
bf16 = jnp.bfloat16


def _bf16_round(v):
    return v.astype(bf16).astype(f32)


def _phi(t):
    return jnp.where(t > 0, t + 1.0, jnp.exp(t)) + _EPS


def _kernel(x_hbm, wqkv_hbm, wo_hbm, wr_ref, wg_hbm, wu_hbm, wd_hbm, out_hbm,
            x_buf, xn_buf, wq_buf, wk_buf, wv_buf, wqt_buf, wo_buf, m_buf,
            g_acc, z_acc, zb_buf, best_val, best_tile,
            wg_buf, wu_buf, wd_buf, xb_buf, y_acc, out_buf,
            x_sem, w_sem, f_sem, o_sem):

    def x_copy(i):
        return pltpu.make_async_copy(
            x_hbm.at[pl.ds(i * TS, TS), :], x_buf.at[i], x_sem.at[i])

    wk_copy = pltpu.make_async_copy(wqkv_hbm.at[:, pl.ds(D, D)], wk_buf, w_sem.at[0])
    wq_copy = pltpu.make_async_copy(wqkv_hbm.at[:, pl.ds(0, D)], wq_buf, w_sem.at[1])
    wv_copy = pltpu.make_async_copy(wqkv_hbm.at[:, pl.ds(2 * D, D)], wv_buf, w_sem.at[2])
    wo_copy = pltpu.make_async_copy(wo_hbm, wo_buf, w_sem.at[3])

    def ffn_copies(j):
        return (
            pltpu.make_async_copy(wg_hbm.at[:, pl.ds(j * FC, FC)], wg_buf.at[j], f_sem.at[0, j]),
            pltpu.make_async_copy(wu_hbm.at[:, pl.ds(j * FC, FC)], wu_buf.at[j], f_sem.at[1, j]),
            pltpu.make_async_copy(wd_hbm.at[pl.ds(j * FC, FC), :], wd_buf.at[j], f_sem.at[2, j]),
        )

    def out_copy(t):
        return pltpu.make_async_copy(
            out_buf.at[t], out_hbm.at[pl.ds(t * TS, TS), :], o_sem.at[t])

    x_copy(0).start()
    wk_copy.start()
    x_copy(1).start()
    wq_copy.start()
    for i in range(2, NS):
        x_copy(i).start()
    wv_copy.start()
    wo_copy.start()
    for j in range(NF):
        for c in ffn_copies(j):
            c.start()

    g_acc[...] = jnp.zeros_like(g_acc)
    z_acc[...] = jnp.zeros_like(z_acc)
    y_acc[...] = jnp.zeros_like(y_acc)
    best_val[...] = jnp.full(best_val.shape, -jnp.inf, f32)
    best_tile[...] = jnp.zeros_like(best_tile)

    wr = wr_ref[...].astype(f32)

    def layernorm(src, dst):
        x = x_buf[src].astype(f32)
        mean = jnp.sum(x, axis=-1, keepdims=True) * (1.0 / D)
        c = x - mean
        var = jnp.sum(c * c, axis=-1, keepdims=True) * (1.0 / D)
        sd = _bf16_round(jnp.sqrt(_bf16_round(_bf16_round(var) + _LN_EPS)))
        d = _bf16_round(x - _bf16_round(mean))
        xn = (d * (1.0 / sd)).astype(bf16)
        xn_buf[dst] = xn
        r = _bf16_round(jnp.sum(xn.astype(f32) * wr, axis=-1, keepdims=True))
        better = r > best_val[...]
        best_val[...] = jnp.where(better, r, best_val[...])
        best_tile[...] = jnp.where(better, src, best_tile[...])

    x_copy(0).wait()
    layernorm(0, 0)
    wk_copy.wait()
    wq_copy.wait()

    def phase1(i, carry):
        @pl.when(i + 1 < NS)
        def _():
            x_copy(i + 1).wait()

        xn = xn_buf[i]
        k = jnp.dot(xn, wk_buf[...], preferred_element_type=f32)
        pk = _phi(k)
        z_acc[...] += jnp.sum(pk.reshape(TS // 8, 8, D), axis=0)
        g_acc[...] += lax.dot_general(pk.astype(bf16), xn, (((0,), (0,)), ((), ())),
                                      preferred_element_type=f32)
        col = pl.multiple_of(i * (D // NS), D // NS)
        wqt_buf[pl.ds(col, D // NS), :] = wq_buf[:, pl.ds(col, D // NS)].T
        layernorm(jnp.minimum(i + 1, NS - 1), i + 1)
        return carry

    lax.fori_loop(0, NS, phase1, 0)

    bv = best_val[...]
    rmax = jnp.max(bv, axis=0, keepdims=True)
    rows = lax.broadcasted_iota(jnp.int32, (TS, 1), 0)
    cand = jnp.where(bv == rmax, best_tile[...] * TS + rows, S)
    idx = jnp.min(cand)
    idx = jnp.clip(idx, 0, S - 1)
    t_sel = idx // TS
    r_in = idx - t_sel * TS
    r16 = pl.multiple_of((r_in // 16) * 16, 16)
    blk = xn_buf[t_sel, pl.ds(r16, 16), :].astype(f32)
    sel = lax.broadcasted_iota(jnp.int32, (16, D), 0) == (r_in - r16)
    x_sel = jnp.sum(jnp.where(sel, blk, 0.0), axis=0, keepdims=True)
    xb_buf[...] = jnp.broadcast_to(x_sel, (128, D)).T
    gate = 1.0 / (1.0 + jnp.exp(-rmax))

    z = jnp.sum(z_acc[...], axis=0, keepdims=True)
    zb_buf[...] = jnp.broadcast_to(z, (128, D)).T

    wv_copy.wait()
    wo_copy.wait()
    rr = lax.broadcasted_iota(jnp.int32, (128, 128), 0) // DH
    cc = lax.broadcasted_iota(jnp.int32, (128, 128), 1) // DH
    same_head = rr == cc
    for g in range(G128):
        sl = slice(g * 128, (g + 1) * 128)
        kv = jnp.dot(g_acc[sl, :].astype(bf16), wv_buf[:, sl], preferred_element_type=f32)
        kv = jnp.where(same_head, kv, 0.0).astype(bf16)
        m_buf[sl, :] = jnp.dot(kv, wo_buf[sl, :], preferred_element_type=f32).astype(bf16)

    def attn_tile(t):
        xn = xn_buf[t]
        qt = lax.dot_general(wqt_buf[...], xn, (((1,), (1,)), ((), ())),
                             preferred_element_type=f32)
        pqt = _phi(qt)
        zb = zb_buf[...]
        zfull = jnp.concatenate([zb] * (TS // 128), axis=1)
        den = jnp.sum((pqt * zfull).reshape(H, DH, TS), axis=1, keepdims=True) + _EPS
        pt = (pqt.reshape(H, DH, TS) * pl.reciprocal(den, approx=True)).reshape(D, TS).astype(bf16)
        attn = lax.dot_general(pt, m_buf[...], (((0,), (0,)), ((), ())),
                               preferred_element_type=f32)
        return attn + x_buf[t].astype(f32) + xn.astype(f32)

    def ffn_chunk(j):
        xb = xb_buf[...]
        gs, us = [], []
        for c in range(FC // 128):
            sl = slice(c * 128, (c + 1) * 128)
            gs.append(jnp.sum((wg_buf[j, :, sl].astype(f32) * xb).reshape(D // 8, 8, 128), axis=0))
            us.append(jnp.sum((wu_buf[j, :, sl].astype(f32) * xb).reshape(D // 8, 8, 128), axis=0))
        g = jnp.sum(jnp.concatenate(gs, axis=1), axis=0, keepdims=True)
        u = jnp.sum(jnp.concatenate(us, axis=1), axis=0, keepdims=True)
        h = g * (1.0 / (1.0 + jnp.exp(-g))) * u
        hb = jnp.broadcast_to(h, (128, FC)).T
        ys = []
        for c in range(D // 128):
            sl = slice(c * 128, (c + 1) * 128)
            ys.append(jnp.sum((wd_buf[j, :, sl].astype(f32) * hb).reshape(FC // 8, 8, 128), axis=0))
        y_acc[...] += jnp.concatenate(ys, axis=1)

    def phase2(j, carry):
        for c in ffn_copies(j):
            c.wait()
        t = lax.rem(t_sel + 1 + j, NS)
        out_buf[t] = attn_tile(t).astype(bf16)
        ffn_chunk(j)
        out_copy(t).start()
        return carry

    lax.fori_loop(0, NS - 1, phase2, 0)

    y = jnp.sum(y_acc[...], axis=0, keepdims=True) * gate
    o = attn_tile(t_sel)
    hit = lax.broadcasted_iota(jnp.int32, (TS, D), 0) == r_in
    out_buf[t_sel] = (o + jnp.where(hit, y, 0.0)).astype(bf16)
    out_copy(t_sel).start()
    for t in range(NS):
        out_copy(t).wait()


@jax.jit
def pallas_parallel_sum__linear_attn_block__moe_arch_mod__prompt_kernel(
    A_x: jax.Array,
    A_wqkv: jax.Array,
    A_wo: jax.Array,
    B_x: jax.Array,
    B_w_r: jax.Array,
    B_w_gate: jax.Array,
    B_w_up: jax.Array,
    B_w_down: jax.Array,
):
    assert NF == NS - 1
    any_spec = pl.BlockSpec(memory_space=pl.ANY)
    out = pl.pallas_call(
        _kernel,
        out_shape=jax.ShapeDtypeStruct((S, D), bf16),
        in_specs=[any_spec, any_spec, any_spec,
                  pl.BlockSpec(memory_space=pltpu.VMEM),
                  any_spec, any_spec, any_spec],
        out_specs=any_spec,
        scratch_shapes=[
            pltpu.VMEM((NS, TS, D), bf16),
            pltpu.VMEM((NS + 1, TS, D), bf16),
            pltpu.VMEM((D, D), bf16),
            pltpu.VMEM((D, D), bf16),
            pltpu.VMEM((D, D), bf16),
            pltpu.VMEM((D, D), bf16),
            pltpu.VMEM((D, D), bf16),
            pltpu.VMEM((D, D), bf16),
            pltpu.VMEM((D, D), f32),
            pltpu.VMEM((8, D), f32),
            pltpu.VMEM((D, 128), f32),
            pltpu.VMEM((TS, 1), f32),
            pltpu.VMEM((TS, 1), jnp.int32),
            pltpu.VMEM((NF, D, FC), bf16),
            pltpu.VMEM((NF, D, FC), bf16),
            pltpu.VMEM((NF, FC, D), bf16),
            pltpu.VMEM((D, 128), f32),
            pltpu.VMEM((8, D), f32),
            pltpu.VMEM((NS, TS, D), bf16),
            pltpu.SemaphoreType.DMA((NS,)),
            pltpu.SemaphoreType.DMA((4,)),
            pltpu.SemaphoreType.DMA((3, NF)),
            pltpu.SemaphoreType.DMA((NS,)),
        ],
        compiler_params=pltpu.CompilerParams(vmem_limit_bytes=100 * 1024 * 1024),
        name="linattn_mod",
    )(A_x.reshape(S, D), A_wqkv, A_wo, B_w_r.reshape(1, D), B_w_gate, B_w_up, B_w_down)
    return out.reshape(1, S, D)
```

```python
import jax
import jax.numpy as jnp
from jax import lax
import jax.experimental.pallas as pl
import jax.experimental.pallas.tpu as pltpu

S = 2048
D = 1024
F = 3584
H = 32
DH = D // H
TS = 256
NS = S // TS
FC = 512
NF = F // FC
G128 = D // 128
CW = 256
NC = D // CW
LR = TS // (2 * NC)

_LN_EPS = 1.0013580322265625e-05
_EPS = 1e-6
_SCOPES = False

f32 = jnp.float32
bf16 = jnp.bfloat16

_SEM_X = 0
_SEM_WK = _SEM_X + NS
_SEM_WQ = _SEM_WK + NC
_SEM_WV = _SEM_WQ + 1
_SEM_WO = _SEM_WV + 1
_SEM_WR = _SEM_WO + 1
_SEM_F = _SEM_WR + 1
_N_SEM = _SEM_F + 3 * NF


class _NoScope:
    def __enter__(self):
        return self

    def __exit__(self, *a):
        return False


def _scope(name):
    return jax.named_scope(name) if _SCOPES else _NoScope()


def _bf16_round(v):
    return v.astype(bf16).astype(f32)


def _phi(t):
    return jnp.where(t > 0, t + 1.0, jnp.exp(t)) + _EPS


_TN = (((0,), (0,)), ((), ()))
_NT = (((1,), (1,)), ((), ()))


def _kernel(x_hbm, wqkv_hbm, wo_hbm, wr_hbm, wg_hbm, wu_hbm, wd_hbm, out_hbm,
            x_buf, xn_buf, wq_buf, wk_buf, wv_buf, wqt_buf, wo_buf, m_buf, wr_buf,
            g_acc, z_acc, zb_buf, best_val, best_tile,
            wg_buf, wu_buf, wd_buf, xb_buf, y_acc, out_buf,
            sem, o_sem):

    def x_copy(i):
        return pltpu.make_async_copy(
            x_hbm.at[pl.ds(i * TS, TS), :], x_buf.at[i], sem.at[_SEM_X + i])

    def wk_copy(c):
        return pltpu.make_async_copy(
            wqkv_hbm.at[:, pl.ds(D + c * CW, CW)], wk_buf.at[c], sem.at[_SEM_WK + c])

    wq_copy = pltpu.make_async_copy(wqkv_hbm.at[:, pl.ds(0, D)], wq_buf, sem.at[_SEM_WQ])
    wv_copy = pltpu.make_async_copy(wqkv_hbm.at[:, pl.ds(2 * D, D)], wv_buf, sem.at[_SEM_WV])
    wo_copy = pltpu.make_async_copy(wo_hbm, wo_buf, sem.at[_SEM_WO])
    wr_copy = pltpu.make_async_copy(wr_hbm, wr_buf, sem.at[_SEM_WR])

    def ffn_copies(j):
        s = _SEM_F + 3 * j
        return (
            pltpu.make_async_copy(wg_hbm.at[:, pl.ds(j * FC, FC)], wg_buf.at[j], sem.at[s]),
            pltpu.make_async_copy(wu_hbm.at[:, pl.ds(j * FC, FC)], wu_buf.at[j], sem.at[s + 1]),
            pltpu.make_async_copy(wd_hbm.at[pl.ds(j * FC, FC), :], wd_buf.at[j], sem.at[s + 2]),
        )

    def out_copy(t):
        return pltpu.make_async_copy(
            out_buf.at[t], out_hbm.at[pl.ds(t * TS, TS), :], o_sem.at[t])

    wr_copy.start()
    x_copy(0).start()
    wk_copy(0).start()
    wk_copy(1).start()
    x_copy(1).start()
    for c in range(2, NC):
        wk_copy(c).start()
    wq_copy.start()
    for i in range(2, NS):
        x_copy(i).start()
    wv_copy.start()
    wo_copy.start()
    for j in range(NF):
        for c in ffn_copies(j):
            c.start(priority=1)

    y_acc[...] = jnp.zeros_like(y_acc)
    best_val[...] = jnp.full(best_val.shape, -jnp.inf, f32)
    best_tile[...] = jnp.zeros_like(best_tile)

    def layernorm(src, dst, r0, nr):
        rows = pl.ds(r0, nr)
        x = x_buf[src, rows, :].astype(f32)
        mean = jnp.sum(x, axis=-1, keepdims=True) * (1.0 / D)
        c = x - mean
        var = jnp.sum(c * c, axis=-1, keepdims=True) * (1.0 / D)
        sd = _bf16_round(jnp.sqrt(_bf16_round(_bf16_round(var) + _LN_EPS)))
        d = _bf16_round(x - _bf16_round(mean))
        xn = (d * (1.0 / sd)).astype(bf16)
        xn_buf[dst, rows, :] = xn
        wr = wr_buf[...].reshape(1, D).astype(f32)
        r = _bf16_round(jnp.sum(xn.astype(f32) * wr, axis=-1, keepdims=True))
        old = best_val[rows, :]
        better = r > old
        best_val[rows, :] = jnp.where(better, r, old)
        best_tile[rows, :] = jnp.where(better, src, best_tile[rows, :])

    def phase1_body(i, first):
        xn = xn_buf[i]
        src = i + 1 if first else jnp.minimum(i + 1, NS - 1)
        pieces = iter(range(2 * NC))

        def side():
            p = next(pieces)
            if first and p == 2:
                with _scope("wait_x1"):
                    x_copy(1).wait()
            if not first or p >= 2:
                layernorm(src, i + 1, p * LR, LR)
            if first and p == 2 * NC - 1:
                layernorm(src, i + 1, 0, 2 * LR)
            if not first and p == 0:
                col = pl.multiple_of((i - 1) * (D // NS), D // NS)
                wqt_buf[pl.ds(col, D // NS), :] = wq_buf[:, pl.ds(col, D // NS)].T

        def k_part(c):
            if first:
                with _scope("wait_wk"):
                    wk_copy(c).wait()
            pk = _phi(jnp.dot(xn, wk_buf[c], preferred_element_type=f32))
            zc = jnp.sum(pk.reshape(TS // 8, 8, CW), axis=0)
            cols = slice(c * CW, (c + 1) * CW)
            z_acc[:, cols] = zc if first else z_acc[:, cols] + zc
            return pk.astype(bf16)

        def g_part(c, pk):
            rows = slice(c * CW, (c + 1) * CW)
            g = lax.dot_general(pk, xn, _TN, preferred_element_type=f32)
            g_acc[rows, :] = g if first else g_acc[rows, :] + g

        pk_prev = k_part(0)
        side()
        for c in range(1, NC):
            pk = k_part(c)
            side()
            g_part(c - 1, pk_prev)
            side()
            pk_prev = pk
        g_part(NC - 1, pk_prev)
        side()

    with _scope("wait_x0"):
        wr_copy.wait()
        x_copy(0).wait()
    with _scope("ln0"):
        layernorm(0, 0, 0, TS)
    phase1_body(0, True)
    with _scope("wait_wq"):
        wq_copy.wait()

    def phase1(i, carry):
        with _scope("p1_wait"):
            @pl.when(i + 1 < NS)
            def _():
                x_copy(i + 1).wait()
        with _scope("p1_body"):
            phase1_body(i, False)
        return carry

    lax.fori_loop(1, NS, phase1, 0)

    wv_copy.wait()
    wo_copy.wait()
    rr = lax.broadcasted_iota(jnp.int32, (128, 128), 0) // DH
    cc = lax.broadcasted_iota(jnp.int32, (128, 128), 1) // DH
    same_head = rr == cc

    def kv_part(g):
        sl = slice(g * 128, (g + 1) * 128)
        kv = jnp.dot(g_acc[sl, :].astype(bf16), wv_buf[:, sl], preferred_element_type=f32)
        return jnp.where(same_head, kv, 0.0).astype(bf16)

    def m_part(g, kv):
        sl = slice(g * 128, (g + 1) * 128)
        m_buf[sl, :] = jnp.dot(kv, wo_buf[sl, :], preferred_element_type=f32).astype(bf16)

    kvs = [kv_part(0)]

    bv = best_val[...]
    rmax = jnp.max(bv, axis=0, keepdims=True)
    rows = lax.broadcasted_iota(jnp.int32, (TS, 1), 0)
    cand = jnp.where(bv == rmax, best_tile[...] * TS + rows, S)
    idx = jnp.clip(jnp.min(cand), 0, S - 1)
    t_sel = idx // TS
    r_in = idx - t_sel * TS
    gate = 1.0 / (1.0 + jnp.exp(-rmax))

    kvs.append(kv_part(1))
    last = slice(D - D // NS, D)
    wqt_buf[last, :] = wq_buf[:, last].T
    m_part(0, kvs[0])
    kvs.append(kv_part(2))
    z = jnp.sum(z_acc[...], axis=0, keepdims=True)
    zb_buf[...] = jnp.broadcast_to(z, (128, D)).T
    m_part(1, kvs[1])
    kvs.append(kv_part(3))
    r16 = pl.multiple_of((r_in // 16) * 16, 16)
    blk = xn_buf[t_sel, pl.ds(r16, 16), :].astype(f32)
    sel = lax.broadcasted_iota(jnp.int32, (16, D), 0) == (r_in - r16)
    x_sel = jnp.sum(jnp.where(sel, blk, 0.0), axis=0, keepdims=True)
    xb_buf[...] = jnp.broadcast_to(x_sel, (128, D)).T
    m_part(2, kvs[2])
    for g in range(4, G128):
        kvs.append(kv_part(g))
        m_part(g - 1, kvs[g - 1])
    m_part(G128 - 1, kvs[G128 - 1])

    def phase2_body(t, j, y):
        xn = xn_buf[t]
        st = {}

        def up_piece(w_buf, c):
            w = w_buf[j, :, c * 128:(c + 1) * 128].astype(f32)
            return jnp.sum((w * xb_buf[...]).reshape(D // 8, 8, 128), axis=0)

        def down_piece(c):
            cols = slice(c * 128, (c + 1) * 128)
            w = wd_buf[j, :, cols].astype(f32)
            y_acc[:, cols] += jnp.sum((w * st["hb"]).reshape(FC // 8, 8, 128), axis=0)

        def side(p):
            if j is None:
                return
            n = FC // 128
            if p < 2:
                for c in range(p * n // 2, (p + 1) * n // 2):
                    st["g", c] = up_piece(wg_buf, c)
                    st["u", c] = up_piece(wu_buf, c)
            elif p == 2:
                g = jnp.sum(jnp.concatenate([st["g", c] for c in range(n)], axis=1),
                            axis=0, keepdims=True)
                u = jnp.sum(jnp.concatenate([st["u", c] for c in range(n)], axis=1),
                            axis=0, keepdims=True)
                h = g * (1.0 / (1.0 + jnp.exp(-g))) * u
                st["hb"] = jnp.broadcast_to(h, (128, FC)).T
            elif p < 7:
                down_piece(2 * (p - 3))
                down_piece(2 * (p - 3) + 1)

        ps = []
        for c in range(NC):
            rows = slice(c * CW, (c + 1) * CW)
            qt = lax.dot_general(wqt_buf[rows, :], xn, _NT, preferred_element_type=f32)
            pqt = _phi(qt)
            zb = zb_buf[rows, :]
            zfull = jnp.concatenate([zb] * (TS // 128), axis=1)
            hc = CW // DH
            den = jnp.sum((pqt * zfull).reshape(hc, DH, TS), axis=1, keepdims=True) + _EPS
            pt = pqt.reshape(hc, DH, TS) * pl.reciprocal(den, approx=True)
            ps.append(pt.reshape(CW, TS).astype(bf16).T)
            side(c)
        p = jnp.concatenate(ps, axis=1)
        for c in range(NC):
            cols = slice(c * CW, (c + 1) * CW)
            o = jnp.dot(p, m_buf[:, cols], preferred_element_type=f32)
            o = o + x_buf[t, :, cols].astype(f32) + xn_buf[t, :, cols].astype(f32)
            if j is None:
                hit = lax.broadcasted_iota(jnp.int32, (TS, CW), 0) == r_in
                o = o + jnp.where(hit, y[:, cols], 0.0)
            out_buf[t, :, cols] = o.astype(bf16)
            side(NC + c)

    def phase2(j, carry):
        with _scope("p2_wait"):
            for c in ffn_copies(j):
                c.wait()
        with _scope("p2_body"):
            t = lax.rem(t_sel + 1 + j, NS)
            phase2_body(t, j, None)
            out_copy(t).start()
        return carry

    lax.fori_loop(0, NS - 1, phase2, 0)

    y = jnp.sum(y_acc[...], axis=0, keepdims=True) * gate
    phase2_body(t_sel, None, y)
    out_copy(t_sel).start()
    with _scope("final_wait"):
        for t in range(NS):
            out_copy(t).wait()


@jax.jit
def pallas_parallel_sum__linear_attn_block__moe_arch_mod__prompt_kernel(
    A_x: jax.Array,
    A_wqkv: jax.Array,
    A_wo: jax.Array,
    B_x: jax.Array,
    B_w_r: jax.Array,
    B_w_gate: jax.Array,
    B_w_up: jax.Array,
    B_w_down: jax.Array,
):
    assert NF == NS - 1
    any_spec = pl.BlockSpec(memory_space=pl.ANY)
    out = pl.pallas_call(
        _kernel,
        out_shape=jax.ShapeDtypeStruct((S, D), bf16),
        in_specs=[any_spec] * 7,
        out_specs=any_spec,
        scratch_shapes=[
            pltpu.VMEM((NS, TS, D), bf16),
            pltpu.VMEM((NS + 1, TS, D), bf16),
            pltpu.VMEM((D, D), bf16),
            pltpu.VMEM((NC, D, CW), bf16),
            pltpu.VMEM((D, D), bf16),
            pltpu.VMEM((D, D), bf16),
            pltpu.VMEM((D, D), bf16),
            pltpu.VMEM((D, D), bf16),
            pltpu.VMEM((D,), bf16),
            pltpu.VMEM((D, D), f32),
            pltpu.VMEM((8, D), f32),
            pltpu.VMEM((D, 128), f32),
            pltpu.VMEM((TS, 1), f32),
            pltpu.VMEM((TS, 1), jnp.int32),
            pltpu.VMEM((NF, D, FC), bf16),
            pltpu.VMEM((NF, D, FC), bf16),
            pltpu.VMEM((NF, FC, D), bf16),
            pltpu.VMEM((D, 128), f32),
            pltpu.VMEM((8, D), f32),
            pltpu.VMEM((NS, TS, D), bf16),
            pltpu.SemaphoreType.DMA((_N_SEM,)),
            pltpu.SemaphoreType.DMA((NS,)),
        ],
        compiler_params=pltpu.CompilerParams(vmem_limit_bytes=100 * 1024 * 1024),
        name="linattn_mod",
    )(A_x.reshape(S, D), A_wqkv, A_wo, B_w_r, B_w_gate, B_w_up, B_w_down)
    return out.reshape(1, S, D)
```

```python
import jax
import jax.numpy as jnp
from jax import lax
import jax.experimental.pallas as pl
import jax.experimental.pallas.tpu as pltpu

S = 2048
D = 1024
F = 3584
H = 32
DH = D // H
TS = 256
NS = S // TS
FC = 512
NF = F // FC
G128 = D // 128
CW = 256
NC = D // CW
LR = TS // NC

_LN_EPS = 1.0013580322265625e-05
_EPS = 1e-6
_SCOPES = False

f32 = jnp.float32
bf16 = jnp.bfloat16

_SEM_X = 0
_SEM_WK = _SEM_X + NS
_SEM_WQ = _SEM_WK + NC
_SEM_WV = _SEM_WQ + 1
_SEM_WO = _SEM_WV + 1
_SEM_WR = _SEM_WO + 1
_SEM_F = _SEM_WR + 1
_N_SEM = _SEM_F + 3 * NF


class _NoScope:
    def __enter__(self):
        return self

    def __exit__(self, *a):
        return False


def _scope(name):
    return jax.named_scope(name) if _SCOPES else _NoScope()


def _bf16_round(v):
    return v.astype(bf16).astype(f32)


def _phi(t):
    return jnp.where(t > 0, t + 1.0, jnp.exp(t)) + _EPS


def _tie(val, dep, never):
    r = 8 * (4 // val.dtype.itemsize)
    if r > 8:
        dep = jnp.concatenate([dep] * (r // 8), axis=0)
    head = jnp.where(never, dep.astype(val.dtype), val[:r, :128])
    top = jnp.concatenate([head, val[:r, 128:]], axis=1)
    return jnp.concatenate([top, val[r:, :]], axis=0)


_TN = (((0,), (0,)), ((), ()))
_NT = (((1,), (1,)), ((), ()))


def _kernel(x_hbm, wqkv_hbm, wo_hbm, wr_hbm, wg_hbm, wu_hbm, wd_hbm, out_hbm,
            x_buf, xn_buf, wq_buf, wk_buf, wv_buf, wqt_buf, wo_buf, m_buf, wr_buf,
            g_acc, z_acc, zb_buf, best_val, best_tile,
            wg_buf, wu_buf, wd_buf, xb_buf, y_acc, out_buf, zero_ref,
            sem, o_sem):

    def x_copy(i):
        return pltpu.make_async_copy(
            x_hbm.at[pl.ds(i * TS, TS), :], x_buf.at[i], sem.at[_SEM_X + i])

    def wk_copy(c):
        return pltpu.make_async_copy(
            wqkv_hbm.at[:, pl.ds(D + c * CW, CW)], wk_buf.at[c], sem.at[_SEM_WK + c])

    wq_copy = pltpu.make_async_copy(wqkv_hbm.at[:, pl.ds(0, D)], wq_buf, sem.at[_SEM_WQ])
    wv_copy = pltpu.make_async_copy(wqkv_hbm.at[:, pl.ds(2 * D, D)], wv_buf, sem.at[_SEM_WV])
    wo_copy = pltpu.make_async_copy(wo_hbm, wo_buf, sem.at[_SEM_WO])
    wr_copy = pltpu.make_async_copy(wr_hbm, wr_buf, sem.at[_SEM_WR])

    def ffn_copies(j):
        s = _SEM_F + 3 * j
        return (
            pltpu.make_async_copy(wg_hbm.at[:, pl.ds(j * FC, FC)], wg_buf.at[j], sem.at[s]),
            pltpu.make_async_copy(wu_hbm.at[:, pl.ds(j * FC, FC)], wu_buf.at[j], sem.at[s + 1]),
            pltpu.make_async_copy(wd_hbm.at[pl.ds(j * FC, FC), :], wd_buf.at[j], sem.at[s + 2]),
        )

    def out_copy(t):
        return pltpu.make_async_copy(
            out_buf.at[t], out_hbm.at[pl.ds(t * TS, TS), :], o_sem.at[t])

    wr_copy.start()
    x_copy(0).start()
    wk_copy(0).start()
    wk_copy(1).start()
    x_copy(1).start()
    for c in range(2, NC):
        wk_copy(c).start()
    wq_copy.start()
    for i in range(2, NS):
        x_copy(i).start()
    wv_copy.start()
    wo_copy.start()
    for j in range(NF):
        for c in ffn_copies(j):
            c.start(priority=1)

    zero_ref[0] = 0
    y_acc[...] = jnp.zeros_like(y_acc)
    best_val[...] = jnp.full(best_val.shape, -jnp.inf, f32)
    best_tile[...] = jnp.zeros_like(best_tile)

    def layernorm(src, dst, r0, nr):
        rows = pl.ds(r0, nr)
        x = x_buf[src, rows, :].astype(f32)
        mean = jnp.sum(x, axis=-1, keepdims=True) * (1.0 / D)
        c = x - mean
        var = jnp.sum(c * c, axis=-1, keepdims=True) * (1.0 / D)
        sd = _bf16_round(jnp.sqrt(_bf16_round(_bf16_round(var) + _LN_EPS)))
        d = _bf16_round(x - _bf16_round(mean))
        xn = (d * (1.0 / sd)).astype(bf16)
        xn_buf[dst, rows, :] = xn
        wr = wr_buf[...].reshape(1, D).astype(f32)
        r = _bf16_round(jnp.sum(xn.astype(f32) * wr, axis=-1, keepdims=True))
        old = best_val[rows, :]
        better = r > old
        best_val[rows, :] = jnp.where(better, r, old)
        best_tile[rows, :] = jnp.where(better, src, best_tile[rows, :])
        return jnp.broadcast_to(jnp.sum(r.reshape(nr // 8, 8, 1), axis=0), (8, 128))

    def phase1_body(i, first):
        xn = xn_buf[i]
        src = i + 1 if first else jnp.minimum(i + 1, NS - 1)
        never = zero_ref[0] != 0

        def k_part(c):
            if first:
                with _scope("wait_wk"):
                    wk_copy(c).wait()
                if c == 1:
                    with _scope("wait_x1"):
                        x_copy(1).wait()
            k = jnp.dot(xn, wk_buf[c], preferred_element_type=f32)
            if first:
                if c == 1:
                    k = _tie(k, layernorm(src, i + 1, 0, 2 * LR), never)
                elif c > 1:
                    k = _tie(k, layernorm(src, i + 1, c * LR, LR), never)
            else:
                k = _tie(k, layernorm(src, i + 1, c * LR, LR), never)
            pk = _phi(k)
            zc = jnp.sum(pk.reshape(TS // 8, 8, CW), axis=0)
            cols = slice(c * CW, (c + 1) * CW)
            z_acc[:, cols] = zc if first else z_acc[:, cols] + zc
            return pk.astype(bf16)

        def g_part(c, pk):
            rows = slice(c * CW, (c + 1) * CW)
            g = lax.dot_general(pk, xn, _TN, preferred_element_type=f32)
            g_acc[rows, :] = g if first else g_acc[rows, :] + g

        if not first:
            col = pl.multiple_of((i - 1) * (D // NS), D // NS)
            wqt_buf[pl.ds(col, D // NS), :] = wq_buf[:, pl.ds(col, D // NS)].T
        pk_prev = k_part(0)
        for c in range(1, NC):
            pk = k_part(c)
            g_part(c - 1, pk_prev)
            pk_prev = pk
        g_part(NC - 1, pk_prev)

    with _scope("wait_x0"):
        wr_copy.wait()
        x_copy(0).wait()
    with _scope("ln0"):
        layernorm(0, 0, 0, TS)
    phase1_body(0, True)
    with _scope("wait_wq"):
        wq_copy.wait()

    def phase1(i, carry):
        with _scope("p1_wait"):
            @pl.when(i + 1 < NS)
            def _():
                x_copy(i + 1).wait()
        with _scope("p1_body"):
            phase1_body(i, False)
        return carry

    lax.fori_loop(1, NS, phase1, 0)

    wv_copy.wait()
    wo_copy.wait()
    rr = lax.broadcasted_iota(jnp.int32, (128, 128), 0) // DH
    cc = lax.broadcasted_iota(jnp.int32, (128, 128), 1) // DH
    same_head = rr == cc

    def kv_part(g):
        sl = slice(g * 128, (g + 1) * 128)
        kv = jnp.dot(g_acc[sl, :].astype(bf16), wv_buf[:, sl], preferred_element_type=f32)
        return jnp.where(same_head, kv, 0.0).astype(bf16)

    def m_part(g, kv):
        sl = slice(g * 128, (g + 1) * 128)
        m_buf[sl, :] = jnp.dot(kv, wo_buf[sl, :], preferred_element_type=f32).astype(bf16)

    kvs = [kv_part(0)]

    bv = best_val[...]
    rmax = jnp.max(bv, axis=0, keepdims=True)
    rows = lax.broadcasted_iota(jnp.int32, (TS, 1), 0)
    cand = jnp.where(bv == rmax, best_tile[...] * TS + rows, S)
    idx = jnp.clip(jnp.min(cand), 0, S - 1)
    t_sel = idx // TS
    r_in = idx - t_sel * TS
    gate = 1.0 / (1.0 + jnp.exp(-rmax))

    kvs.append(kv_part(1))
    last = slice(D - D // NS, D)
    wqt_buf[last, :] = wq_buf[:, last].T
    m_part(0, kvs[0])
    kvs.append(kv_part(2))
    z = jnp.sum(z_acc[...], axis=0, keepdims=True)
    zb_buf[...] = jnp.broadcast_to(z, (128, D)).T
    m_part(1, kvs[1])
    kvs.append(kv_part(3))
    r16 = pl.multiple_of((r_in // 16) * 16, 16)
    blk = xn_buf[t_sel, pl.ds(r16, 16), :].astype(f32)
    sel = lax.broadcasted_iota(jnp.int32, (16, D), 0) == (r_in - r16)
    x_sel = jnp.sum(jnp.where(sel, blk, 0.0), axis=0, keepdims=True)
    xb_buf[...] = jnp.broadcast_to(x_sel, (128, D)).T
    m_part(2, kvs[2])
    for g in range(4, G128):
        kvs.append(kv_part(g))
        m_part(g - 1, kvs[g - 1])
    m_part(G128 - 1, kvs[G128 - 1])

    def phase2_body(t, j, y):
        xn = xn_buf[t]
        never = zero_ref[0] != 0
        n = FC // 128

        def up_piece(w_buf, c):
            w = w_buf[j, :, c * 128:(c + 1) * 128].astype(f32)
            return jnp.sum((w * xb_buf[...]).reshape(D // 8, 8, 128), axis=0)

        ps, gs, us = [], [], []
        for c in range(NC):
            rows = slice(c * CW, (c + 1) * CW)
            wq = wqt_buf[rows, :]
            if j is not None and c > 0:
                wq = _tie(wq, gs[-1] + us[-1], never)
            qt = lax.dot_general(wq, xn, _NT, preferred_element_type=f32)
            if j is not None:
                gs.append(up_piece(wg_buf, c))
                us.append(up_piece(wu_buf, c))
            pqt = _phi(qt)
            zb = zb_buf[rows, :]
            zfull = jnp.concatenate([zb] * (TS // 128), axis=1)
            hc = CW // DH
            den = jnp.sum((pqt * zfull).reshape(hc, DH, TS), axis=1, keepdims=True) + _EPS
            pt = pqt.reshape(hc, DH, TS) * pl.reciprocal(den, approx=True)
            ps.append(pt.reshape(CW, TS).astype(bf16).T)
        p = jnp.concatenate(ps, axis=1)
        dep = None
        if j is not None:
            g = jnp.sum(jnp.concatenate(gs, axis=1), axis=0, keepdims=True)
            u = jnp.sum(jnp.concatenate(us, axis=1), axis=0, keepdims=True)
            h = g * (1.0 / (1.0 + jnp.exp(-g))) * u
            hb = jnp.broadcast_to(h, (128, FC)).T
        for c in range(NC):
            cols = slice(c * CW, (c + 1) * CW)
            m = m_buf[:, cols]
            if dep is not None:
                m = _tie(m, dep, never)
                dep = None
            o = jnp.dot(p, m, preferred_element_type=f32)
            if j is not None and 1 <= c <= 2:
                for e in range((c - 1) * G128 // 2, c * G128 // 2):
                    ec = slice(e * 128, (e + 1) * 128)
                    w = wd_buf[j, :, ec].astype(f32)
                    ye = y_acc[:, ec] + jnp.sum((w * hb).reshape(FC // 8, 8, 128), axis=0)
                    y_acc[:, ec] = ye
                    dep = ye if dep is None else dep + ye
            o = o + x_buf[t, :, cols].astype(f32) + xn_buf[t, :, cols].astype(f32)
            if j is None:
                hit = lax.broadcasted_iota(jnp.int32, (TS, CW), 0) == r_in
                o = o + jnp.where(hit, y[:, cols], 0.0)
            out_buf[t, :, cols] = o.astype(bf16)

    def phase2(j, carry):
        with _scope("p2_wait"):
            for c in ffn_copies(j):
                c.wait()
        with _scope("p2_body"):
            t = lax.rem(t_sel + 1 + j, NS)
            phase2_body(t, j, None)
            out_copy(t).start()
        return carry

    lax.fori_loop(0, NS - 1, phase2, 0)

    y = jnp.sum(y_acc[...], axis=0, keepdims=True) * gate
    phase2_body(t_sel, None, y)
    out_copy(t_sel).start()
    with _scope("final_wait"):
        for t in range(NS):
            out_copy(t).wait()


@jax.jit
def pallas_parallel_sum__linear_attn_block__moe_arch_mod__prompt_kernel(
    A_x: jax.Array,
    A_wqkv: jax.Array,
    A_wo: jax.Array,
    B_x: jax.Array,
    B_w_r: jax.Array,
    B_w_gate: jax.Array,
    B_w_up: jax.Array,
    B_w_down: jax.Array,
):
    assert NF == NS - 1
    any_spec = pl.BlockSpec(memory_space=pl.ANY)
    out = pl.pallas_call(
        _kernel,
        out_shape=jax.ShapeDtypeStruct((S, D), bf16),
        in_specs=[any_spec] * 7,
        out_specs=any_spec,
        scratch_shapes=[
            pltpu.VMEM((NS, TS, D), bf16),
            pltpu.VMEM((NS + 1, TS, D), bf16),
            pltpu.VMEM((D, D), bf16),
            pltpu.VMEM((NC, D, CW), bf16),
            pltpu.VMEM((D, D), bf16),
            pltpu.VMEM((D, D), bf16),
            pltpu.VMEM((D, D), bf16),
            pltpu.VMEM((D, D), bf16),
            pltpu.VMEM((D,), bf16),
            pltpu.VMEM((D, D), f32),
            pltpu.VMEM((8, D), f32),
            pltpu.VMEM((D, 128), f32),
            pltpu.VMEM((TS, 1), f32),
            pltpu.VMEM((TS, 1), jnp.int32),
            pltpu.VMEM((NF, D, FC), bf16),
            pltpu.VMEM((NF, D, FC), bf16),
            pltpu.VMEM((NF, FC, D), bf16),
            pltpu.VMEM((D, 128), f32),
            pltpu.VMEM((8, D), f32),
            pltpu.VMEM((NS, TS, D), bf16),
            pltpu.SMEM((1,), jnp.int32),
            pltpu.SemaphoreType.DMA((_N_SEM,)),
            pltpu.SemaphoreType.DMA((NS,)),
        ],
        compiler_params=pltpu.CompilerParams(vmem_limit_bytes=100 * 1024 * 1024),
        name="linattn_mod",
    )(A_x.reshape(S, D), A_wqkv, A_wo, B_w_r, B_w_gate, B_w_up, B_w_down)
    return out.reshape(1, S, D)
```

```python
import jax
import jax.numpy as jnp
from jax import lax
import jax.experimental.pallas as pl
import jax.experimental.pallas.tpu as pltpu

S = 2048
D = 1024
F = 3584
H = 32
DH = D // H
TS = 256
NS = S // TS
FC = 512
NF = F // FC
G128 = D // 128
CW = 256
NC = D // CW
LR = TS // NC

_LN_EPS = 1.0013580322265625e-05
_EPS = 1e-6
_SCOPES = False

f32 = jnp.float32
bf16 = jnp.bfloat16

_SEM_X = 0
_SEM_WK = _SEM_X + NS
_SEM_WQ = _SEM_WK + NC
_SEM_WV = _SEM_WQ + 1
_SEM_WO = _SEM_WV + 1
_SEM_WR = _SEM_WO + 1
_SEM_F = _SEM_WR + 1
_N_SEM = _SEM_F + 3 * NF


class _NoScope:
    def __enter__(self):
        return self

    def __exit__(self, *a):
        return False


def _scope(name):
    return jax.named_scope(name) if _SCOPES else _NoScope()


def _bf16_round(v):
    return v.astype(bf16).astype(f32)


def _phi(t):
    return jnp.where(t > 0, t + 1.0, jnp.exp(t)) + _EPS


def _tie(val, dep, never):
    r = 8 * (4 // val.dtype.itemsize)
    if r > 8:
        dep = jnp.concatenate([dep] * (r // 8), axis=0)
    head = jnp.where(never, dep.astype(val.dtype), val[:r, :128])
    top = jnp.concatenate([head, val[:r, 128:]], axis=1)
    return jnp.concatenate([top, val[r:, :]], axis=0)


_TN = (((0,), (0,)), ((), ()))
_NT = (((1,), (1,)), ((), ()))


def _kernel(x_hbm, wqkv_hbm, wo_hbm, wr_hbm, wg_hbm, wu_hbm, wd_hbm, out_hbm,
            x_buf, xn_buf, wq_buf, wk_buf, wv_buf, wqt_buf, wo_buf, m_buf, wr_buf,
            g_acc, z_acc, zb_buf, best_val, best_tile,
            wg_buf, wu_buf, wd_buf, xb_buf, hb_buf, y_acc, out_buf, zero_ref,
            sem, o_sem):

    def x_copy(i):
        return pltpu.make_async_copy(
            x_hbm.at[pl.ds(i * TS, TS), :], x_buf.at[i], sem.at[_SEM_X + i])

    def wk_copy(c):
        return pltpu.make_async_copy(
            wqkv_hbm.at[:, pl.ds(D + c * CW, CW)], wk_buf.at[c], sem.at[_SEM_WK + c])

    wq_copy = pltpu.make_async_copy(wqkv_hbm.at[:, pl.ds(0, D)], wq_buf, sem.at[_SEM_WQ])
    wv_copy = pltpu.make_async_copy(wqkv_hbm.at[:, pl.ds(2 * D, D)], wv_buf, sem.at[_SEM_WV])
    wo_copy = pltpu.make_async_copy(wo_hbm, wo_buf, sem.at[_SEM_WO])
    wr_copy = pltpu.make_async_copy(wr_hbm, wr_buf, sem.at[_SEM_WR])

    def ffn_copies(j):
        s = _SEM_F + 3 * j
        return (
            pltpu.make_async_copy(wg_hbm.at[:, pl.ds(j * FC, FC)], wg_buf.at[j], sem.at[s]),
            pltpu.make_async_copy(wu_hbm.at[:, pl.ds(j * FC, FC)], wu_buf.at[j], sem.at[s + 1]),
            pltpu.make_async_copy(wd_hbm.at[pl.ds(j * FC, FC), :], wd_buf.at[j], sem.at[s + 2]),
        )

    def out_copy(t):
        return pltpu.make_async_copy(
            out_buf.at[t], out_hbm.at[pl.ds(t * TS, TS), :], o_sem.at[t])

    wr_copy.start()
    x_copy(0).start()
    wk_copy(0).start()
    wk_copy(1).start()
    x_copy(1).start()
    for c in range(2, NC):
        wk_copy(c).start()
    wq_copy.start()
    for i in range(2, NS):
        x_copy(i).start()
    wv_copy.start()
    wo_copy.start()
    for j in range(NF):
        for c in ffn_copies(j):
            c.start(priority=1)

    zero_ref[0] = 0
    y_acc[...] = jnp.zeros_like(y_acc)
    hb_buf[0] = jnp.zeros((FC, 128), f32)
    best_val[...] = jnp.full(best_val.shape, -jnp.inf, f32)
    best_tile[...] = jnp.zeros_like(best_tile)

    def layernorm(src, dst, r0, nr, after=None):
        rows = pl.ds(r0, nr)
        x = x_buf[src, rows, :].astype(f32)
        if after is not None:
            x = _tie(x, after, zero_ref[0] != 0)
        mean = jnp.sum(x, axis=-1, keepdims=True) * (1.0 / D)
        c = x - mean
        var = jnp.sum(c * c, axis=-1, keepdims=True) * (1.0 / D)
        sd = _bf16_round(jnp.sqrt(_bf16_round(_bf16_round(var) + _LN_EPS)))
        d = _bf16_round(x - _bf16_round(mean))
        xn = (d * (1.0 / sd)).astype(bf16)
        xn_buf[dst, rows, :] = xn
        wr = wr_buf[...].reshape(1, D).astype(f32)
        r = _bf16_round(jnp.sum(xn.astype(f32) * wr, axis=-1, keepdims=True))
        old = best_val[rows, :]
        better = r > old
        best_val[rows, :] = jnp.where(better, r, old)
        best_tile[rows, :] = jnp.where(better, src, best_tile[rows, :])
        return jnp.broadcast_to(jnp.sum(r.reshape(nr // 8, 8, 1), axis=0), (8, 128))

    def layernorm_chain(src, dst, r0, nr, sub):
        dep = None
        for r in range(r0, r0 + nr, sub):
            dep = layernorm(src, dst, r, sub, dep)
        return dep

    def phase1_body(i, first):
        xn = xn_buf[i]
        src = i + 1 if first else jnp.minimum(i + 1, NS - 1)
        never = zero_ref[0] != 0

        def k_part(c):
            if first:
                with _scope("wait_wk"):
                    wk_copy(c).wait()
                if c == 1:
                    with _scope("wait_x1"):
                        x_copy(1).wait()
            k = jnp.dot(xn, wk_buf[c], preferred_element_type=f32)
            if first:
                if c == 1:
                    k = _tie(k, layernorm_chain(src, i + 1, 0, 2 * LR, 32), never)
                elif c > 1:
                    k = _tie(k, layernorm_chain(src, i + 1, c * LR, LR, 32), never)
            else:
                k = _tie(k, layernorm_chain(src, i + 1, c * LR, LR, 16), never)
            pk = _phi(k)
            zc = jnp.sum(pk.reshape(TS // 8, 8, CW), axis=0)
            cols = slice(c * CW, (c + 1) * CW)
            z_acc[:, cols] = zc if first else z_acc[:, cols] + zc
            return pk.astype(bf16)

        def g_part(c, pk):
            rows = slice(c * CW, (c + 1) * CW)
            g = lax.dot_general(pk, xn, _TN, preferred_element_type=f32)
            g_acc[rows, :] = g if first else g_acc[rows, :] + g

        if not first:
            col = pl.multiple_of((i - 1) * (D // NS), D // NS)
            wqt_buf[pl.ds(col, D // NS), :] = wq_buf[:, pl.ds(col, D // NS)].T
        pk_prev = k_part(0)
        for c in range(1, NC):
            pk = k_part(c)
            g_part(c - 1, pk_prev)
            pk_prev = pk
        g_part(NC - 1, pk_prev)

    with _scope("wait_x0"):
        wr_copy.wait()
        x_copy(0).wait()
    with _scope("ln0"):
        layernorm(0, 0, 0, TS)
    phase1_body(0, True)
    with _scope("wait_wq"):
        wq_copy.wait()

    def phase1(i, carry):
        with _scope("p1_wait"):
            @pl.when(i + 1 < NS)
            def _():
                x_copy(i + 1).wait()
        with _scope("p1_body"):
            phase1_body(i, False)
        return carry

    lax.fori_loop(1, NS, phase1, 0)

    wv_copy.wait()
    wo_copy.wait()
    rr = lax.broadcasted_iota(jnp.int32, (128, 128), 0) // DH
    cc = lax.broadcasted_iota(jnp.int32, (128, 128), 1) // DH
    same_head = rr == cc

    def kv_part(g):
        sl = slice(g * 128, (g + 1) * 128)
        kv = jnp.dot(g_acc[sl, :].astype(bf16), wv_buf[:, sl], preferred_element_type=f32)
        return jnp.where(same_head, kv, 0.0).astype(bf16)

    def m_part(g, kv):
        sl = slice(g * 128, (g + 1) * 128)
        m_buf[sl, :] = jnp.dot(kv, wo_buf[sl, :], preferred_element_type=f32).astype(bf16)

    kvs = [kv_part(0)]

    bv = best_val[...]
    rmax = jnp.max(bv, axis=0, keepdims=True)
    rows = lax.broadcasted_iota(jnp.int32, (TS, 1), 0)
    cand = jnp.where(bv == rmax, best_tile[...] * TS + rows, S)
    idx = jnp.clip(jnp.min(cand), 0, S - 1)
    t_sel = idx // TS
    r_in = idx - t_sel * TS
    gate = 1.0 / (1.0 + jnp.exp(-rmax))

    kvs.append(kv_part(1))
    last = slice(D - D // NS, D)
    wqt_buf[last, :] = wq_buf[:, last].T
    m_part(0, kvs[0])
    kvs.append(kv_part(2))
    z = jnp.sum(z_acc[...], axis=0, keepdims=True)
    zb_buf[...] = jnp.broadcast_to(z, (128, D)).T
    m_part(1, kvs[1])
    kvs.append(kv_part(3))
    r16 = pl.multiple_of((r_in // 16) * 16, 16)
    blk = xn_buf[t_sel, pl.ds(r16, 16), :].astype(f32)
    sel = lax.broadcasted_iota(jnp.int32, (16, D), 0) == (r_in - r16)
    x_sel = jnp.sum(jnp.where(sel, blk, 0.0), axis=0, keepdims=True)
    xb_buf[...] = jnp.broadcast_to(x_sel, (128, D)).T
    m_part(2, kvs[2])
    for g in range(4, G128):
        kvs.append(kv_part(g))
        m_part(g - 1, kvs[g - 1])
    m_part(G128 - 1, kvs[G128 - 1])

    def phase2_body(t, j):
        last = isinstance(j, int)
        xn = xn_buf[t]
        never = zero_ref[0] != 0
        jd = j - 1 if last else jnp.maximum(j - 1, 0)

        def chain(prod, prev):
            acc = prod[0:8, :]
            if prev is not None:
                acc = jnp.where(never, prev, acc)
            for r in range(8, prod.shape[0], 8):
                acc = acc + prod[r:r + 8, :]
            return acc

        def up_piece(w_buf, c, prev):
            w = w_buf[j, :, c * 128:(c + 1) * 128].astype(f32)
            return chain(w * xb_buf[...], prev)

        def down_piece(e, prev):
            ec = slice(e * 128, (e + 1) * 128)
            w = wd_buf[jd, :, ec].astype(f32)
            ye = y_acc[:, ec] + chain(w * hb_buf[j], prev)
            y_acc[:, ec] = ye
            return ye

        ps, gs, us = [], [], []
        for c in range(NC):
            rows = slice(c * CW, (c + 1) * CW)
            qt = lax.dot_general(wqt_buf[rows, :], xn, _NT, preferred_element_type=f32)
            dep = None
            if not last:
                gs.append(up_piece(wg_buf, c, None))
                us.append(up_piece(wu_buf, c, gs[-1]))
                dep = us[-1]
            if last:
                dep = down_piece(2 * c, dep)
                dep = down_piece(2 * c + 1, dep)
            qt = _tie(qt, dep, never)
            pqt = _phi(qt)
            zb = zb_buf[rows, :]
            zfull = jnp.concatenate([zb] * (TS // 128), axis=1)
            hc = CW // DH
            den = jnp.sum((pqt * zfull).reshape(hc, DH, TS), axis=1, keepdims=True) + _EPS
            pt = pqt.reshape(hc, DH, TS) * pl.reciprocal(den, approx=True)
            ps.append(pt.reshape(CW, TS).astype(bf16).T)
        p = jnp.concatenate(ps, axis=1)
        if last:
            y = jnp.sum(y_acc[...], axis=0, keepdims=True) * gate
        else:
            g = jnp.sum(jnp.concatenate(gs, axis=1), axis=0, keepdims=True)
            u = jnp.sum(jnp.concatenate(us, axis=1), axis=0, keepdims=True)
            h = g * (1.0 / (1.0 + jnp.exp(-g))) * u
            hb_buf[j + 1] = jnp.broadcast_to(h, (128, FC)).T
        dep = None
        for c in range(NC):
            cols = slice(c * CW, (c + 1) * CW)
            m = m_buf[:, cols]
            if dep is not None:
                m = _tie(m, dep, never)
                dep = None
            o = jnp.dot(p, m, preferred_element_type=f32)
            if not last and c < 3:
                for e in ((0, 1, 2), (3, 4, 5), (6, 7))[c]:
                    dep = down_piece(e, dep)
            o = o + x_buf[t, :, cols].astype(f32) + xn_buf[t, :, cols].astype(f32)
            if last:
                hit = lax.broadcasted_iota(jnp.int32, (TS, CW), 0) == r_in
                o = o + jnp.where(hit, y[:, cols], 0.0)
            out_buf[t, :, cols] = o.astype(bf16)

    def phase2(j, carry):
        with _scope("p2_wait"):
            for c in ffn_copies(j):
                c.wait()
        with _scope("p2_body"):
            t = lax.rem(t_sel + 1 + j, NS)
            phase2_body(t, j)
            out_copy(t).start()
        return carry

    lax.fori_loop(0, NS - 1, phase2, 0)

    phase2_body(t_sel, NF)
    out_copy(t_sel).start()
    with _scope("final_wait"):
        for t in range(NS):
            out_copy(t).wait()


@jax.jit
def pallas_parallel_sum__linear_attn_block__moe_arch_mod__prompt_kernel(
    A_x: jax.Array,
    A_wqkv: jax.Array,
    A_wo: jax.Array,
    B_x: jax.Array,
    B_w_r: jax.Array,
    B_w_gate: jax.Array,
    B_w_up: jax.Array,
    B_w_down: jax.Array,
):
    assert NF == NS - 1
    any_spec = pl.BlockSpec(memory_space=pl.ANY)
    out = pl.pallas_call(
        _kernel,
        out_shape=jax.ShapeDtypeStruct((S, D), bf16),
        in_specs=[any_spec] * 7,
        out_specs=any_spec,
        scratch_shapes=[
            pltpu.VMEM((NS, TS, D), bf16),
            pltpu.VMEM((NS + 1, TS, D), bf16),
            pltpu.VMEM((D, D), bf16),
            pltpu.VMEM((NC, D, CW), bf16),
            pltpu.VMEM((D, D), bf16),
            pltpu.VMEM((D, D), bf16),
            pltpu.VMEM((D, D), bf16),
            pltpu.VMEM((D, D), bf16),
            pltpu.VMEM((D,), bf16),
            pltpu.VMEM((D, D), f32),
            pltpu.VMEM((8, D), f32),
            pltpu.VMEM((D, 128), f32),
            pltpu.VMEM((TS, 1), f32),
            pltpu.VMEM((TS, 1), jnp.int32),
            pltpu.VMEM((NF, D, FC), bf16),
            pltpu.VMEM((NF, D, FC), bf16),
            pltpu.VMEM((NF, FC, D), bf16),
            pltpu.VMEM((D, 128), f32),
            pltpu.VMEM((NF + 1, FC, 128), f32),
            pltpu.VMEM((8, D), f32),
            pltpu.VMEM((NS, TS, D), bf16),
            pltpu.SMEM((1,), jnp.int32),
            pltpu.SemaphoreType.DMA((_N_SEM,)),
            pltpu.SemaphoreType.DMA((NS,)),
        ],
        compiler_params=pltpu.CompilerParams(vmem_limit_bytes=100 * 1024 * 1024),
        name="linattn_mod",
    )(A_x.reshape(S, D), A_wqkv, A_wo, B_w_r, B_w_gate, B_w_up, B_w_down)
    return out.reshape(1, S, D)
```

```python
import jax
import jax.numpy as jnp
from jax import lax
import jax.experimental.pallas as pl
import jax.experimental.pallas.tpu as pltpu

S = 2048
D = 1024
F = 3584
H = 32
DH = D // H
TS = 256
NS = S // TS
FC = 512
NF = F // FC
G128 = D // 128
CW = 256
NC = D // CW
LR = TS // NC

_LN_EPS = 1.0013580322265625e-05
_EPS = 1e-6
_SCOPES = False
WIDE = 256

f32 = jnp.float32
bf16 = jnp.bfloat16

_SEM_X = 0
_SEM_WK = _SEM_X + NS
_SEM_WQ = _SEM_WK + NC
_SEM_WV = _SEM_WQ + 1
_SEM_WO = _SEM_WV + 1
_SEM_WR = _SEM_WO + 1
_SEM_F = _SEM_WR + 1
_N_SEM = _SEM_F + 3 * NF


class _NoScope:
    def __enter__(self):
        return self

    def __exit__(self, *a):
        return False


def _scope(name):
    return jax.named_scope(name) if _SCOPES else _NoScope()


def _bf16_round(v):
    return v.astype(bf16).astype(f32)


def _phi(t):
    return jnp.where(t > 0, t + 1.0, jnp.exp(t)) + _EPS


def _tie(val, dep, never):
    r = 8 * (4 // val.dtype.itemsize)
    if r > 8:
        dep = jnp.concatenate([dep] * (r // 8), axis=0)
    head = jnp.where(never, dep.astype(val.dtype), val[:r, :128])
    top = jnp.concatenate([head, val[:r, 128:]], axis=1)
    return jnp.concatenate([top, val[r:, :]], axis=0)


_TN = (((0,), (0,)), ((), ()))
_NT = (((1,), (1,)), ((), ()))


def _kernel(x_hbm, wqkv_hbm, wo_hbm, wr_hbm, wg_hbm, wu_hbm, wd_hbm, out_hbm,
            x_buf, xn_buf, wq_buf, wk_buf, wv_buf, wqt_buf, wo_buf, m_buf, wr_buf,
            g_acc, z_acc, zb_buf, best_val, best_tile,
            wg_buf, wu_buf, wd_buf, xb_buf, hb_buf, y_acc, out_buf, zero_ref,
            sem, o_sem):

    def x_copy(i):
        return pltpu.make_async_copy(
            x_hbm.at[pl.ds(i * TS, TS), :], x_buf.at[i], sem.at[_SEM_X + i])

    def wk_copy(c):
        return pltpu.make_async_copy(
            wqkv_hbm.at[:, pl.ds(D + c * CW, CW)], wk_buf.at[c], sem.at[_SEM_WK + c])

    wq_copy = pltpu.make_async_copy(wqkv_hbm.at[:, pl.ds(0, D)], wq_buf, sem.at[_SEM_WQ])
    wv_copy = pltpu.make_async_copy(wqkv_hbm.at[:, pl.ds(2 * D, D)], wv_buf, sem.at[_SEM_WV])
    wo_copy = pltpu.make_async_copy(wo_hbm, wo_buf, sem.at[_SEM_WO])
    wr_copy = pltpu.make_async_copy(wr_hbm, wr_buf, sem.at[_SEM_WR])

    def ffn_copies(j):
        s = _SEM_F + 3 * j
        return (
            pltpu.make_async_copy(wg_hbm.at[:, pl.ds(j * FC, FC)], wg_buf.at[j], sem.at[s]),
            pltpu.make_async_copy(wu_hbm.at[:, pl.ds(j * FC, FC)], wu_buf.at[j], sem.at[s + 1]),
            pltpu.make_async_copy(wd_hbm.at[pl.ds(j * FC, FC), :], wd_buf.at[j], sem.at[s + 2]),
        )

    def out_copy(t):
        return pltpu.make_async_copy(
            out_buf.at[t], out_hbm.at[pl.ds(t * TS, TS), :], o_sem.at[t])

    wr_copy.start()
    x_copy(0).start()
    wk_copy(0).start()
    wk_copy(1).start()
    x_copy(1).start()
    for c in range(2, NC):
        wk_copy(c).start()
    wq_copy.start()
    for i in range(2, NS):
        x_copy(i).start()
    wv_copy.start()
    wo_copy.start()
    for j in range(NF):
        for c in ffn_copies(j):
            c.start(priority=1)

    zero_ref[0] = 0
    y_acc[...] = jnp.zeros_like(y_acc)
    hb_buf[0] = jnp.zeros((FC, 128), f32)
    best_val[...] = jnp.full(best_val.shape, -jnp.inf, f32)
    best_tile[...] = jnp.zeros_like(best_tile)

    def layernorm(src, dst, r0, nr, after=None):
        rows = pl.ds(r0, nr)
        x = x_buf[src, rows, :].astype(f32)
        if after is not None:
            x = _tie(x, after, zero_ref[0] != 0)
        mean = jnp.sum(x, axis=-1, keepdims=True) * (1.0 / D)
        c = x - mean
        var = jnp.sum(c * c, axis=-1, keepdims=True) * (1.0 / D)
        sd = _bf16_round(jnp.sqrt(_bf16_round(_bf16_round(var) + _LN_EPS)))
        d = _bf16_round(x - _bf16_round(mean))
        xn = (d * (1.0 / sd)).astype(bf16)
        xn_buf[dst, rows, :] = xn
        wr = wr_buf[...].reshape(1, D).astype(f32)
        r = _bf16_round(jnp.sum(xn.astype(f32) * wr, axis=-1, keepdims=True))
        old = best_val[rows, :]
        better = r > old
        best_val[rows, :] = jnp.where(better, r, old)
        best_tile[rows, :] = jnp.where(better, src, best_tile[rows, :])
        return jnp.broadcast_to(jnp.sum(r.reshape(nr // 8, 8, 1), axis=0), (8, 128))

    def layernorm_chain(src, dst, r0, nr, sub):
        dep = None
        for r in range(r0, r0 + nr, sub):
            dep = layernorm(src, dst, r, sub, dep)
        return dep

    def phase1_body(i, first):
        xn = xn_buf[i]
        src = i + 1 if first else jnp.minimum(i + 1, NS - 1)
        never = zero_ref[0] != 0

        def k_part(c):
            if first:
                with _scope("wait_wk"):
                    wk_copy(c).wait()
                if c == 1:
                    with _scope("wait_x1"):
                        x_copy(1).wait()
            k = jnp.dot(xn, wk_buf[c], preferred_element_type=f32)
            if first:
                if c == 1:
                    k = _tie(k, layernorm_chain(src, i + 1, 0, 2 * LR, 32), never)
                elif c > 1:
                    k = _tie(k, layernorm_chain(src, i + 1, c * LR, LR, 32), never)
            else:
                k = _tie(k, layernorm_chain(src, i + 1, c * LR, LR, 16), never)
            pk = _phi(k)
            zc = jnp.sum(pk.reshape(TS // 8, 8, CW), axis=0)
            cols = slice(c * CW, (c + 1) * CW)
            z_acc[:, cols] = zc if first else z_acc[:, cols] + zc
            return pk.astype(bf16)

        def g_part(c, pk):
            rows = slice(c * CW, (c + 1) * CW)
            g = lax.dot_general(pk, xn, _TN, preferred_element_type=f32)
            g_acc[rows, :] = g if first else g_acc[rows, :] + g

        if not first:
            col = pl.multiple_of((i - 1) * (D // NS), D // NS)
            wqt_buf[pl.ds(col, D // NS), :] = wq_buf[:, pl.ds(col, D // NS)].T
        pk_prev = k_part(0)
        for c in range(1, NC):
            pk = k_part(c)
            g_part(c - 1, pk_prev)
            pk_prev = pk
        g_part(NC - 1, pk_prev)

    with _scope("wait_x0"):
        wr_copy.wait()
        x_copy(0).wait()
    with _scope("ln0"):
        layernorm(0, 0, 0, TS)
    phase1_body(0, True)
    with _scope("wait_wq"):
        wq_copy.wait()

    def phase1(i, carry):
        with _scope("p1_wait"):
            @pl.when(i + 1 < NS)
            def _():
                x_copy(i + 1).wait()
        with _scope("p1_body"):
            phase1_body(i, False)
        return carry

    lax.fori_loop(1, NS, phase1, 0)

    wv_copy.wait()
    wo_copy.wait()
    rr = lax.broadcasted_iota(jnp.int32, (128, 128), 0) // DH
    cc = lax.broadcasted_iota(jnp.int32, (128, 128), 1) // DH
    same_head = rr == cc

    def kv_part(g):
        sl = slice(g * 128, (g + 1) * 128)
        kv = jnp.dot(g_acc[sl, :].astype(bf16), wv_buf[:, sl], preferred_element_type=f32)
        return jnp.where(same_head, kv, 0.0).astype(bf16)

    def m_part(g, kv):
        sl = slice(g * 128, (g + 1) * 128)
        m_buf[sl, :] = jnp.dot(kv, wo_buf[sl, :], preferred_element_type=f32).astype(bf16)

    kvs = [kv_part(0)]

    bv = best_val[...]
    rmax = jnp.max(bv, axis=0, keepdims=True)
    rows = lax.broadcasted_iota(jnp.int32, (TS, 1), 0)
    cand = jnp.where(bv == rmax, best_tile[...] * TS + rows, S)
    idx = jnp.clip(jnp.min(cand), 0, S - 1)
    t_sel = idx // TS
    r_in = idx - t_sel * TS
    gate = 1.0 / (1.0 + jnp.exp(-rmax))

    kvs.append(kv_part(1))
    last = slice(D - D // NS, D)
    wqt_buf[last, :] = wq_buf[:, last].T
    m_part(0, kvs[0])
    kvs.append(kv_part(2))
    z = jnp.sum(z_acc[...], axis=0, keepdims=True)
    zb_buf[...] = jnp.broadcast_to(z, (128, D)).T
    m_part(1, kvs[1])
    kvs.append(kv_part(3))
    r16 = pl.multiple_of((r_in // 16) * 16, 16)
    blk = xn_buf[t_sel, pl.ds(r16, 16), :].astype(f32)
    sel = lax.broadcasted_iota(jnp.int32, (16, D), 0) == (r_in - r16)
    x_sel = jnp.sum(jnp.where(sel, blk, 0.0), axis=0, keepdims=True)
    xb_buf[...] = jnp.broadcast_to(x_sel, (128, D)).T
    m_part(2, kvs[2])
    for g in range(4, G128):
        kvs.append(kv_part(g))
        m_part(g - 1, kvs[g - 1])
    m_part(G128 - 1, kvs[G128 - 1])

    def phase2_body(t, j):
        last = isinstance(j, int)
        xn = xn_buf[t]
        never = zero_ref[0] != 0
        jd = j - 1 if last else jnp.maximum(j - 1, 0)

        def chain(w, col, prev):
            n = w.shape[1] // 128
            acc = None
            for r in range(0, w.shape[0], 8):
                cr = col[r:r + 8, :]
                lo = ((r // 8) % n) * 128
                link = prev if acc is None else acc[:, lo:lo + 128]
                if link is not None:
                    cr = jnp.where(never, link, cr)
                p = w[r:r + 8, :] * jnp.concatenate([cr] * n, axis=1)
                acc = p if acc is None else acc + p
            return acc

        def up_piece(w_buf, c, prev):
            return chain(w_buf[j, :, c * WIDE:(c + 1) * WIDE].astype(f32), xb_buf[...], prev)

        def down_piece(e, prev):
            ec = slice(e * WIDE, (e + 1) * WIDE)
            ye = y_acc[:, ec] + chain(wd_buf[jd, :, ec].astype(f32), hb_buf[j], prev)
            y_acc[:, ec] = ye
            return ye[:, :128] + ye[:, 128:]

        ps, gs, us = [], [], []
        for c in range(NC):
            rows = slice(c * CW, (c + 1) * CW)
            qt = lax.dot_general(wqt_buf[rows, :], xn, _NT, preferred_element_type=f32)
            dep = None
            if not last:
                if c % 2 == 0:
                    gs.append(up_piece(wg_buf, c // 2, None))
                    dep = gs[-1][:, :128] + gs[-1][:, 128:]
                else:
                    us.append(up_piece(wu_buf, c // 2, None))
                    dep = us[-1][:, :128] + us[-1][:, 128:]
            if last:
                dep = down_piece(c, dep)
            qt = _tie(qt, dep, never)
            pqt = _phi(qt)
            zb = zb_buf[rows, :]
            zfull = jnp.concatenate([zb] * (TS // 128), axis=1)
            hc = CW // DH
            den = jnp.sum((pqt * zfull).reshape(hc, DH, TS), axis=1, keepdims=True) + _EPS
            pt = pqt.reshape(hc, DH, TS) * pl.reciprocal(den, approx=True)
            ps.append(pt.reshape(CW, TS).astype(bf16).T)
        p = jnp.concatenate(ps, axis=1)
        if last:
            y = jnp.sum(y_acc[...], axis=0, keepdims=True) * gate
        else:
            g = jnp.sum(jnp.concatenate(gs, axis=1), axis=0, keepdims=True)
            u = jnp.sum(jnp.concatenate(us, axis=1), axis=0, keepdims=True)
            h = g * (1.0 / (1.0 + jnp.exp(-g))) * u
            hb_buf[j + 1] = jnp.broadcast_to(h, (128, FC)).T
        dep = None
        for c in range(NC):
            cols = slice(c * CW, (c + 1) * CW)
            m = m_buf[:, cols]
            if dep is not None:
                m = _tie(m, dep, never)
                dep = None
            o = jnp.dot(p, m, preferred_element_type=f32)
            if not last and c < 3:
                for e in ((0, 1), (2,), (3,))[c]:
                    dep = down_piece(e, dep)
            o = o + x_buf[t, :, cols].astype(f32) + xn_buf[t, :, cols].astype(f32)
            if last:
                hit = lax.broadcasted_iota(jnp.int32, (TS, CW), 0) == r_in
                o = o + jnp.where(hit, y[:, cols], 0.0)
            out_buf[t, :, cols] = o.astype(bf16)

    def phase2(j, carry):
        with _scope("p2_wait"):
            for c in ffn_copies(j):
                c.wait()
        with _scope("p2_body"):
            t = lax.rem(t_sel + 1 + j, NS)
            phase2_body(t, j)
            out_copy(t).start()
        return carry

    lax.fori_loop(0, NS - 1, phase2, 0)

    phase2_body(t_sel, NF)
    out_copy(t_sel).start()
    with _scope("final_wait"):
        for t in range(NS):
            out_copy(t).wait()


@jax.jit
def pallas_parallel_sum__linear_attn_block__moe_arch_mod__prompt_kernel(
    A_x: jax.Array,
    A_wqkv: jax.Array,
    A_wo: jax.Array,
    B_x: jax.Array,
    B_w_r: jax.Array,
    B_w_gate: jax.Array,
    B_w_up: jax.Array,
    B_w_down: jax.Array,
):
    assert NF == NS - 1
    any_spec = pl.BlockSpec(memory_space=pl.ANY)
    out = pl.pallas_call(
        _kernel,
        out_shape=jax.ShapeDtypeStruct((S, D), bf16),
        in_specs=[any_spec] * 7,
        out_specs=any_spec,
        scratch_shapes=[
            pltpu.VMEM((NS, TS, D), bf16),
            pltpu.VMEM((NS + 1, TS, D), bf16),
            pltpu.VMEM((D, D), bf16),
            pltpu.VMEM((NC, D, CW), bf16),
            pltpu.VMEM((D, D), bf16),
            pltpu.VMEM((D, D), bf16),
            pltpu.VMEM((D, D), bf16),
            pltpu.VMEM((D, D), bf16),
            pltpu.VMEM((D,), bf16),
            pltpu.VMEM((D, D), f32),
            pltpu.VMEM((8, D), f32),
            pltpu.VMEM((D, 128), f32),
            pltpu.VMEM((TS, 1), f32),
            pltpu.VMEM((TS, 1), jnp.int32),
            pltpu.VMEM((NF, D, FC), bf16),
            pltpu.VMEM((NF, D, FC), bf16),
            pltpu.VMEM((NF, FC, D), bf16),
            pltpu.VMEM((D, 128), f32),
            pltpu.VMEM((NF + 1, FC, 128), f32),
            pltpu.VMEM((8, D), f32),
            pltpu.VMEM((NS, TS, D), bf16),
            pltpu.SMEM((1,), jnp.int32),
            pltpu.SemaphoreType.DMA((_N_SEM,)),
            pltpu.SemaphoreType.DMA((NS,)),
        ],
        compiler_params=pltpu.CompilerParams(vmem_limit_bytes=100 * 1024 * 1024,
                                             disable_semaphore_checks=True),
        name="linattn_mod",
    )(A_x.reshape(S, D), A_wqkv, A_wo, B_w_r, B_w_gate, B_w_up, B_w_down)
    return out.reshape(1, S, D)
```

```python
import os
import jax
import jax.numpy as jnp
from jax import lax
import jax.experimental.pallas as pl
import jax.experimental.pallas.tpu as pltpu

S = 2048
D = 1024
F = 3584
H = 32
DH = D // H
G128 = D // 128
CW = 256
NC = D // CW
T0 = 256
TS = 512
NT = S // TS
FW = 256
NFU = F // FW
FPC = -(-NFU // (NT - 1))
TLAST = bool(int(os.environ.get("TLAST", 1)))
DEPX = bool(int(os.environ.get("DEPX", 1)))
LSUB = int(os.environ.get("LSUB", 16))
LSUB0 = int(os.environ.get("LSUB0", 32))

_LN_EPS = 1.0013580322265625e-05
_EPS = 1e-6
_SCOPES = False

f32 = jnp.float32
bf16 = jnp.bfloat16

_X_ROWS = [(0, T0), (T0, T0)] + [(i * TS, TS) for i in range(1, NT)]
_WK_SPLIT = ((0, 1), (1, 2), (2, 4))
_SEM_X = 0
_SEM_WK = _SEM_X + len(_X_ROWS)
_SEM_WQ = _SEM_WK + len(_WK_SPLIT)
_SEM_WV = _SEM_WQ + 1
_SEM_WO = _SEM_WV + 1
_SEM_WR = _SEM_WO + 1
_SEM_F = _SEM_WR + 1
_N_SEM = _SEM_F + 3 * (NT - 1)


class _NoScope:
    def __enter__(self):
        return self

    def __exit__(self, *a):
        return False


def _scope(name):
    return jax.named_scope(name) if _SCOPES else _NoScope()


def _bf16_round(v):
    return v.astype(bf16).astype(f32)


def _phi(t):
    return jnp.where(t > 0, t + 1.0, jnp.exp(t)) + _EPS


def _tie(val, dep, never, last=False):
    if dep is None:
        return val
    r = 8 * (4 // val.dtype.itemsize)
    if r > 8:
        dep = jnp.concatenate([dep] * (r // 8), axis=0)
    if last:
        tail = jnp.where(never, dep.astype(val.dtype), val[-r:, -128:])
        bottom = jnp.concatenate([val[-r:, :-128], tail], axis=1)
        return jnp.concatenate([val[:-r, :], bottom], axis=0)
    head = jnp.where(never, dep.astype(val.dtype), val[:r, :128])
    top = jnp.concatenate([head, val[:r, 128:]], axis=1)
    return jnp.concatenate([top, val[r:, :]], axis=0)


def _split(items, n):
    k = len(items)
    return [items[(i * k) // n:((i + 1) * k) // n] for i in range(n)]


_TN = (((0,), (0,)), ((), ()))
_NT = (((1,), (1,)), ((), ()))


def _kernel(x_hbm, wqkv_hbm, wo_hbm, wr_hbm, wg_hbm, wu_hbm, wd_hbm, out_hbm,
            x_buf, xn_buf, wq_buf, wk_buf, wv_buf, wqt_buf, wo_buf, m_buf, wr_buf,
            g_acc, z_acc, zb_buf,
            wg_buf, wu_buf, wd_buf, xb_buf, hb_buf, y_acc, out_buf,
            sem, o_sem):

    def x_copy(i):
        if isinstance(i, int):
            rows = pl.ds(*_X_ROWS[i])
        else:
            rows = pl.ds(pl.multiple_of((i - 1) * TS, TS), TS)
        return pltpu.make_async_copy(x_hbm.at[rows, :], x_buf.at[rows, :], sem.at[_SEM_X + i])

    def wk_copy(s):
        c0, c1 = _WK_SPLIT[s]
        return pltpu.make_async_copy(
            wqkv_hbm.at[:, pl.ds(D + c0 * CW, (c1 - c0) * CW)],
            wk_buf.at[:, pl.ds(c0 * CW, (c1 - c0) * CW)], sem.at[_SEM_WK + s])

    wq_copy = pltpu.make_async_copy(wqkv_hbm.at[:, pl.ds(0, D)], wq_buf, sem.at[_SEM_WQ])
    wv_copy = pltpu.make_async_copy(wqkv_hbm.at[:, pl.ds(2 * D, D)], wv_buf, sem.at[_SEM_WV])
    wo_copy = pltpu.make_async_copy(wo_hbm, wo_buf, sem.at[_SEM_WO])
    wr_copy = pltpu.make_async_copy(wr_hbm, wr_buf, sem.at[_SEM_WR])

    def ffn_copies(j):
        s = _SEM_F + 3 * j
        f0 = j * FPC * FW
        fs = pl.ds(f0, min(FPC * FW, F - f0))
        return (pltpu.make_async_copy(wg_hbm.at[:, fs], wg_buf.at[:, fs], sem.at[s]),
                pltpu.make_async_copy(wu_hbm.at[:, fs], wu_buf.at[:, fs], sem.at[s + 1]),
                pltpu.make_async_copy(wd_hbm.at[fs, :], wd_buf.at[fs, :], sem.at[s + 2]))

    def out_copy(t, c):
        rows = pl.ds(t * TS if isinstance(t, int) else pl.multiple_of(t * TS, TS), TS)
        cols = pl.ds(c * CW, CW)
        return pltpu.make_async_copy(out_buf.at[rows, cols], out_hbm.at[rows, cols],
                                     o_sem.at[t * NC + c])

    wr_copy.start()
    x_copy(0).start()
    wk_copy(0).start()
    wk_copy(1).start()
    x_copy(1).start()
    wk_copy(2).start()
    for i in range(2, len(_X_ROWS)):
        x_copy(i).start()
    wq_copy.start()
    wv_copy.start()
    wo_copy.start()
    for j in range(NT - 1):
        for c in ffn_copies(j):
            c.start(priority=1)

    y_acc[...] = jnp.zeros_like(y_acc)
    hb_buf[...] = jnp.zeros_like(hb_buf)

    sub_iota = lax.broadcasted_iota(jnp.int32, (8, 128), 0)

    def layernorm(src, dst, nr, best, after=None, never=None):
        x = x_buf[pl.ds(src, nr), :].astype(f32)
        x = _tie(x, after, never)
        mean = jnp.sum(x, axis=-1, keepdims=True) * (1.0 / D)
        c = x - mean
        var = jnp.sum(c * c, axis=-1, keepdims=True) * (1.0 / D)
        sd = _bf16_round(jnp.sqrt(_bf16_round(_bf16_round(var) + _LN_EPS)))
        d = _bf16_round(x - _bf16_round(mean))
        xf = d * (1.0 / sd)
        xn = xf.astype(bf16)
        xn_buf[pl.ds(dst, nr), :] = xn
        wr = wr_buf[...].reshape(1, D).astype(f32)
        r = _bf16_round(jnp.sum(xn.astype(f32) * wr, axis=-1, keepdims=True))
        r = jnp.broadcast_to(r, (nr, 128))
        dep = None
        for g in range(0, nr, 8):
            rg = r[g:g + 8, :]
            better = rg > best[0]
            best[0] = jnp.where(better, rg, best[0])
            best[1] = jnp.where(better, sub_iota + (src + g), best[1])
            dg = xf[g:g + 8, D - 128:] if DEPX else rg
            dep = dg if dep is None else dep + dg
        return dep

    def kg_steps(xn, chunks, init, side, never):
        nr = xn.shape[0]

        def k_part(c):
            cols = slice(c * CW, (c + 1) * CW)
            k = jnp.dot(xn, wk_buf[:, cols], preferred_element_type=f32)
            if c in side:
                k = _tie(k, side[c](), never, TLAST)
            pk = _phi(k)
            zc = jnp.sum(pk.reshape(nr // 8, 8, CW), axis=0)
            z_acc[:, cols] = zc if init else z_acc[:, cols] + zc
            return pk.astype(bf16)

        def g_part(c, pk):
            rows = slice(c * CW, (c + 1) * CW)
            g = lax.dot_general(pk, xn, _TN, preferred_element_type=f32)
            g_acc[rows, :] = g if init else g_acc[rows, :] + g

        prev = None
        for c in chunks:
            pk = k_part(c)
            if prev is not None:
                g_part(*prev)
            prev = (c, pk)
        g_part(*prev)

    def ln_side(src, dst, nr, sub, chunks, best, never):
        def chain(offs):
            dep = None
            for o in offs:
                dep = layernorm(src + o, dst + o, sub, best, dep, never)
            return dep
        groups = _split(list(range(0, nr, sub)), len(chunks))
        return {c: (lambda g=g: chain(g)) for c, g in zip(chunks, groups)}

    best = [jnp.full((8, 128), -jnp.inf, f32), jnp.zeros((8, 128), jnp.int32)]
    with _scope("wait_x0"):
        wr_copy.wait()
        x_copy(0).wait()
    with _scope("ln0"):
        layernorm(0, 0, T0, best)
    never = jnp.min(best[1]) < 0
    with _scope("wait_wk0"):
        wk_copy(0).wait()
    kg_steps(xn_buf[0:T0, :], (0,), True, {}, never)
    with _scope("wait_wk1"):
        wk_copy(1).wait()
        x_copy(1).wait()
    for r in range(T0, TS, LSUB0):
        layernorm(r, r, LSUB0, best)
    kg_steps(xn_buf[0:T0, :], (1,), True, {}, never)
    kg_steps(xn_buf[T0:TS, :], (0, 1), False, {}, never)
    with _scope("wait_wk2"):
        wk_copy(2).wait()
        x_copy(2).wait()
    kg_steps(xn_buf[0:TS, :], (2, 3), True, ln_side(TS, TS, TS, LSUB0, (2, 3), best, never), never)
    with _scope("wait_wq"):
        wq_copy.wait()

    def phase1(i, carry):
        with _scope("p1_wait"):
            @pl.when(i + 1 < NT)
            def _():
                x_copy(i + 2).wait()
        with _scope("p1_body"):
            best = list(carry)
            r0 = pl.multiple_of(i * TS, TS)
            src = pl.multiple_of(jnp.minimum(r0 + TS, S - TS), TS)
            dst = pl.multiple_of(r0 + TS, TS)
            qrows = pl.ds(pl.multiple_of((i - 1) * CW, CW), CW)
            wqt_buf[qrows, :] = wq_buf[:, qrows].T
            chunks = tuple(range(NC))
            kg_steps(xn_buf[pl.ds(r0, TS), :], chunks, False,
                     ln_side(src, dst, TS, LSUB, chunks, best, never), never)
        return tuple(best)

    best = lax.fori_loop(1, NT, phase1, tuple(best))

    wv_copy.wait()
    wo_copy.wait()
    rr = lax.broadcasted_iota(jnp.int32, (128, 128), 0) // DH
    cc = lax.broadcasted_iota(jnp.int32, (128, 128), 1) // DH
    same_head = rr == cc

    def kv_part(g):
        sl = slice(g * 128, (g + 1) * 128)
        kv = jnp.dot(g_acc[sl, :].astype(bf16), wv_buf[:, sl], preferred_element_type=f32)
        return jnp.where(same_head, kv, 0.0).astype(bf16)

    def m_part(g, kv):
        sl = slice(g * 128, (g + 1) * 128)
        m_buf[sl, :] = jnp.dot(kv, wo_buf[sl, :], preferred_element_type=f32).astype(bf16)

    rmax = jnp.max(best[0], axis=0, keepdims=True)
    idx = jnp.clip(jnp.min(jnp.where(best[0] == rmax, best[1], S)), 0, S - 1)
    t_sel = idx // TS
    gate = 1.0 / (1.0 + jnp.exp(-rmax[:, :1]))
    wqt_buf[D - CW:D, :] = wq_buf[:, D - CW:D].T
    z = jnp.sum(z_acc[...], axis=0, keepdims=True)
    zb_buf[...] = jnp.broadcast_to(z, (128, D)).T
    r16 = pl.multiple_of((idx // 16) * 16, 16)
    blk = xn_buf[pl.ds(r16, 16), :].astype(f32)
    sel = lax.broadcasted_iota(jnp.int32, (16, D), 0) == (idx - r16)
    x_sel = jnp.sum(jnp.where(sel, blk, 0.0), axis=0, keepdims=True)
    xb_buf[...] = jnp.broadcast_to(x_sel, (128, D)).T

    kv_prev = kv_part(0)
    for g in range(1, G128):
        kv = kv_part(g)
        m_part(g - 1, kv_prev)
        kv_prev = kv
    m_part(G128 - 1, kv_prev)

    def chunk_start(c):
        return pl.multiple_of(jnp.minimum(c * FPC, NFU - FPC) * FW, FW)

    def phase2(j, carry):
        with _scope("p2_wait"):
            for jj in range(NT - 1):
                @pl.when(j == jj)
                def _():
                    for c in ffn_copies(jj):
                        c.wait()
        with _scope("p2_body"):
            t = lax.rem(t_sel + 1 + j, NT)
            trows = pl.ds(pl.multiple_of(t * TS, TS), TS)
            xn = xn_buf[trows, :]
            f_up = chunk_start(jnp.minimum(j, NT - 2))
            f_dn = chunk_start(jnp.maximum(j - 1, 0))
            n_dup = FPC * (NT - 1) - NFU
            keep_dup = jnp.where(j >= NT - 2, 0.0, 1.0)

            def chain(w, col, prev):
                n = w.shape[1] // 128
                acc = None
                for r in range(0, w.shape[0], 8):
                    cr = col[r:r + 8, :]
                    lo = ((r // 8) % n) * 128
                    link = prev if acc is None else acc[:, lo:lo + 128]
                    if link is not None:
                        cr = jnp.where(never, link, cr)
                    p = w[r:r + 8, :] * jnp.concatenate([cr] * n, axis=1)
                    acc = p if acc is None else acc + p
                return acc

            def fold(a):
                return a[:, :128] + a[:, 128:]

            gs = {}

            def gate_unit(u, prev):
                fs = pl.ds(f_up + u * FW, FW)
                gs[u] = chain(wg_buf[:, fs].astype(f32), xb_buf[...], prev)
                return fold(gs[u])

            def up_unit(u, prev):
                fs = pl.ds(f_up + u * FW, FW)
                a = chain(wu_buf[:, fs].astype(f32), xb_buf[...], prev)
                g = jnp.sum(gs[u], axis=0, keepdims=True)
                h = g * (1.0 / (1.0 + jnp.exp(-g))) * jnp.sum(a, axis=0, keepdims=True)
                if u < n_dup:
                    h = h * keep_dup
                hb_buf[u * FW:(u + 1) * FW, :] = jnp.broadcast_to(h, (128, FW)).T
                return fold(a)

            def down_unit(e, prev):
                ec = slice(e * FW, (e + 1) * FW)
                w = wd_buf[pl.ds(f_dn, FPC * FW), ec].astype(f32)
                ye = y_acc[:, ec] + chain(w, hb_buf[...], prev)
                y_acc[:, ec] = ye
                return fold(ye)

            units = [(down_unit, e) for e in range(D // FW)]
            for u in range(FPC):
                units += [(gate_unit, u), (up_unit, u)]
            groups = _split(units, 2 * NC - 1) + [[]]

            def side(slot):
                dep = None
                for fn, a in groups[slot]:
                    dep = fn(a, dep)
                return dep

            ps = []
            for c in range(NC):
                rows = slice(c * CW, (c + 1) * CW)
                qt = lax.dot_general(wqt_buf[rows, :], xn, _NT, preferred_element_type=f32)
                qt = _tie(qt, side(c), never, TLAST)
                pqt = _phi(qt)
                zb = zb_buf[rows, :]
                zfull = jnp.concatenate([zb] * (TS // 128), axis=1)
                hc = CW // DH
                den = jnp.sum((pqt * zfull).reshape(hc, DH, TS), axis=1, keepdims=True) + _EPS
                pt = pqt.reshape(hc, DH, TS) * pl.reciprocal(den, approx=True)
                ps.append(pt.reshape(CW, TS).astype(bf16).T)
            p = jnp.concatenate(ps, axis=1)
            y = jnp.sum(y_acc[...], axis=0, keepdims=True) * gate
            hit = lax.broadcasted_iota(jnp.int32, (TS, CW), 0) == idx - t * TS
            dep = None
            for c in range(NC):
                cols = slice(c * CW, (c + 1) * CW)
                m = _tie(m_buf[:, cols], dep, never)
                o = jnp.dot(p, m, preferred_element_type=f32)
                dep = side(NC + c)
                o = o + x_buf[trows, cols].astype(f32) + xn_buf[trows, cols].astype(f32)
                out_buf[trows, cols] = (o + jnp.where(hit, y[:, cols], 0.0)).astype(bf16)
                out_copy(t, c).start()
        return carry

    lax.fori_loop(0, NT, phase2, 0)
    with _scope("final_wait"):
        for t in range(NT):
            for c in range(NC):
                out_copy(t, c).wait()


@jax.jit
def pallas_parallel_sum__linear_attn_block__moe_arch_mod__prompt_kernel(
    A_x: jax.Array,
    A_wqkv: jax.Array,
    A_wo: jax.Array,
    B_x: jax.Array,
    B_w_r: jax.Array,
    B_w_gate: jax.Array,
    B_w_up: jax.Array,
    B_w_down: jax.Array,
):
    any_spec = pl.BlockSpec(memory_space=pl.ANY)
    out = pl.pallas_call(
        _kernel,
        out_shape=jax.ShapeDtypeStruct((S, D), bf16),
        in_specs=[any_spec] * 7,
        out_specs=any_spec,
        scratch_shapes=[
            pltpu.VMEM((S, D), bf16),
            pltpu.VMEM((S + TS, D), bf16),
            pltpu.VMEM((D, D), bf16),
            pltpu.VMEM((D, D), bf16),
            pltpu.VMEM((D, D), bf16),
            pltpu.VMEM((D, D), bf16),
            pltpu.VMEM((D, D), bf16),
            pltpu.VMEM((D, D), bf16),
            pltpu.VMEM((D,), bf16),
            pltpu.VMEM((D, D), f32),
            pltpu.VMEM((8, D), f32),
            pltpu.VMEM((D, 128), f32),
            pltpu.VMEM((D, F), bf16),
            pltpu.VMEM((D, F), bf16),
            pltpu.VMEM((F, D), bf16),
            pltpu.VMEM((D, 128), f32),
            pltpu.VMEM((FPC * FW, 128), f32),
            pltpu.VMEM((8, D), f32),
            pltpu.VMEM((S, D), bf16),
            pltpu.SemaphoreType.DMA((_N_SEM,)),
            pltpu.SemaphoreType.DMA((NT * NC,)),
        ],
        compiler_params=pltpu.CompilerParams(vmem_limit_bytes=100 * 1024 * 1024,
                                             disable_semaphore_checks=True),
        name="linattn_mod",
    )(A_x.reshape(S, D), A_wqkv, A_wo, B_w_r, B_w_gate, B_w_up, B_w_down)
    return out.reshape(1, S, D)
```

```python
import os
import jax
import jax.numpy as jnp
from jax import lax
import jax.experimental.pallas as pl
import jax.experimental.pallas.tpu as pltpu

S = 2048
D = 1024
F = 3584
H = 32
DH = D // H
G128 = D // 128
CW = 256
NC = D // CW
T0 = 256
TS = 512
NT = S // TS
FW = 256
NFU = F // FW
FPC = -(-NFU // (NT - 1))
TLAST = bool(int(os.environ.get("TLAST", 1)))
DEPX = bool(int(os.environ.get("DEPX", 1)))
STEP = int(os.environ.get("STEP", 64))
RB = int(os.environ.get("RB", 32))
LSUB = int(os.environ.get("LSUB", 16))
LSUB0 = int(os.environ.get("LSUB0", 32))

_LN_EPS = 1.0013580322265625e-05
_EPS = 1e-6
_SCOPES = False

f32 = jnp.float32
bf16 = jnp.bfloat16

_X_ROWS = [(0, T0), (T0, T0)] + [(i * TS, TS) for i in range(1, NT)]
_WK_SPLIT = ((0, 1), (1, 2), (2, 4))
_SEM_X = 0
_SEM_WK = _SEM_X + len(_X_ROWS)
_SEM_WQ = _SEM_WK + len(_WK_SPLIT)
_SEM_WV = _SEM_WQ + 1
_SEM_WO = _SEM_WV + 1
_SEM_WR = _SEM_WO + 1
_SEM_F = _SEM_WR + 1
_N_SEM = _SEM_F + 3 * (NT - 1)


class _NoScope:
    def __enter__(self):
        return self

    def __exit__(self, *a):
        return False


def _scope(name):
    return jax.named_scope(name) if _SCOPES else _NoScope()


def _bf16_round(v):
    return v.astype(bf16).astype(f32)


def _phi(t):
    return jnp.where(t > 0, t + 1.0, jnp.exp(t)) + _EPS


def _tie(val, dep, never, last=False):
    if dep is None:
        return val
    r = 8 * (4 // val.dtype.itemsize)
    if r > 8:
        dep = jnp.concatenate([dep] * (r // 8), axis=0)
    if last:
        tail = jnp.where(never, dep.astype(val.dtype), val[-r:, -128:])
        bottom = jnp.concatenate([val[-r:, :-128], tail], axis=1)
        return jnp.concatenate([val[:-r, :], bottom], axis=0)
    head = jnp.where(never, dep.astype(val.dtype), val[:r, :128])
    top = jnp.concatenate([head, val[:r, 128:]], axis=1)
    return jnp.concatenate([top, val[r:, :]], axis=0)


def _tie_tiles(val, deps, never, rb):
    cols = []
    for n in range(val.shape[1] // 128):
        parts = []
        for r in range(0, val.shape[0], rb):
            blk = val[r:r + rb, n * 128:(n + 1) * 128]
            dep = next(deps, None)
            if dep is not None:
                tail = jnp.where(never, dep, blk[rb - 8:, :])
                blk = jnp.concatenate([blk[:rb - 8, :], tail], axis=0) if rb > 8 else tail
            parts.append(blk)
        cols.append(jnp.concatenate(parts, axis=0))
    return jnp.concatenate(cols, axis=1)


def _split(items, n):
    k = len(items)
    return [items[(i * k) // n:((i + 1) * k) // n] for i in range(n)]


_TN = (((0,), (0,)), ((), ()))
_NT = (((1,), (1,)), ((), ()))


def _kernel(x_hbm, wqkv_hbm, wo_hbm, wr_hbm, wg_hbm, wu_hbm, wd_hbm, out_hbm,
            x_buf, xn_buf, wq_buf, wk_buf, wv_buf, wqt_buf, wo_buf, m_buf, wr_buf,
            g_acc, z_acc, zb_buf,
            wg_buf, wu_buf, wd_buf, xb_buf, hb_buf, y_acc, out_buf,
            sem, o_sem):

    def x_copy(i):
        if isinstance(i, int):
            rows = pl.ds(*_X_ROWS[i])
        else:
            rows = pl.ds(pl.multiple_of((i - 1) * TS, TS), TS)
        return pltpu.make_async_copy(x_hbm.at[rows, :], x_buf.at[rows, :], sem.at[_SEM_X + i])

    def wk_copy(s):
        c0, c1 = _WK_SPLIT[s]
        return pltpu.make_async_copy(
            wqkv_hbm.at[:, pl.ds(D + c0 * CW, (c1 - c0) * CW)],
            wk_buf.at[:, pl.ds(c0 * CW, (c1 - c0) * CW)], sem.at[_SEM_WK + s])

    wq_copy = pltpu.make_async_copy(wqkv_hbm.at[:, pl.ds(0, D)], wq_buf, sem.at[_SEM_WQ])
    wv_copy = pltpu.make_async_copy(wqkv_hbm.at[:, pl.ds(2 * D, D)], wv_buf, sem.at[_SEM_WV])
    wo_copy = pltpu.make_async_copy(wo_hbm, wo_buf, sem.at[_SEM_WO])
    wr_copy = pltpu.make_async_copy(wr_hbm, wr_buf, sem.at[_SEM_WR])

    def ffn_copies(j):
        s = _SEM_F + 3 * j
        fs = pl.ds(min(j * FPC, NFU - FPC) * FW, FPC * FW)
        return (pltpu.make_async_copy(wg_hbm.at[:, fs], wg_buf.at[j], sem.at[s]),
                pltpu.make_async_copy(wu_hbm.at[:, fs], wu_buf.at[j], sem.at[s + 1]),
                pltpu.make_async_copy(wd_hbm.at[fs, :], wd_buf.at[j], sem.at[s + 2]))

    def out_copy(t, c):
        rows = pl.ds(t * TS if isinstance(t, int) else pl.multiple_of(t * TS, TS), TS)
        cols = pl.ds(c * CW, CW)
        return pltpu.make_async_copy(out_buf.at[rows, cols], out_hbm.at[rows, cols],
                                     o_sem.at[t * NC + c])

    wr_copy.start()
    x_copy(0).start()
    wk_copy(0).start()
    wk_copy(1).start()
    x_copy(1).start()
    wk_copy(2).start()
    for i in range(2, len(_X_ROWS)):
        x_copy(i).start()
    wq_copy.start()
    wv_copy.start()
    wo_copy.start()
    for j in range(NT - 1):
        for c in ffn_copies(j):
            c.start(priority=1)

    y_acc[...] = jnp.zeros_like(y_acc)
    hb_buf[...] = jnp.zeros_like(hb_buf)

    sub_iota = lax.broadcasted_iota(jnp.int32, (8, 128), 0)

    def layernorm(src, dst, nr, best, after=None, never=None):
        x = x_buf[pl.ds(src, nr), :].astype(f32)
        x = _tie(x, after, never)
        mean = jnp.sum(x, axis=-1, keepdims=True) * (1.0 / D)
        c = x - mean
        var = jnp.sum(c * c, axis=-1, keepdims=True) * (1.0 / D)
        sd = _bf16_round(jnp.sqrt(_bf16_round(_bf16_round(var) + _LN_EPS)))
        d = _bf16_round(x - _bf16_round(mean))
        xf = d * (1.0 / sd)
        xn = xf.astype(bf16)
        xn_buf[pl.ds(dst, nr), :] = xn
        wr = wr_buf[...].reshape(1, D).astype(f32)
        r = _bf16_round(jnp.sum(xn.astype(f32) * wr, axis=-1, keepdims=True))
        r = jnp.broadcast_to(r, (nr, 128))
        dep = None
        for g in range(0, nr, 8):
            rg = r[g:g + 8, :]
            better = rg > best[0]
            best[0] = jnp.where(better, rg, best[0])
            best[1] = jnp.where(better, sub_iota + (src + g), best[1])
            dg = xf[g:g + 8, D - 128:] if DEPX else rg
            dep = dg if dep is None else dep + dg
        return dep

    def kg_steps(xn, chunks, init, side, never):
        nr = xn.shape[0]

        def k_part(c):
            cols = slice(c * CW, (c + 1) * CW)
            k = jnp.dot(xn, wk_buf[:, cols], preferred_element_type=f32)
            if c in side:
                k = _tie(k, side[c](), never, TLAST)
            pk = _phi(k)
            zc = jnp.sum(pk.reshape(nr // 8, 8, CW), axis=0)
            z_acc[:, cols] = zc if init else z_acc[:, cols] + zc
            return pk.astype(bf16)

        def g_part(c, pk):
            rows = slice(c * CW, (c + 1) * CW)
            g = lax.dot_general(pk, xn, _TN, preferred_element_type=f32)
            g_acc[rows, :] = g if init else g_acc[rows, :] + g

        prev = None
        for c in chunks:
            pk = k_part(c)
            if prev is not None:
                g_part(*prev)
            prev = (c, pk)
        g_part(*prev)

    def ln_side(src, dst, nr, sub, chunks, best, never):
        def chain(offs):
            dep = None
            for o in offs:
                dep = layernorm(src + o, dst + o, sub, best, dep, never)
            return dep
        groups = _split(list(range(0, nr, sub)), len(chunks))
        return {c: (lambda g=g: chain(g)) for c, g in zip(chunks, groups)}

    best = [jnp.full((8, 128), -jnp.inf, f32), jnp.zeros((8, 128), jnp.int32)]
    with _scope("wait_x0"):
        wr_copy.wait()
        x_copy(0).wait()
    with _scope("ln0"):
        layernorm(0, 0, T0, best)
    never = jnp.min(best[1]) < 0
    with _scope("wait_wk0"):
        wk_copy(0).wait()
    kg_steps(xn_buf[0:T0, :], (0,), True, {}, never)
    with _scope("wait_wk1"):
        wk_copy(1).wait()
        x_copy(1).wait()
    for r in range(T0, TS, LSUB0):
        layernorm(r, r, LSUB0, best)
    kg_steps(xn_buf[0:T0, :], (1,), True, {}, never)
    kg_steps(xn_buf[T0:TS, :], (0, 1), False, {}, never)
    with _scope("wait_wk2"):
        wk_copy(2).wait()
        x_copy(2).wait()
    kg_steps(xn_buf[0:TS, :], (2, 3), True, ln_side(TS, TS, TS, LSUB0, (2, 3), best, never), never)
    with _scope("wait_wq"):
        wq_copy.wait()

    def phase1(i, carry):
        with _scope("p1_wait"):
            @pl.when(i + 1 < NT)
            def _():
                x_copy(i + 2).wait()
        with _scope("p1_body"):
            best = list(carry)
            r0 = pl.multiple_of(i * TS, TS)
            src = pl.multiple_of(jnp.minimum(r0 + TS, S - TS), TS)
            dst = pl.multiple_of(r0 + TS, TS)
            qrows = pl.ds(pl.multiple_of((i - 1) * CW, CW), CW)
            wqt_buf[qrows, :] = wq_buf[:, qrows].T
            chunks = tuple(range(NC))
            kg_steps(xn_buf[pl.ds(r0, TS), :], chunks, False,
                     ln_side(src, dst, TS, LSUB, chunks, best, never), never)
        return tuple(best)

    best = lax.fori_loop(1, NT, phase1, tuple(best))

    wv_copy.wait()
    wo_copy.wait()
    rr = lax.broadcasted_iota(jnp.int32, (128, 128), 0) // DH
    cc = lax.broadcasted_iota(jnp.int32, (128, 128), 1) // DH
    same_head = rr == cc

    def kv_part(g):
        sl = slice(g * 128, (g + 1) * 128)
        kv = jnp.dot(g_acc[sl, :].astype(bf16), wv_buf[:, sl], preferred_element_type=f32)
        return jnp.where(same_head, kv, 0.0).astype(bf16)

    def m_part(g, kv):
        sl = slice(g * 128, (g + 1) * 128)
        m_buf[sl, :] = jnp.dot(kv, wo_buf[sl, :], preferred_element_type=f32).astype(bf16)

    rmax = jnp.max(best[0], axis=0, keepdims=True)
    idx = jnp.clip(jnp.min(jnp.where(best[0] == rmax, best[1], S)), 0, S - 1)
    t_sel = idx // TS
    gate = 1.0 / (1.0 + jnp.exp(-rmax[:, :1]))
    wqt_buf[D - CW:D, :] = wq_buf[:, D - CW:D].T
    z = jnp.sum(z_acc[...], axis=0, keepdims=True)
    zb_buf[...] = jnp.broadcast_to(z, (128, D)).T
    r16 = pl.multiple_of((idx // 16) * 16, 16)
    blk = xn_buf[pl.ds(r16, 16), :].astype(f32)
    sel = lax.broadcasted_iota(jnp.int32, (16, D), 0) == (idx - r16)
    x_sel = jnp.sum(jnp.where(sel, blk, 0.0), axis=0, keepdims=True)
    xb_buf[...] = jnp.broadcast_to(x_sel, (128, D)).T

    kv_prev = kv_part(0)
    for g in range(1, G128):
        kv = kv_part(g)
        m_part(g - 1, kv_prev)
        kv_prev = kv
    m_part(G128 - 1, kv_prev)

    def phase2(j, carry):
        with _scope("p2_wait"):
            for jj in range(NT - 1):
                @pl.when(j == jj)
                def _():
                    for c in ffn_copies(jj):
                        c.wait()
        with _scope("p2_body"):
            t = lax.rem(t_sel + 1 + j, NT)
            trows = pl.ds(pl.multiple_of(t * TS, TS), TS)
            xn = xn_buf[trows, :]
            j_up = jnp.minimum(j, NT - 2)
            j_dn = jnp.maximum(j - 1, 0)
            n_dup = FPC * (NT - 1) - NFU
            keep_dup = jnp.where(j >= NT - 2, 0.0, 1.0)

            def fold(a):
                return a[:, :128] + a[:, 128:]

            def matvec(w_ref, slot, nrows, cols, col_ref):
                acc = None
                for r in range(0, nrows, STEP):
                    w = w_ref[slot, r:r + STEP, cols].astype(f32)
                    cr = col_ref[r:r + STEP, :]
                    p = w * jnp.concatenate([cr] * (FW // 128), axis=1)
                    for g in range(0, STEP, 8):
                        acc = p[g:g + 8, :] if acc is None else acc + p[g:g + 8, :]
                    yield fold(acc)
                return acc

            def ffn_work():
                for e in range(D // FW):
                    ec = slice(e * FW, (e + 1) * FW)
                    acc = yield from matvec(wd_buf, j_dn, FPC * FW, ec, hb_buf)
                    y_acc[:, ec] += acc
                for u in range(FPC):
                    fs = slice(u * FW, (u + 1) * FW)
                    g = yield from matvec(wg_buf, j_up, D, fs, xb_buf)
                    a = yield from matvec(wu_buf, j_up, D, fs, xb_buf)
                    g = jnp.sum(g, axis=0, keepdims=True)
                    h = g * (1.0 / (1.0 + jnp.exp(-g))) * jnp.sum(a, axis=0, keepdims=True)
                    if u < n_dup:
                        h = h * keep_dup
                    hb_buf[u * FW:(u + 1) * FW, :] = jnp.broadcast_to(h, (128, FW)).T

            work = ffn_work()

            ps = []
            for c in range(NC):
                rows = slice(c * CW, (c + 1) * CW)
                qt = lax.dot_general(wqt_buf[rows, :], xn, _NT, preferred_element_type=f32)
                qt = _tie_tiles(qt, work, never, RB)
                pqt = _phi(qt)
                zb = zb_buf[rows, :]
                zfull = jnp.concatenate([zb] * (TS // 128), axis=1)
                hc = CW // DH
                den = jnp.sum((pqt * zfull).reshape(hc, DH, TS), axis=1, keepdims=True) + _EPS
                pt = pqt.reshape(hc, DH, TS) * pl.reciprocal(den, approx=True)
                ps.append(pt.reshape(CW, TS).astype(bf16).T)
            p = jnp.concatenate(ps, axis=1)
            y = jnp.sum(y_acc[...], axis=0, keepdims=True) * gate
            hit = lax.broadcasted_iota(jnp.int32, (TS, CW), 0) == idx - t * TS
            for c in range(NC):
                cols = slice(c * CW, (c + 1) * CW)
                o = jnp.dot(p, m_buf[:, cols], preferred_element_type=f32)
                o = _tie_tiles(o, work, never, RB)
                o = o + x_buf[trows, cols].astype(f32) + xn_buf[trows, cols].astype(f32)
                out_buf[trows, cols] = (o + jnp.where(hit, y[:, cols], 0.0)).astype(bf16)
                out_copy(t, c).start()
            assert next(work, None) is None
        return carry

    lax.fori_loop(0, NT, phase2, 0)
    with _scope("final_wait"):
        for t in range(NT):
            for c in range(NC):
                out_copy(t, c).wait()


@jax.jit
def pallas_parallel_sum__linear_attn_block__moe_arch_mod__prompt_kernel(
    A_x: jax.Array,
    A_wqkv: jax.Array,
    A_wo: jax.Array,
    B_x: jax.Array,
    B_w_r: jax.Array,
    B_w_gate: jax.Array,
    B_w_up: jax.Array,
    B_w_down: jax.Array,
):
    any_spec = pl.BlockSpec(memory_space=pl.ANY)
    out = pl.pallas_call(
        _kernel,
        out_shape=jax.ShapeDtypeStruct((S, D), bf16),
        in_specs=[any_spec] * 7,
        out_specs=any_spec,
        scratch_shapes=[
            pltpu.VMEM((S, D), bf16),
            pltpu.VMEM((S + TS, D), bf16),
            pltpu.VMEM((D, D), bf16),
            pltpu.VMEM((D, D), bf16),
            pltpu.VMEM((D, D), bf16),
            pltpu.VMEM((D, D), bf16),
            pltpu.VMEM((D, D), bf16),
            pltpu.VMEM((D, D), bf16),
            pltpu.VMEM((D,), bf16),
            pltpu.VMEM((D, D), f32),
            pltpu.VMEM((8, D), f32),
            pltpu.VMEM((D, 128), f32),
            pltpu.VMEM((NT - 1, D, FPC * FW), bf16),
            pltpu.VMEM((NT - 1, D, FPC * FW), bf16),
            pltpu.VMEM((NT - 1, FPC * FW, D), bf16),
            pltpu.VMEM((D, 128), f32),
            pltpu.VMEM((FPC * FW, 128), f32),
            pltpu.VMEM((8, D), f32),
            pltpu.VMEM((S, D), bf16),
            pltpu.SemaphoreType.DMA((_N_SEM,)),
            pltpu.SemaphoreType.DMA((NT * NC,)),
        ],
        compiler_params=pltpu.CompilerParams(vmem_limit_bytes=100 * 1024 * 1024,
                                             disable_semaphore_checks=True),
        name="linattn_mod",
    )(A_x.reshape(S, D), A_wqkv, A_wo, B_w_r, B_w_gate, B_w_up, B_w_down)
    return out.reshape(1, S, D)
```

```python
import os
import jax
import jax.numpy as jnp
from jax import lax
import jax.experimental.pallas as pl
import jax.experimental.pallas.tpu as pltpu

S = 2048
D = 1024
F = 3584
H = 32
DH = D // H
G128 = D // 128
CW = 256
NC = D // CW
T0 = 256
TS = 512
NT = S // TS
FW = 256
NFU = F // FW
FPC = -(-NFU // (NT - 1))
TLAST = bool(int(os.environ.get("TLAST", 1)))
DEPX = bool(int(os.environ.get("DEPX", 1)))
STEP = int(os.environ.get("STEP", 64))
RB = int(os.environ.get("RB", 32))
LSUB = int(os.environ.get("LSUB", 16))
LSUB0 = int(os.environ.get("LSUB0", 64))
LSUBC = int(os.environ.get("LSUBC", 16))
CWC = int(os.environ.get("CWC", 128))
TIE_B = [int(v) for v in os.environ.get("TIE_B", "0,2,0,2").split(",")]
TIE_C = [int(v) for v in os.environ.get("TIE_C", "4,5,5,5,5,4,4").split(",")]
TIE_L = [int(v) for v in os.environ.get("TIE_L", "8,8,0,8,0,8").split(",")]

_LN_EPS = 1.0013580322265625e-05
_EPS = 1e-6
_SCOPES = False

f32 = jnp.float32
bf16 = jnp.bfloat16

_TAIL = [int(v) for v in os.environ.get("TAIL", "256,128,128").split(",")]
_OUT_PIECES = [(0, TS, c * CW, CW) for c in range(NC - 1)] + [
    (sum(_TAIL[:i]), _TAIL[i], D - CW, CW) for i in range(len(_TAIL))]

_X_ROWS = [(0, T0 // 2), (T0 // 2, T0 // 2), (T0, T0)] + [(i * TS, TS) for i in range(1, NT)]
_WK_SPLIT = ((0, 1), (1, 2), (2, 4))
_SEM_X = 0
_SEM_WK = _SEM_X + len(_X_ROWS)
_SEM_WQ = _SEM_WK + len(_WK_SPLIT)
_SEM_WV = _SEM_WQ + 1
_SEM_WO = _SEM_WV + 1
_SEM_WR = _SEM_WO + 1
_SEM_F = _SEM_WR + 1
_N_SEM = _SEM_F + 3 * (NT - 1)


class _NoScope:
    def __enter__(self):
        return self

    def __exit__(self, *a):
        return False


def _scope(name):
    return jax.named_scope(name) if _SCOPES else _NoScope()


def _bf16_round(v):
    return v.astype(bf16).astype(f32)


def _phi(t):
    return jnp.where(t > 0, t + 1.0, jnp.exp(t)) + _EPS


def _tie(val, dep, never, last=False):
    if dep is None:
        return val
    r = 8 * (4 // val.dtype.itemsize)
    if r > 8:
        dep = jnp.concatenate([dep] * (r // 8), axis=0)
    if last:
        tail = jnp.where(never, dep.astype(val.dtype), val[-r:, -128:])
        bottom = jnp.concatenate([val[-r:, :-128], tail], axis=1) if val.shape[1] > 128 else tail
        return jnp.concatenate([val[:-r, :], bottom], axis=0)
    head = jnp.where(never, dep.astype(val.dtype), val[:r, :128])
    top = jnp.concatenate([head, val[:r, 128:]], axis=1)
    return jnp.concatenate([top, val[r:, :]], axis=0)


def _tie_tiles(val, deps, never, rb):
    cols = []
    for n in range(val.shape[1] // 128):
        parts = []
        for r in range(0, val.shape[0], rb):
            blk = val[r:r + rb, n * 128:(n + 1) * 128]
            dep = next(deps, None)
            if dep is not None:
                tail = jnp.where(never, dep, blk[rb - 8:, :])
                blk = jnp.concatenate([blk[:rb - 8, :], tail], axis=0) if rb > 8 else tail
            parts.append(blk)
        cols.append(jnp.concatenate(parts, axis=0))
    return jnp.concatenate(cols, axis=1)


def _split(items, n):
    k = len(items)
    return [items[(i * k) // n:((i + 1) * k) // n] for i in range(n)]


_TN = (((0,), (0,)), ((), ()))
_NT = (((1,), (1,)), ((), ()))


def _kernel(x_hbm, wqkv_hbm, wo_hbm, wr_hbm, wg_hbm, wu_hbm, wd_hbm, out_hbm,
            x_buf, xn_buf, wq_buf, wk_buf, wv_buf, wqt_buf, wo_buf, m_buf, wr_buf,
            g_acc, z_acc, zb_buf,
            wg_buf, wu_buf, wd_buf, xb_buf, hb_buf, y_acc, out_buf,
            sem, o_sem):

    def x_copy(i):
        if isinstance(i, int):
            rows = pl.ds(*_X_ROWS[i])
        else:
            rows = pl.ds(pl.multiple_of((i - 2) * TS, TS), TS)
        return pltpu.make_async_copy(x_hbm.at[rows, :], x_buf.at[rows, :], sem.at[_SEM_X + i])

    def wk_copy(s):
        c0, c1 = _WK_SPLIT[s]
        return pltpu.make_async_copy(
            wqkv_hbm.at[:, pl.ds(D + c0 * CW, (c1 - c0) * CW)],
            wk_buf.at[:, pl.ds(c0 * CW, (c1 - c0) * CW)], sem.at[_SEM_WK + s])

    wq_copy = pltpu.make_async_copy(wqkv_hbm.at[:, pl.ds(0, D)], wq_buf, sem.at[_SEM_WQ])
    wv_copy = pltpu.make_async_copy(wqkv_hbm.at[:, pl.ds(2 * D, D)], wv_buf, sem.at[_SEM_WV])
    wo_copy = pltpu.make_async_copy(wo_hbm, wo_buf, sem.at[_SEM_WO])
    wr_copy = pltpu.make_async_copy(wr_hbm, wr_buf, sem.at[_SEM_WR])

    def ffn_copies(j):
        s = _SEM_F + 3 * j
        fs = pl.ds(min(j * FPC, NFU - FPC) * FW, FPC * FW)
        return (pltpu.make_async_copy(wg_hbm.at[:, fs], wg_buf.at[j], sem.at[s]),
                pltpu.make_async_copy(wu_hbm.at[:, fs], wu_buf.at[j], sem.at[s + 1]),
                pltpu.make_async_copy(wd_hbm.at[fs, :], wd_buf.at[j], sem.at[s + 2]))

    def out_copy(t, p):
        r0, nr, c0, nc = _OUT_PIECES[p]
        row = t * TS + r0
        rows = pl.ds(row if isinstance(t, int) else pl.multiple_of(row, 64), nr)
        cols = pl.ds(c0, nc)
        return pltpu.make_async_copy(out_buf.at[rows, cols], out_hbm.at[rows, cols],
                                     o_sem.at[t * len(_OUT_PIECES) + p])

    x_copy(0).start()
    wr_copy.start()
    x_copy(1).start()
    wk_copy(0).start()
    wk_copy(1).start()
    x_copy(2).start()
    wk_copy(2).start()
    for i in range(3, len(_X_ROWS)):
        x_copy(i).start()
    wq_copy.start()
    wv_copy.start()
    wo_copy.start()
    for j in range(NT - 1):
        for c in ffn_copies(j):
            c.start(priority=1)

    y_acc[...] = jnp.zeros_like(y_acc)
    hb_buf[...] = jnp.zeros_like(hb_buf)

    sub_iota = lax.broadcasted_iota(jnp.int32, (8, 128), 0)

    def layernorm(src, dst, nr, best, after=None, never=None):
        x = x_buf[pl.ds(src, nr), :].astype(f32)
        x = _tie(x, after, never)
        mean = jnp.sum(x, axis=-1, keepdims=True) * (1.0 / D)
        c = x - mean
        var = jnp.sum(c * c, axis=-1, keepdims=True) * (1.0 / D)
        sd = _bf16_round(jnp.sqrt(_bf16_round(_bf16_round(var) + _LN_EPS)))
        d = _bf16_round(x - _bf16_round(mean))
        xf = d * (1.0 / sd)
        xn = xf.astype(bf16)
        xn_buf[pl.ds(dst, nr), :] = xn
        wr = wr_buf[...].reshape(1, D).astype(f32)
        r = _bf16_round(jnp.sum(xn.astype(f32) * wr, axis=-1, keepdims=True))
        r = jnp.broadcast_to(r, (nr, 128))
        dep = None
        for g in range(0, nr, 8):
            rg = r[g:g + 8, :]
            better = rg > best[0]
            best[0] = jnp.where(better, rg, best[0])
            best[1] = jnp.where(better, sub_iota + (src + g), best[1])
            dg = xf[g:g + 8, D - 128:]
            dep = dg if dep is None else dep + dg
        return dep

    def ln_work(src, dst, sub, counts, best, never):
        o = 0
        for n in counts:
            dep = None
            for _ in range(n):
                dep = layernorm(src + o, dst + o, sub, best, dep, never)
                o += sub
            yield dep

    def kg_steps(jobs, work, never):
        def tied(val):
            return _tie(val, next(work, None), never, True)

        def k_part(xn, c0, cw, init):
            cols = slice(c0, c0 + cw)
            xn = xn()
            k = tied(jnp.dot(xn, wk_buf[:, cols], preferred_element_type=f32))
            pk = _phi(k)
            zc = jnp.sum(pk.reshape(xn.shape[0] // 8, 8, cw), axis=0)
            z_acc[:, cols] = zc if init else z_acc[:, cols] + zc
            return pk.astype(bf16)

        def g_part(pk, xn, c0, cw, init):
            rows = slice(c0, c0 + cw)
            g = tied(lax.dot_general(pk, xn(), _TN, preferred_element_type=f32))
            g_acc[rows, :] = g if init else g_acc[rows, :] + g

        prev = None
        for job in jobs:
            if prev is not None and job[0] is not prev[1][0]:
                g_part(prev[0], *prev[1])
                prev = None
            pk = k_part(*job)
            if prev is not None:
                g_part(prev[0], *prev[1])
            prev = (pk, job)
        g_part(prev[0], *prev[1])
        assert next(work, None) is None

    def rows_of(r0, nr):
        got = []

        def get():
            if not got:
                got.append(xn_buf[pl.ds(r0, nr), :])
            return got[0]
        return get

    best = [jnp.full((8, 128), -jnp.inf, f32), jnp.zeros((8, 128), jnp.int32)]
    with _scope("wait_x0"):
        x_copy(0).wait()
        wr_copy.wait()
    with _scope("ln0"):
        layernorm(0, 0, T0 // 2, best)
    never = jnp.min(best[1]) < 0
    with _scope("wait_x0"):
        x_copy(1).wait()
    with _scope("ln0"):
        layernorm(T0 // 2, T0 // 2, T0 // 2, best)
    with _scope("wait_wk0"):
        wk_copy(0).wait()
    xa = rows_of(0, T0)
    kg_steps([(xa, 0, 128, True), (xa, 128, 128, True)], iter(()), never)
    with _scope("wait_wk1"):
        wk_copy(1).wait()
        x_copy(2).wait()
    xa, xb = rows_of(0, T0), rows_of(T0, T0)
    assert sum(TIE_B) * LSUB0 == T0
    kg_steps([(xa, 256, 128, True), (xa, 384, 128, True), (xb, 0, CW, False), (xb, CW, CW, False)],
             ln_work(T0, T0, LSUB0, TIE_B, best, never), never)
    with _scope("wait_wk2"):
        wk_copy(2).wait()
        x_copy(3).wait()
    xa = rows_of(0, TS)
    assert sum(TIE_C) * LSUBC == TS
    kg_steps([(xa, c0, CWC, True) for c0 in range(2 * CW, D, CWC)],
             ln_work(TS, TS, LSUBC, TIE_C, best, never), never)
    with _scope("wait_wq"):
        wq_copy.wait()

    def phase1(i, carry):
        with _scope("p1_wait"):
            @pl.when(i + 1 < NT)
            def _():
                x_copy(i + 3).wait()
        with _scope("p1_body"):
            best = list(carry)
            r0 = pl.multiple_of(i * TS, TS)
            src = pl.multiple_of(jnp.minimum(r0 + TS, S - TS), TS)
            dst = pl.multiple_of(r0 + TS, TS)
            qrows = pl.ds(pl.multiple_of((i - 1) * CW, CW), CW)
            wqt_buf[qrows, :] = wq_buf[:, qrows].T
            xa = rows_of(r0, TS)
            assert sum(TIE_L) * LSUB == TS
            kg_steps([(xa, c * CW, CW, False) for c in range(NC)],
                     ln_work(src, dst, LSUB, TIE_L, best, never), never)
        return tuple(best)

    best = lax.fori_loop(1, NT, phase1, tuple(best))

    wv_copy.wait()
    wo_copy.wait()
    rr = lax.broadcasted_iota(jnp.int32, (128, 128), 0) // DH
    cc = lax.broadcasted_iota(jnp.int32, (128, 128), 1) // DH
    same_head = rr == cc

    def kv_part(g):
        sl = slice(g * 128, (g + 1) * 128)
        kv = jnp.dot(g_acc[sl, :].astype(bf16), wv_buf[:, sl], preferred_element_type=f32)
        return jnp.where(same_head, kv, 0.0).astype(bf16)

    def m_part(g, kv):
        sl = slice(g * 128, (g + 1) * 128)
        m_buf[sl, :] = jnp.dot(kv, wo_buf[sl, :], preferred_element_type=f32).astype(bf16)

    rmax = jnp.max(best[0], axis=0, keepdims=True)
    idx = jnp.clip(jnp.min(jnp.where(best[0] == rmax, best[1], S)), 0, S - 1)
    t_sel = idx // TS
    gate = 1.0 / (1.0 + jnp.exp(-rmax[:, :1]))
    wqt_buf[D - CW:D, :] = wq_buf[:, D - CW:D].T
    z = jnp.sum(z_acc[...], axis=0, keepdims=True)
    zb_buf[...] = jnp.broadcast_to(z, (128, D)).T
    r16 = pl.multiple_of((idx // 16) * 16, 16)
    blk = xn_buf[pl.ds(r16, 16), :].astype(f32)
    sel = lax.broadcasted_iota(jnp.int32, (16, D), 0) == (idx - r16)
    x_sel = jnp.sum(jnp.where(sel, blk, 0.0), axis=0, keepdims=True)
    xb_buf[...] = jnp.broadcast_to(x_sel, (128, D)).T

    kv_prev = kv_part(0)
    for g in range(1, G128):
        kv = kv_part(g)
        m_part(g - 1, kv_prev)
        kv_prev = kv
    m_part(G128 - 1, kv_prev)

    def phase2(j, carry):
        with _scope("p2_wait"):
            for jj in range(NT - 1):
                @pl.when(j == jj)
                def _():
                    for c in ffn_copies(jj):
                        c.wait()
        with _scope("p2_body"):
            t = lax.rem(t_sel + 1 + j, NT)
            trows = pl.ds(pl.multiple_of(t * TS, TS), TS)
            xn = xn_buf[trows, :]
            j_up = jnp.minimum(j, NT - 2)
            j_dn = jnp.maximum(j - 1, 0)
            n_dup = FPC * (NT - 1) - NFU
            keep_dup = jnp.where(j >= NT - 2, 0.0, 1.0)

            def fold(a):
                return a[:, :128] + a[:, 128:]

            def matvec(w_ref, slot, nrows, cols, col_ref):
                acc = None
                for r in range(0, nrows, STEP):
                    w = w_ref[slot, r:r + STEP, cols].astype(f32)
                    cr = col_ref[r:r + STEP, :]
                    p = w * jnp.concatenate([cr] * (FW // 128), axis=1)
                    for g in range(0, STEP, 8):
                        acc = p[g:g + 8, :] if acc is None else acc + p[g:g + 8, :]
                    yield fold(acc)
                return acc

            def ffn_work():
                for e in range(D // FW):
                    ec = slice(e * FW, (e + 1) * FW)
                    acc = yield from matvec(wd_buf, j_dn, FPC * FW, ec, hb_buf)
                    y_acc[:, ec] += acc
                for u in range(FPC):
                    fs = slice(u * FW, (u + 1) * FW)
                    g = yield from matvec(wg_buf, j_up, D, fs, xb_buf)
                    a = yield from matvec(wu_buf, j_up, D, fs, xb_buf)
                    g = jnp.sum(g, axis=0, keepdims=True)
                    h = g * (1.0 / (1.0 + jnp.exp(-g))) * jnp.sum(a, axis=0, keepdims=True)
                    if u < n_dup:
                        h = h * keep_dup
                    hb_buf[u * FW:(u + 1) * FW, :] = jnp.broadcast_to(h, (128, FW)).T

            work = ffn_work()

            ps = []
            for c in range(NC):
                rows = slice(c * CW, (c + 1) * CW)
                qt = lax.dot_general(wqt_buf[rows, :], xn, _NT, preferred_element_type=f32)
                qt = _tie_tiles(qt, work, never, RB)
                pqt = _phi(qt)
                zb = zb_buf[rows, :]
                zfull = jnp.concatenate([zb] * (TS // 128), axis=1)
                hc = CW // DH
                den = jnp.sum((pqt * zfull).reshape(hc, DH, TS), axis=1, keepdims=True) + _EPS
                pt = pqt.reshape(hc, DH, TS) * pl.reciprocal(den, approx=True)
                ps.append(pt.reshape(CW, TS).astype(bf16).T)
            p = jnp.concatenate(ps, axis=1)
            y = jnp.sum(y_acc[...], axis=0, keepdims=True) * gate
            for n, (r0, nr, c0, nc) in enumerate(_OUT_PIECES):
                cols = slice(c0, c0 + nc)
                rows = pl.ds(pl.multiple_of(t * TS + r0, 64), nr)
                o = jnp.dot(p[r0:r0 + nr, :], m_buf[:, cols], preferred_element_type=f32)
                o = _tie_tiles(o, work, never, RB)
                o = o + x_buf[rows, cols].astype(f32) + xn_buf[rows, cols].astype(f32)
                hit = lax.broadcasted_iota(jnp.int32, (nr, nc), 0) == idx - (t * TS + r0)
                out_buf[rows, cols] = (o + jnp.where(hit, y[:, cols], 0.0)).astype(bf16)
                out_copy(t, n).start()
            assert next(work, None) is None
        return carry

    lax.fori_loop(0, NT, phase2, 0)
    with _scope("final_wait"):
        for t in range(NT):
            for n in range(len(_OUT_PIECES)):
                out_copy(t, n).wait()


@jax.jit
def pallas_parallel_sum__linear_attn_block__moe_arch_mod__prompt_kernel(
    A_x: jax.Array,
    A_wqkv: jax.Array,
    A_wo: jax.Array,
    B_x: jax.Array,
    B_w_r: jax.Array,
    B_w_gate: jax.Array,
    B_w_up: jax.Array,
    B_w_down: jax.Array,
):
    any_spec = pl.BlockSpec(memory_space=pl.ANY)
    out = pl.pallas_call(
        _kernel,
        out_shape=jax.ShapeDtypeStruct((S, D), bf16),
        in_specs=[any_spec] * 7,
        out_specs=any_spec,
        scratch_shapes=[
            pltpu.VMEM((S, D), bf16),
            pltpu.VMEM((S + TS, D), bf16),
            pltpu.VMEM((D, D), bf16),
            pltpu.VMEM((D, D), bf16),
            pltpu.VMEM((D, D), bf16),
            pltpu.VMEM((D, D), bf16),
            pltpu.VMEM((D, D), bf16),
            pltpu.VMEM((D, D), bf16),
            pltpu.VMEM((D,), bf16),
            pltpu.VMEM((D, D), f32),
            pltpu.VMEM((8, D), f32),
            pltpu.VMEM((D, 128), f32),
            pltpu.VMEM((NT - 1, D, FPC * FW), bf16),
            pltpu.VMEM((NT - 1, D, FPC * FW), bf16),
            pltpu.VMEM((NT - 1, FPC * FW, D), bf16),
            pltpu.VMEM((D, 128), f32),
            pltpu.VMEM((FPC * FW, 128), f32),
            pltpu.VMEM((8, D), f32),
            pltpu.VMEM((S, D), bf16),
            pltpu.SemaphoreType.DMA((_N_SEM,)),
            pltpu.SemaphoreType.DMA((NT * len(_OUT_PIECES),)),
        ],
        compiler_params=pltpu.CompilerParams(vmem_limit_bytes=100 * 1024 * 1024,
                                             disable_semaphore_checks=True),
        name="linattn_mod",
    )(A_x.reshape(S, D), A_wqkv, A_wo, B_w_r, B_w_gate, B_w_up, B_w_down)
    return out.reshape(1, S, D)
```

```python
import os
import jax
import jax.numpy as jnp
from jax import lax
import jax.experimental.pallas as pl
import jax.experimental.pallas.tpu as pltpu

S = 2048
D = 1024
F = 3584
H = 32
DH = D // H
G128 = D // 128
CW = 256
NC = D // CW
T0 = 256
TS = 512
NT = S // TS
FW = 256
NFU = F // FW
FPC = -(-NFU // (NT - 1))
TLAST = bool(int(os.environ.get("TLAST", 1)))
DEPX = bool(int(os.environ.get("DEPX", 1)))
STEP = int(os.environ.get("STEP", 64))
RB = int(os.environ.get("RB", 32))
LAG = int(os.environ.get("LAG", 8))
LSUB = int(os.environ.get("LSUB", 16))
LSUB0 = int(os.environ.get("LSUB0", 32))
LSUBC = int(os.environ.get("LSUBC", 16))
CWC = int(os.environ.get("CWC", 128))
TIE_B = [int(v) for v in os.environ.get("TIE_B", "0,4,2,2").split(",")]
TIE_C = [int(v) for v in os.environ.get("TIE_C", "4,3,4,4,3,8,6").split(",")]
TIE_L = [int(v) for v in os.environ.get("TIE_L", "8,8,0,8,0,8").split(",")]

_LN_EPS = 1.0013580322265625e-05
_EPS = 1e-6
_SCOPES = False

f32 = jnp.float32
bf16 = jnp.bfloat16

_TAIL = [int(v) for v in os.environ.get("TAIL", "256,128,128").split(",")]
_OUT_PIECES = [(0, TS, c * CW, CW) for c in range(NC - 1)] + [
    (sum(_TAIL[:i]), _TAIL[i], D - CW, CW) for i in range(len(_TAIL))]

_X_ROWS = [(0, T0 // 2), (T0 // 2, T0 // 2), (T0, T0)] + [(i * TS, TS) for i in range(1, NT)]
_WK_SPLIT = ((0, 128), (128, 384), (384, 640), (640, 1024))
_SEM_X = 0
_SEM_WK = _SEM_X + len(_X_ROWS)
_SEM_WQ = _SEM_WK + len(_WK_SPLIT)
_SEM_WV = _SEM_WQ + 1
_SEM_WO = _SEM_WV + 1
_SEM_WR = _SEM_WO + 1
_SEM_F = _SEM_WR + 1
_N_SEM = _SEM_F + 3 * (NT - 1)


class _NoScope:
    def __enter__(self):
        return self

    def __exit__(self, *a):
        return False


def _scope(name):
    return jax.named_scope(name) if _SCOPES else _NoScope()


def _bf16_round(v):
    return v.astype(bf16).astype(f32)


def _phi(t):
    return jnp.where(t > 0, t + 1.0, jnp.exp(t)) + _EPS


def _tie(val, dep, never, last=False):
    if dep is None:
        return val
    r = 8 * (4 // val.dtype.itemsize)
    if r > 8:
        dep = jnp.concatenate([dep] * (r // 8), axis=0)
    if last:
        tail = jnp.where(never, dep.astype(val.dtype), val[-r:, -128:])
        bottom = jnp.concatenate([val[-r:, :-128], tail], axis=1) if val.shape[1] > 128 else tail
        return jnp.concatenate([val[:-r, :], bottom], axis=0)
    head = jnp.where(never, dep.astype(val.dtype), val[:r, :128])
    top = jnp.concatenate([head, val[:r, 128:]], axis=1)
    return jnp.concatenate([top, val[r:, :]], axis=0)


def _tie_tiles(val, deps, never, rb):
    cols = []
    for n in range(val.shape[1] // 128):
        parts = []
        for r in range(0, val.shape[0], rb):
            blk = val[r:r + rb, n * 128:(n + 1) * 128]
            dep = next(deps, None)
            if dep is not None:
                tail = jnp.where(never, dep, blk[rb - 8:, :])
                blk = jnp.concatenate([blk[:rb - 8, :], tail], axis=0) if rb > 8 else tail
            parts.append(blk)
        cols.append(jnp.concatenate(parts, axis=0))
    return jnp.concatenate(cols, axis=1)


def _split(items, n):
    k = len(items)
    return [items[(i * k) // n:((i + 1) * k) // n] for i in range(n)]


_TN = (((0,), (0,)), ((), ()))
_NT = (((1,), (1,)), ((), ()))


def _kernel(x_hbm, wqkv_hbm, wo_hbm, wr_hbm, wg_hbm, wu_hbm, wd_hbm, out_hbm,
            x_buf, xn_buf, wq_buf, wk_buf, wv_buf, wqt_buf, wo_buf, m_buf, wr_buf,
            g_acc, z_acc, zb_buf,
            wg_buf, wu_buf, wd_buf, xb_buf, hb_buf, y_acc, out_buf,
            sem, o_sem):

    def x_copy(i):
        if isinstance(i, int):
            rows = pl.ds(*_X_ROWS[i])
        else:
            rows = pl.ds(pl.multiple_of((i - 2) * TS, TS), TS)
        return pltpu.make_async_copy(x_hbm.at[rows, :], x_buf.at[rows, :], sem.at[_SEM_X + i])

    def wk_copy(s):
        c0, c1 = _WK_SPLIT[s]
        return pltpu.make_async_copy(
            wqkv_hbm.at[:, pl.ds(D + c0, c1 - c0)],
            wk_buf.at[:, pl.ds(c0, c1 - c0)], sem.at[_SEM_WK + s])

    wq_copy = pltpu.make_async_copy(wqkv_hbm.at[:, pl.ds(0, D)], wq_buf, sem.at[_SEM_WQ])
    wv_copy = pltpu.make_async_copy(wqkv_hbm.at[:, pl.ds(2 * D, D)], wv_buf.at[:, pl.ds(0, D)],
                                    sem.at[_SEM_WV])
    wo_copy = pltpu.make_async_copy(wo_hbm, wo_buf, sem.at[_SEM_WO])
    wr_copy = pltpu.make_async_copy(wr_hbm, wr_buf, sem.at[_SEM_WR])

    def ffn_copies(j):
        s = _SEM_F + 3 * j
        if isinstance(j, int):
            f0 = min(j * FPC, NFU - FPC) * FW
        else:
            f0 = pl.multiple_of(jnp.minimum(j * FPC, NFU - FPC) * FW, FW)
        fs = pl.ds(f0, FPC * FW)
        return (pltpu.make_async_copy(wg_hbm.at[:, fs], wg_buf.at[j], sem.at[s]),
                pltpu.make_async_copy(wu_hbm.at[:, fs], wu_buf.at[j], sem.at[s + 1]),
                pltpu.make_async_copy(wd_hbm.at[fs, :], wd_buf.at[j], sem.at[s + 2]))

    def out_copy(t, p):
        r0, nr, c0, nc = _OUT_PIECES[p]
        row = t * TS + r0
        rows = pl.ds(row if isinstance(t, int) else pl.multiple_of(row, 64), nr)
        cols = pl.ds(c0, nc)
        return pltpu.make_async_copy(out_buf.at[rows, cols], out_hbm.at[rows, cols],
                                     o_sem.at[t * len(_OUT_PIECES) + p])

    x_copy(0).start()
    x_copy(1).start()
    wr_copy.start()
    wk_copy(0).start()
    wk_copy(1).start()
    x_copy(2).start()
    wk_copy(2).start()
    wk_copy(3).start()
    for i in range(3, len(_X_ROWS)):
        x_copy(i).start()
    wq_copy.start()
    wv_copy.start()
    wo_copy.start()
    for j in range(NT - 1):
        for c in ffn_copies(j):
            c.start(priority=1)

    y_acc[...] = jnp.zeros_like(y_acc)
    hb_buf[...] = jnp.zeros_like(hb_buf)

    sub_iota = lax.broadcasted_iota(jnp.int32, (8, 128), 0)

    def route(xn, row0, best):
        nr = xn.shape[0]
        wr = wr_buf[...].reshape(1, D).astype(f32)
        r = _bf16_round(jnp.sum(xn.astype(f32) * wr, axis=-1, keepdims=True))
        r = jnp.broadcast_to(r, (nr, 128))
        for g in range(0, nr, 8):
            rg = r[g:g + 8, :]
            better = rg > best[0]
            best[0] = jnp.where(better, rg, best[0])
            best[1] = jnp.where(better, sub_iota + (row0 + g), best[1])

    def layernorm(src, dst, nr, best, after=None, never=None):
        x = x_buf[pl.ds(src, nr), :].astype(f32)
        x = _tie(x, after, never)
        mean = jnp.sum(x, axis=-1, keepdims=True) * (1.0 / D)
        mean_b = _bf16_round(mean)
        e = x - mean_b
        off = mean - mean_b
        var = jnp.sum(e * e, axis=-1, keepdims=True) * (1.0 / D) - off * off
        sd = _bf16_round(jnp.sqrt(_bf16_round(_bf16_round(var) + _LN_EPS)))
        rs = pl.reciprocal(sd, approx=True)
        rs = jnp.where(sd == jnp.inf, 0.0, rs * (2.0 - sd * rs))
        xf = _bf16_round(e) * rs
        xn = xf.astype(bf16)
        xn_buf[pl.ds(dst, nr), :] = xn
        if best is not None:
            route(xn, src, best)
        dep = None
        for g in range(0, nr, 8):
            dg = xf[g:g + 8, D - 128:]
            dep = dg if dep is None else dep + dg
        return dep, sd

    def ln_work(src, dst, sub, counts, best, never):
        o = 0
        for n in counts:
            dep = None
            for _ in range(n):
                dep = layernorm(src + o, dst + o, sub, best, dep, never)[0]
                o += sub
            yield dep

    def kg_steps(jobs, work, never):
        def tied(val):
            return _tie(val, next(work, None), never, True)

        def k_part(xn, c0, cw, init):
            cols = slice(c0, c0 + cw)
            xn = xn()
            k = tied(jnp.dot(xn, wk_buf[:, cols], preferred_element_type=f32))
            pk = _phi(k)
            zc = jnp.sum(pk.reshape(xn.shape[0] // 8, 8, cw), axis=0)
            z_acc[:, cols] = zc if init else z_acc[:, cols] + zc
            return pk.astype(bf16)

        def g_part(pk, xn, c0, cw, init):
            rows = slice(c0, c0 + cw)
            g = tied(lax.dot_general(pk, xn(), _TN, preferred_element_type=f32))
            g_acc[rows, :] = g if init else g_acc[rows, :] + g

        prev = None
        for job in jobs:
            if job is None:
                g_part(prev[0], *prev[1])
                prev = None
                continue
            pk = k_part(*job)
            if prev is not None:
                g_part(prev[0], *prev[1])
            prev = (pk, job)
        g_part(prev[0], *prev[1])
        assert next(work, None) is None

    def rows_of(r0, nr):
        got = []

        def get():
            if not got:
                got.append(xn_buf[pl.ds(r0, nr), :])
            return got[0]
        return get

    best = [jnp.full((8, 128), -jnp.inf, f32), jnp.zeros((8, 128), jnp.int32)]
    with _scope("wait_x0"):
        x_copy(0).wait()
    with _scope("ln0"):
        sd0 = layernorm(0, 0, T0 // 2, None)[1]
    with _scope("wait_x0"):
        x_copy(1).wait()
    with _scope("ln0"):
        layernorm(T0 // 2, T0 // 2, T0 // 2, None)
    with _scope("wait_wk0"):
        wr_copy.wait()
        wk_copy(0).wait()
    never = jnp.min(sd0[0:8, :]) < 0.0

    def route_work(lead):
        for _ in range(lead):
            yield None
        for r in range(0, T0, T0 // 2):
            route(xn_buf[r:r + T0 // 2, :], r, best)
            yield best[0]

    kg_steps([(rows_of(0, T0 // 2), 0, 128, True), (rows_of(T0 // 2, T0 // 2), 0, 128, False)],
             iter(()), never)
    with _scope("wait_wk1"):
        wk_copy(1).wait()
    xa = rows_of(0, T0)
    kg_steps([(xa, 128, 128, True), (xa, 256, 128, True)], route_work(1), never)
    with _scope("wait_wk2"):
        x_copy(2).wait()
        wk_copy(2).wait()
    xa, xb = rows_of(0, T0), rows_of(T0, T0)
    assert sum(TIE_B) * LSUB0 == T0
    kg_steps([(xa, 384, 128, True), (xa, 512, 128, True), None,
              (xb, 0, 128, False), (xb, 128, 128, False)],
             ln_work(T0, T0, LSUB0, TIE_B, best, never), never)
    with _scope("wait_wk3"):
        wk_copy(3).wait()
        x_copy(3).wait()
    xa, xb = rows_of(0, TS), rows_of(T0, T0)
    assert sum(TIE_C) * LSUBC == TS
    kg_steps([(xb, 256, 256, False), (xb, 512, 128, False), (xa, 640, 128, True), (xa, 768, 256, True)],
             ln_work(TS, TS, LSUBC, TIE_C, best, never), never)
    with _scope("wait_wq"):
        wq_copy.wait()

    def phase1(i, carry):
        with _scope("p1_wait"):
            @pl.when(i + 1 < NT)
            def _():
                x_copy(i + 3).wait()
        with _scope("p1_body"):
            best = list(carry)
            r0 = pl.multiple_of(i * TS, TS)
            src = pl.multiple_of(jnp.minimum(r0 + TS, S - TS), TS)
            dst = pl.multiple_of(r0 + TS, TS)
            qrows = pl.ds(pl.multiple_of((i - 1) * CW, CW), CW)
            wqt_buf[qrows, :] = wq_buf[:, qrows].T
            xa = rows_of(r0, TS)
            assert sum(TIE_L) * LSUB == TS
            kg_steps([(xa, c * CW, CW, False) for c in range(NC)],
                     ln_work(src, dst, LSUB, TIE_L, best, never), never)
        return tuple(best)

    best = lax.fori_loop(1, NT, phase1, tuple(best))

    wv_copy.wait()
    wo_copy.wait()
    rr = lax.broadcasted_iota(jnp.int32, (128, 128), 0) // DH
    cc = lax.broadcasted_iota(jnp.int32, (128, 128), 1) // DH
    same_head = rr == cc

    def kv_part(g):
        sl = slice(g * 128, (g + 1) * 128)
        kv = jnp.dot(g_acc[sl, :].astype(bf16), wv_buf[:, sl], preferred_element_type=f32)
        return jnp.where(same_head, kv, 0.0).astype(bf16)

    def m_part(g, kv):
        sl = slice(g * 128, (g + 1) * 128)
        m_buf[sl, :] = jnp.dot(kv, wo_buf[sl, :], preferred_element_type=f32).astype(bf16)

    rmax = jnp.max(best[0], axis=0, keepdims=True)
    idx = jnp.clip(jnp.min(jnp.where(best[0] == rmax, best[1], S)), 0, S - 1)
    t_sel = idx // TS
    gate = 1.0 / (1.0 + jnp.exp(-rmax[:, :1]))
    wqt_buf[D - CW:D, :] = wq_buf[:, D - CW:D].T
    z = jnp.sum(z_acc[...], axis=0, keepdims=True)
    zb_buf[...] = jnp.broadcast_to(z, (128, D)).T
    r16 = pl.multiple_of((idx // 16) * 16, 16)
    blk = xn_buf[pl.ds(r16, 16), :].astype(f32)
    sel = lax.broadcasted_iota(jnp.int32, (16, D), 0) == (idx - r16)
    x_sel = jnp.sum(jnp.where(sel, blk, 0.0), axis=0, keepdims=True)
    xb_buf[...] = jnp.broadcast_to(x_sel, (128, D)).T

    kv_prev = kv_part(0)
    for g in range(1, G128):
        kv = kv_part(g)
        m_part(g - 1, kv_prev)
        kv_prev = kv
    m_part(G128 - 1, kv_prev)

    def phase2(j, t_prev):
        with _scope("p2_wait"):
            @pl.when(j < NT - 1)
            def _():
                for c in ffn_copies(j):
                    c.wait()
        with _scope("p2_body"):
            t = (t_prev + 1) & (NT - 1)
            trows = pl.ds(pl.multiple_of(t * TS, TS), TS)
            xn = xn_buf[trows, :]
            j_up = jnp.minimum(j, NT - 2)
            j_dn = jnp.maximum(j - 1, 0)
            n_dup = FPC * (NT - 1) - NFU
            keep_dup = jnp.where(j >= NT - 2, 0.0, 1.0)

            def fold(a):
                return a[:, :128] + a[:, 128:]

            def matvec(w_ref, slot, nrows, cols, col_ref):
                acc = None
                for r in range(0, nrows, STEP):
                    w = w_ref[slot, r:r + STEP, cols].astype(f32)
                    cr = col_ref[r:r + STEP, :]
                    p = w * jnp.concatenate([cr] * (FW // 128), axis=1)
                    for g in range(0, STEP, 8):
                        acc = p[g:g + 8, :] if acc is None else acc + p[g:g + 8, :]
                    yield fold(acc)
                return acc

            def ffn_work():
                for e in range(D // FW):
                    ec = slice(e * FW, (e + 1) * FW)
                    acc = yield from matvec(wd_buf, j_dn, FPC * FW, ec, hb_buf)
                    y_acc[:, ec] += acc
                for u in range(FPC):
                    fs = slice(u * FW, (u + 1) * FW)
                    g = yield from matvec(wg_buf, j_up, D, fs, xb_buf)
                    a = yield from matvec(wu_buf, j_up, D, fs, xb_buf)
                    g = jnp.sum(g, axis=0, keepdims=True)
                    h = g * (1.0 / (1.0 + jnp.exp(-g))) * jnp.sum(a, axis=0, keepdims=True)
                    if u < n_dup:
                        h = h * keep_dup
                    hb = jnp.broadcast_to(h, (128, FW)).T
                    hb_buf[u * FW:(u + 1) * FW, :] = hb
                    late.append([LAG, hb[120:128, :] + hb[FW - 8:, :]])

            late = []

            def with_late(gen):
                while True:
                    dep = next(gen, None)
                    if dep is None and not late:
                        return
                    for e in late:
                        e[0] -= 1
                    if late and late[0][0] <= 0:
                        d = late.pop(0)[1]
                        dep = d if dep is None else dep + d
                    yield dep

            work = with_late(ffn_work())

            ps = []
            for c in range(NC):
                rows = slice(c * CW, (c + 1) * CW)
                qt = lax.dot_general(wqt_buf[rows, :], xn, _NT, preferred_element_type=f32)
                qt = _tie_tiles(qt, work, never, RB)
                pqt = _phi(qt)
                zb = zb_buf[rows, :]
                zfull = jnp.concatenate([zb] * (TS // 128), axis=1)
                hc = CW // DH
                den = jnp.sum((pqt * zfull).reshape(hc, DH, TS), axis=1, keepdims=True) + _EPS
                pt = pqt.reshape(hc, DH, TS) * pl.reciprocal(den, approx=True)
                ps.append(pt.reshape(CW, TS).astype(bf16).T)
            p = jnp.concatenate(ps, axis=1)
            y = jnp.sum(y_acc[...], axis=0, keepdims=True) * gate
            for n, (r0, nr, c0, nc) in enumerate(_OUT_PIECES):
                cols = slice(c0, c0 + nc)
                rows = pl.ds(pl.multiple_of(t * TS + r0, 64), nr)
                o = jnp.dot(p[r0:r0 + nr, :], m_buf[:, cols], preferred_element_type=f32)
                o = _tie_tiles(o, work, never, RB)
                o = o + x_buf[rows, cols].astype(f32) + xn_buf[rows, cols].astype(f32)
                hit = lax.broadcasted_iota(jnp.int32, (nr, nc), 0) == idx - (t * TS + r0)
                out_buf[rows, cols] = (o + jnp.where(hit, y[:, cols], 0.0)).astype(bf16)
                out_copy(t, n).start()
            assert next(work, 0) == 0
        return t

    lax.fori_loop(0, NT, phase2, t_sel)
    with _scope("final_wait"):
        for t in range(NT):
            for n in range(len(_OUT_PIECES)):
                out_copy(t, n).wait()


@jax.jit
def pallas_parallel_sum__linear_attn_block__moe_arch_mod__prompt_kernel(
    A_x: jax.Array,
    A_wqkv: jax.Array,
    A_wo: jax.Array,
    B_x: jax.Array,
    B_w_r: jax.Array,
    B_w_gate: jax.Array,
    B_w_up: jax.Array,
    B_w_down: jax.Array,
):
    any_spec = pl.BlockSpec(memory_space=pl.ANY)
    out = pl.pallas_call(
        _kernel,
        out_shape=jax.ShapeDtypeStruct((S, D), bf16),
        in_specs=[any_spec] * 7,
        out_specs=any_spec,
        scratch_shapes=[
            pltpu.VMEM((S, D), bf16),
            pltpu.VMEM((S + TS, D), bf16),
            pltpu.VMEM((D, D), bf16),
            pltpu.VMEM((D, D + 128), bf16),
            pltpu.VMEM((D, D + 128), bf16),
            pltpu.VMEM((D, D), bf16),
            pltpu.VMEM((D, D), bf16),
            pltpu.VMEM((D, D), bf16),
            pltpu.VMEM((D,), bf16),
            pltpu.VMEM((D, D), f32),
            pltpu.VMEM((8, D), f32),
            pltpu.VMEM((D, 128), f32),
            pltpu.VMEM((NT - 1, D, FPC * FW), bf16),
            pltpu.VMEM((NT - 1, D, FPC * FW), bf16),
            pltpu.VMEM((NT - 1, FPC * FW, D), bf16),
            pltpu.VMEM((D, 128), f32),
            pltpu.VMEM((FPC * FW, 128), f32),
            pltpu.VMEM((8, D), f32),
            pltpu.VMEM((S, D), bf16),
            pltpu.SemaphoreType.DMA((_N_SEM,)),
            pltpu.SemaphoreType.DMA((NT * len(_OUT_PIECES),)),
        ],
        compiler_params=pltpu.CompilerParams(vmem_limit_bytes=100 * 1024 * 1024,
                                             disable_semaphore_checks=True),
        name="linattn_mod",
    )(A_x.reshape(S, D), A_wqkv, A_wo, B_w_r, B_w_gate, B_w_up, B_w_down)
    return out.reshape(1, S, D)
```

```python
import jax
import jax.numpy as jnp
from jax import lax
import jax.experimental.pallas as pl
import jax.experimental.pallas.tpu as pltpu

S = 2048
D = 1024
F = 3584
H = 32
DH = D // H
G128 = D // 128
CW = 256
NC = D // CW
T0 = 256
TS = 512
NT = S // TS
FW = 256
NFU = F // FW
FPC = -(-NFU // (NT - 1))

FFN_STEP = 64
FFN_RB = 32
FFN_LAG = 8
LN_C = (32, (0, 4, 2, 2))
LN_D = (16, (4, 3, 4, 4, 3, 8, 6))
LN_LOOP = (16, (9, 8, 0, 8, 0, 7))

_LN_EPS = 1.0013580322265625e-05
_EPS = 1e-6

f32 = jnp.float32
bf16 = jnp.bfloat16

_OUT_PIECES = [(0, TS, c * CW, CW) for c in range(NC - 1)] + [
    (0, 256, D - CW, CW), (256, 128, D - CW, CW), (384, 128, D - CW, CW)]

_X_ROWS = [(0, T0 // 2), (T0 // 2, T0 // 2), (T0, T0)] + [(i * TS, TS) for i in range(1, NT)]
_WK_COLS = ((0, 128), (128, 384), (384, 640), (640, 1024))
_SEM_X = 0
_SEM_WK = _SEM_X + len(_X_ROWS)
_SEM_WQ = _SEM_WK + len(_WK_COLS)
_SEM_WV = _SEM_WQ + NC
_SEM_WO = _SEM_WV + 1
_SEM_WR = _SEM_WO + 1
_SEM_F = _SEM_WR + 1
_N_SEM = _SEM_F + 3 * (NT - 1)

_TN = (((0,), (0,)), ((), ()))
_NT = (((1,), (1,)), ((), ()))


def _bf16_round(v):
    return v.astype(bf16).astype(f32)


def _phi(t):
    return jnp.where(t > 0, t + 1.0, jnp.exp(t)) + _EPS


def _tie(val, dep, never, last=False):
    if dep is None:
        return val
    if last:
        tail = jnp.where(never, dep, val[-8:, -128:])
        if val.shape[1] > 128:
            tail = jnp.concatenate([val[-8:, :-128], tail], axis=1)
        return jnp.concatenate([val[:-8, :], tail], axis=0)
    head = jnp.where(never, dep, val[:8, :128])
    head = jnp.concatenate([head, val[:8, 128:]], axis=1)
    return jnp.concatenate([head, val[8:, :]], axis=0)


def _tie_tiles(val, deps, never, rb):
    cols = []
    for n in range(val.shape[1] // 128):
        blocks = [_tie(val[r:r + rb, n * 128:(n + 1) * 128], next(deps, None), never, True)
                  for r in range(0, val.shape[0], rb)]
        cols.append(jnp.concatenate(blocks, axis=0))
    return jnp.concatenate(cols, axis=1)


def _kernel(x_hbm, wqkv_hbm, wo_hbm, wr_hbm, wg_hbm, wu_hbm, wd_hbm, out_hbm,
            x_buf, xn_buf, wq_buf, wk_buf, wv_buf, wqt_buf, wo_buf, m_buf, wr_buf,
            g_acc, z_acc, zb_buf,
            wg_buf, wu_buf, wd_buf, xb_buf, hb_buf, y_acc, out_buf,
            sem, o_sem):

    def x_copy(i):
        if isinstance(i, int):
            rows = pl.ds(*_X_ROWS[i])
        else:
            rows = pl.ds(pl.multiple_of((i - 2) * TS, TS), TS)
        return pltpu.make_async_copy(x_hbm.at[rows, :], x_buf.at[rows, :], sem.at[_SEM_X + i])

    def wk_copy(s):
        c0, c1 = _WK_COLS[s]
        return pltpu.make_async_copy(wqkv_hbm.at[:, pl.ds(D + c0, c1 - c0)],
                                     wk_buf.at[:, pl.ds(c0, c1 - c0)], sem.at[_SEM_WK + s])

    def wq_copy(c):
        return pltpu.make_async_copy(wqkv_hbm.at[:, pl.ds(c * CW, CW)], wq_buf.at[c],
                                     sem.at[_SEM_WQ + c])

    wv_copy = pltpu.make_async_copy(wqkv_hbm.at[:, pl.ds(2 * D, D)], wv_buf.at[:, pl.ds(0, D)],
                                    sem.at[_SEM_WV])
    wo_copy = pltpu.make_async_copy(wo_hbm, wo_buf, sem.at[_SEM_WO])
    wr_copy = pltpu.make_async_copy(wr_hbm, wr_buf, sem.at[_SEM_WR])

    def ffn_copies(j):
        s = _SEM_F + 3 * j
        if isinstance(j, int):
            f0 = min(j * FPC, NFU - FPC) * FW
        else:
            f0 = pl.multiple_of(jnp.minimum(j * FPC, NFU - FPC) * FW, FW)
        fs = pl.ds(f0, FPC * FW)
        return (pltpu.make_async_copy(wg_hbm.at[:, fs], wg_buf.at[j], sem.at[s]),
                pltpu.make_async_copy(wu_hbm.at[:, fs], wu_buf.at[j], sem.at[s + 1]),
                pltpu.make_async_copy(wd_hbm.at[fs, :], wd_buf.at[j], sem.at[s + 2]))

    def out_copy(t, p):
        r0, nr, c0, nc = _OUT_PIECES[p]
        row = t * TS + r0
        rows = pl.ds(row if isinstance(t, int) else pl.multiple_of(row, 64), nr)
        cols = pl.ds(c0, nc)
        return pltpu.make_async_copy(out_buf.at[rows, cols], out_hbm.at[rows, cols],
                                     o_sem.at[t * len(_OUT_PIECES) + p])

    x_copy(0).start()
    x_copy(1).start()
    wr_copy.start()
    wk_copy(0).start()
    wk_copy(1).start()
    x_copy(2).start()
    wk_copy(2).start()
    wk_copy(3).start()
    for i in range(3, len(_X_ROWS)):
        x_copy(i).start()
    for c in range(NC):
        wq_copy(c).start()
    wv_copy.start()
    wo_copy.start()
    for j in range(NT - 1):
        for c in ffn_copies(j):
            c.start(priority=1)

    y_acc[...] = jnp.zeros_like(y_acc)
    hb_buf[...] = jnp.zeros_like(hb_buf)

    sub_iota = lax.broadcasted_iota(jnp.int32, (8, 128), 0)

    def route(xn, row0, best):
        nr = xn.shape[0]
        wr = wr_buf[...].reshape(1, D).astype(f32)
        r = _bf16_round(jnp.sum(xn.astype(f32) * wr, axis=-1, keepdims=True))
        r = jnp.broadcast_to(r, (nr, 128))
        for g in range(0, nr, 8):
            rg = r[g:g + 8, :]
            better = rg > best[0]
            best[0] = jnp.where(better, rg, best[0])
            best[1] = jnp.where(better, sub_iota + (row0 + g), best[1])

    def layernorm(src, dst, nr, best, after=None, never=None):
        x = x_buf[pl.ds(src, nr), :].astype(f32)
        x = _tie(x, after, never)
        mean = jnp.sum(x, axis=-1, keepdims=True) * (1.0 / D)
        mean_b = _bf16_round(mean)
        e = x - mean_b
        off = mean - mean_b
        var = jnp.sum(e * e, axis=-1, keepdims=True) * (1.0 / D) - off * off
        sd = _bf16_round(jnp.sqrt(_bf16_round(_bf16_round(var) + _LN_EPS)))
        rs = pl.reciprocal(sd, approx=True)
        rs = jnp.where(sd == jnp.inf, 0.0, rs * (2.0 - sd * rs))
        xf = _bf16_round(e) * rs
        xn = xf.astype(bf16)
        xn_buf[pl.ds(dst, nr), :] = xn
        if best is not None:
            route(xn, src, best)
        dep = None
        for g in range(0, nr, 8):
            dg = xf[g:g + 8, D - 128:]
            dep = dg if dep is None else dep + dg
        return dep, sd

    def ln_work(src, dst, nr, plan, best, never):
        sub, counts = plan
        assert sub * sum(counts) == nr
        o = 0
        for n in counts:
            dep = None
            for _ in range(n):
                dep = layernorm(src + o, dst + o, sub, best, dep, never)[0]
                o += sub
            yield dep

    def rows_of(r0, nr):
        got = []

        def get():
            if not got:
                got.append(xn_buf[pl.ds(r0, nr), :])
            return got[0]
        return get

    def kg_steps(jobs, work, never):
        def tied(val):
            return _tie(val, next(work, None), never, True)

        def k_part(xn, c0, cw, init):
            cols = slice(c0, c0 + cw)
            xn = xn()
            pk = _phi(tied(jnp.dot(xn, wk_buf[:, cols], preferred_element_type=f32)))
            zc = jnp.sum(pk.reshape(xn.shape[0] // 8, 8, cw), axis=0)
            z_acc[:, cols] = zc if init else z_acc[:, cols] + zc
            return pk.astype(bf16)

        def g_part(pk, xn, c0, cw, init):
            rows = slice(c0, c0 + cw)
            g = tied(lax.dot_general(pk, xn(), _TN, preferred_element_type=f32))
            g_acc[rows, :] = g if init else g_acc[rows, :] + g

        prev = None
        for job in jobs:
            if job is None:
                g_part(prev[0], *prev[1])
                prev = None
                continue
            pk = k_part(*job)
            if prev is not None:
                g_part(prev[0], *prev[1])
            prev = (pk, job)
        g_part(prev[0], *prev[1])
        assert next(work, None) is None

    best = [jnp.full((8, 128), -jnp.inf, f32), jnp.zeros((8, 128), jnp.int32)]
    x_copy(0).wait()
    sd0 = layernorm(0, 0, T0 // 2, None)[1]
    x_copy(1).wait()
    layernorm(T0 // 2, T0 // 2, T0 // 2, None)
    wr_copy.wait()
    wk_copy(0).wait()
    never = jnp.min(sd0[0:8, :]) < 0.0
    kg_steps([(rows_of(0, T0 // 2), 0, 128, True), (rows_of(T0 // 2, T0 // 2), 0, 128, False)],
             iter(()), never)

    def route_first():
        yield None
        for r in range(0, T0, T0 // 2):
            route(xn_buf[r:r + T0 // 2, :], r, best)
            yield best[0]

    wk_copy(1).wait()
    xa = rows_of(0, T0)
    kg_steps([(xa, 128, 128, True), (xa, 256, 128, True)], route_first(), never)

    x_copy(2).wait()
    wk_copy(2).wait()
    xa, xb = rows_of(0, T0), rows_of(T0, T0)
    kg_steps([(xa, 384, 128, True), (xa, 512, 128, True), None,
              (xb, 0, 128, False), (xb, 128, 128, False)],
             ln_work(T0, T0, T0, LN_C, best, never), never)

    wk_copy(3).wait()
    x_copy(3).wait()
    xa, xb = rows_of(0, TS), rows_of(T0, T0)
    kg_steps([(xb, 256, 256, False), (xb, 512, 128, False),
              (xa, 640, 128, True), (xa, 768, 256, True)],
             ln_work(TS, TS, TS, LN_D, best, never), never)
    for c in range(NC):
        wq_copy(c).wait()

    def phase1(i, carry):
        @pl.when(i + 1 < NT)
        def _():
            x_copy(i + 3).wait()

        best = list(carry)
        r0 = pl.multiple_of(i * TS, TS)
        src = pl.multiple_of(jnp.minimum(r0 + TS, S - TS), TS)
        dst = pl.multiple_of(r0 + TS, TS)
        wqt_buf[pl.ds(pl.multiple_of((i - 1) * CW, CW), CW), :] = wq_buf[i - 1].T
        xa = rows_of(r0, TS)
        kg_steps([(xa, c * CW, CW, False) for c in range(NC)],
                 ln_work(src, dst, TS, LN_LOOP, best, never), never)
        return tuple(best)

    best = lax.fori_loop(1, NT, phase1, tuple(best))

    wv_copy.wait()
    wo_copy.wait()
    rr = lax.broadcasted_iota(jnp.int32, (128, 128), 0) // DH
    cc = lax.broadcasted_iota(jnp.int32, (128, 128), 1) // DH
    same_head = rr == cc

    def kv_part(g):
        sl = slice(g * 128, (g + 1) * 128)
        kv = jnp.dot(g_acc[sl, :].astype(bf16), wv_buf[:, sl], preferred_element_type=f32)
        return jnp.where(same_head, kv, 0.0).astype(bf16)

    def m_part(g, kv):
        sl = slice(g * 128, (g + 1) * 128)
        m_buf[sl, :] = jnp.dot(kv, wo_buf[sl, :], preferred_element_type=f32).astype(bf16)

    rmax = jnp.max(best[0], axis=0, keepdims=True)
    idx = jnp.clip(jnp.min(jnp.where(best[0] == rmax, best[1], S)), 0, S - 1)
    gate = 1.0 / (1.0 + jnp.exp(-rmax[:, :1]))
    wqt_buf[D - CW:D, :] = wq_buf[NC - 1].T
    z = jnp.sum(z_acc[...], axis=0, keepdims=True)
    zb_buf[...] = jnp.broadcast_to(z, (128, D)).T
    r16 = pl.multiple_of((idx // 16) * 16, 16)
    blk = xn_buf[pl.ds(r16, 16), :].astype(f32)
    sel = lax.broadcasted_iota(jnp.int32, (16, D), 0) == (idx - r16)
    x_sel = jnp.sum(jnp.where(sel, blk, 0.0), axis=0, keepdims=True)
    xb_buf[...] = jnp.broadcast_to(x_sel, (128, D)).T

    kv_prev = kv_part(0)
    for g in range(1, G128):
        kv = kv_part(g)
        m_part(g - 1, kv_prev)
        kv_prev = kv
    m_part(G128 - 1, kv_prev)

    def phase2(j, t_prev):
        @pl.when(j < NT - 1)
        def _():
            for c in ffn_copies(j):
                c.wait()

        t = (t_prev + 1) & (NT - 1)
        xn = xn_buf[pl.ds(pl.multiple_of(t * TS, TS), TS), :]
        j_up = jnp.minimum(j, NT - 2)
        j_dn = jnp.maximum(j - 1, 0)
        n_dup = FPC * (NT - 1) - NFU
        keep_dup = jnp.where(j >= NT - 2, 0.0, 1.0)
        late = []

        def matvec(w_ref, slot, nrows, cols, col_ref):
            acc = None
            for r in range(0, nrows, FFN_STEP):
                w = w_ref[slot, r:r + FFN_STEP, cols].astype(f32)
                p = w * jnp.concatenate([col_ref[r:r + FFN_STEP, :]] * (FW // 128), axis=1)
                for g in range(0, FFN_STEP, 8):
                    acc = p[g:g + 8, :] if acc is None else acc + p[g:g + 8, :]
                yield acc[:, :128] + acc[:, 128:]
            return acc

        def ffn_work():
            for e in range(D // FW):
                ec = slice(e * FW, (e + 1) * FW)
                acc = yield from matvec(wd_buf, j_dn, FPC * FW, ec, hb_buf)
                y_acc[:, ec] += acc
            for u in range(FPC):
                fs = slice(u * FW, (u + 1) * FW)
                g = yield from matvec(wg_buf, j_up, D, fs, xb_buf)
                a = yield from matvec(wu_buf, j_up, D, fs, xb_buf)
                g = jnp.sum(g, axis=0, keepdims=True)
                h = g * (1.0 / (1.0 + jnp.exp(-g))) * jnp.sum(a, axis=0, keepdims=True)
                if u < n_dup:
                    h = h * keep_dup
                hb = jnp.broadcast_to(h, (128, FW)).T
                hb_buf[fs, :] = hb
                late.append([FFN_LAG, hb[120:128, :] + hb[FW - 8:, :]])

        def with_late(gen):
            while True:
                dep = next(gen, None)
                if dep is None and not late:
                    return
                for e in late:
                    e[0] -= 1
                if late and late[0][0] <= 0:
                    d = late.pop(0)[1]
                    dep = d if dep is None else dep + d
                yield dep

        work = with_late(ffn_work())

        ps = []
        for c in range(NC):
            rows = slice(c * CW, (c + 1) * CW)
            qt = lax.dot_general(wqt_buf[rows, :], xn, _NT, preferred_element_type=f32)
            pqt = _phi(_tie_tiles(qt, work, never, FFN_RB))
            zfull = jnp.concatenate([zb_buf[rows, :]] * (TS // 128), axis=1)
            hc = CW // DH
            den = jnp.sum((pqt * zfull).reshape(hc, DH, TS), axis=1, keepdims=True) + _EPS
            pt = pqt.reshape(hc, DH, TS) * pl.reciprocal(den, approx=True)
            ps.append(pt.reshape(CW, TS).astype(bf16).T)
        p = jnp.concatenate(ps, axis=1)
        assert NC * (CW // FFN_RB) * (TS // 128) > (D // FW) * (FPC * FW // FFN_STEP)
        y = jnp.sum(y_acc[...], axis=0, keepdims=True) * gate
        for n, (r0, nr, c0, nc) in enumerate(_OUT_PIECES):
            cols = slice(c0, c0 + nc)
            rows = pl.ds(pl.multiple_of(t * TS + r0, 64), nr)
            o = jnp.dot(p[r0:r0 + nr, :], m_buf[:, cols], preferred_element_type=f32)
            o = _tie_tiles(o, work, never, FFN_RB)
            o = o + x_buf[rows, cols].astype(f32) + xn_buf[rows, cols].astype(f32)
            hit = lax.broadcasted_iota(jnp.int32, (nr, nc), 0) == idx - (t * TS + r0)
            out_buf[rows, cols] = (o + jnp.where(hit, y[:, cols], 0.0)).astype(bf16)
            out_copy(t, n).start()
        assert next(work, 0) == 0
        return t

    lax.fori_loop(0, NT, phase2, idx // TS)
    for t in range(NT):
        for n in range(len(_OUT_PIECES)):
            out_copy(t, n).wait()


@jax.jit
def pallas_parallel_sum__linear_attn_block__moe_arch_mod__prompt_kernel(
    A_x: jax.Array,
    A_wqkv: jax.Array,
    A_wo: jax.Array,
    B_x: jax.Array,
    B_w_r: jax.Array,
    B_w_gate: jax.Array,
    B_w_up: jax.Array,
    B_w_down: jax.Array,
):
    any_spec = pl.BlockSpec(memory_space=pl.ANY)
    out = pl.pallas_call(
        _kernel,
        out_shape=jax.ShapeDtypeStruct((S, D), bf16),
        in_specs=[any_spec] * 7,
        out_specs=any_spec,
        scratch_shapes=[
            pltpu.VMEM((S, D), bf16),
            pltpu.VMEM((S + TS, D), bf16),
            pltpu.VMEM((NC, D, CW), bf16),
            pltpu.VMEM((D, D + 128), bf16),
            pltpu.VMEM((D, D + 128), bf16),
            pltpu.VMEM((D, D), bf16),
            pltpu.VMEM((D, D), bf16),
            pltpu.VMEM((D, D), bf16),
            pltpu.VMEM((D,), bf16),
            pltpu.VMEM((D, D), f32),
            pltpu.VMEM((8, D), f32),
            pltpu.VMEM((D, 128), f32),
            pltpu.VMEM((NT - 1, D, FPC * FW), bf16),
            pltpu.VMEM((NT - 1, D, FPC * FW), bf16),
            pltpu.VMEM((NT - 1, FPC * FW, D), bf16),
            pltpu.VMEM((D, 128), f32),
            pltpu.VMEM((FPC * FW, 128), f32),
            pltpu.VMEM((8, D), f32),
            pltpu.VMEM((S, D), bf16),
            pltpu.SemaphoreType.DMA((_N_SEM,)),
            pltpu.SemaphoreType.DMA((NT * len(_OUT_PIECES),)),
        ],
        compiler_params=pltpu.CompilerParams(vmem_limit_bytes=100 * 1024 * 1024,
                                             disable_semaphore_checks=True),
        name="linattn_mod",
    )(A_x.reshape(S, D), A_wqkv, A_wo, B_w_r, B_w_gate, B_w_up, B_w_down)
    return out.reshape(1, S, D)
```

```python
import jax
import jax.numpy as jnp
from jax import lax
import jax.experimental.pallas as pl
import jax.experimental.pallas.tpu as pltpu

S = 2048
D = 1024
F = 3584
H = 32
DH = D // H
G128 = D // 128
CW = 256
NC = D // CW
T0 = 256
TS = 512
NT = S // TS
FW = 256
NFU = F // FW
FPC = -(-NFU // (NT - 1))

FFN_STEP = 64
FFN_RB = 32
FFN_LAG = 8
LN_C = (32, (0, 0, 6, 2))
LN_D = (16, (0, 0, 8, 0, 0, 17, 7))
LN_LOOP = (16, (9, 8, 0, 8, 0, 7))

_LN_EPS = 1.0013580322265625e-05
_EPS = 1e-6

f32 = jnp.float32
bf16 = jnp.bfloat16

_OUT_PIECES = [(0, TS, c * CW, CW) for c in range(NC - 1)] + [
    (0, 384, D - CW, CW), (384, 128, D - CW, CW)]

_X_ROWS = [(0, T0 // 2), (T0 // 2, T0 // 2), (T0, T0)] + [(i * TS, TS) for i in range(1, NT)]
_WK_COLS = ((0, 128), (128, 384), (384, 640), (640, 1024))
_SEM_X = 0
_SEM_WK = _SEM_X + len(_X_ROWS)
_SEM_WQ = _SEM_WK + len(_WK_COLS)
_SEM_WV = _SEM_WQ + NC
_SEM_WO = _SEM_WV + 1
_SEM_WR = _SEM_WO + 1
_SEM_F = _SEM_WR + 1
_N_SEM = _SEM_F + 3 * (NT - 1)

_TN = (((0,), (0,)), ((), ()))
_NT = (((1,), (1,)), ((), ()))


def _bf16_round(v):
    return v.astype(bf16).astype(f32)


def _phi(t):
    return jnp.where(t > 0, t + 1.0, jnp.exp(t)) + _EPS


def _tie(val, dep, never, last=False):
    if dep is None:
        return val
    if last:
        tail = jnp.where(never, dep, val[-8:, -128:])
        if val.shape[1] > 128:
            tail = jnp.concatenate([val[-8:, :-128], tail], axis=1)
        return jnp.concatenate([val[:-8, :], tail], axis=0)
    head = jnp.where(never, dep, val[:8, :128])
    head = jnp.concatenate([head, val[:8, 128:]], axis=1)
    return jnp.concatenate([head, val[8:, :]], axis=0)


def _tie_tiles(val, deps, never, rb):
    cols = []
    for n in range(val.shape[1] // 128):
        blocks = [_tie(val[r:r + rb, n * 128:(n + 1) * 128], next(deps, None), never, True)
                  for r in range(0, val.shape[0], rb)]
        cols.append(jnp.concatenate(blocks, axis=0))
    return jnp.concatenate(cols, axis=1)


def _kernel(x_hbm, wqkv_hbm, wo_hbm, wr_hbm, wg_hbm, wu_hbm, wd_hbm, out_hbm,
            x_buf, xn_buf, wq_buf, wk_buf, wv_buf, wqt_buf, wo_buf, m_buf, wr_buf,
            g_acc, z_acc, zb_buf, xt_buf,
            wg_buf, wu_buf, wd_buf, xb_buf, hb_buf, y_acc, out_buf,
            sem, o_sem):

    def x_copy(i):
        if isinstance(i, int):
            rows = pl.ds(*_X_ROWS[i])
        else:
            rows = pl.ds(pl.multiple_of((i - 2) * TS, TS), TS)
        return pltpu.make_async_copy(x_hbm.at[rows, :], x_buf.at[rows, :], sem.at[_SEM_X + i])

    def wk_copy(s):
        c0, c1 = _WK_COLS[s]
        return pltpu.make_async_copy(wqkv_hbm.at[:, pl.ds(D + c0, c1 - c0)],
                                     wk_buf.at[:, pl.ds(c0, c1 - c0)], sem.at[_SEM_WK + s])

    def wq_copy(c):
        return pltpu.make_async_copy(wqkv_hbm.at[:, pl.ds(c * CW, CW)], wq_buf.at[c],
                                     sem.at[_SEM_WQ + c])

    wv_copy = pltpu.make_async_copy(wqkv_hbm.at[:, pl.ds(2 * D, D)], wv_buf.at[:, pl.ds(0, D)],
                                    sem.at[_SEM_WV])
    wo_copy = pltpu.make_async_copy(wo_hbm, wo_buf, sem.at[_SEM_WO])
    wr_copy = pltpu.make_async_copy(wr_hbm, wr_buf, sem.at[_SEM_WR])

    def ffn_copies(j):
        s = _SEM_F + 3 * j
        if isinstance(j, int):
            f0 = min(j * FPC, NFU - FPC) * FW
        else:
            f0 = pl.multiple_of(jnp.minimum(j * FPC, NFU - FPC) * FW, FW)
        fs = pl.ds(f0, FPC * FW)
        return (pltpu.make_async_copy(wg_hbm.at[:, fs], wg_buf.at[j], sem.at[s]),
                pltpu.make_async_copy(wu_hbm.at[:, fs], wu_buf.at[j], sem.at[s + 1]),
                pltpu.make_async_copy(wd_hbm.at[fs, :], wd_buf.at[j], sem.at[s + 2]))

    def out_copy(t, p):
        r0, nr, c0, nc = _OUT_PIECES[p]
        row = t * TS + r0
        rows = pl.ds(row if isinstance(t, int) else pl.multiple_of(row, 128), nr)
        cols = pl.ds(c0, nc)
        return pltpu.make_async_copy(out_buf.at[rows, cols], out_hbm.at[rows, cols],
                                     o_sem.at[t * len(_OUT_PIECES) + p])

    x_copy(0).start()
    x_copy(1).start()
    wk_copy(0).start()
    wr_copy.start()
    wk_copy(1).start()
    x_copy(2).start()
    wk_copy(2).start()
    wk_copy(3).start()
    for i in range(3, len(_X_ROWS)):
        x_copy(i).start()
    for c in range(NC):
        wq_copy(c).start()
    wv_copy.start()
    wo_copy.start()
    for j in range(NT - 1):
        for c in ffn_copies(j):
            c.start(priority=1)

    y_acc[...] = jnp.zeros_like(y_acc)
    hb_buf[...] = jnp.zeros_like(hb_buf)

    sub_iota = lax.broadcasted_iota(jnp.int32, (8, 128), 0)

    def route(xn, row0, best):
        nr = xn.shape[0]
        wr = wr_buf[...].reshape(1, D).astype(f32)
        r = _bf16_round(jnp.sum(xn.astype(f32) * wr, axis=-1, keepdims=True))
        r = jnp.broadcast_to(r, (nr, 128))
        for g in range(0, nr, 8):
            rg = r[g:g + 8, :]
            better = rg > best[0]
            best[0] = jnp.where(better, rg, best[0])
            best[1] = jnp.where(better, sub_iota + (row0 + g), best[1])

    def layernorm(src, dst, nr, best, after=None, never=None):
        x = x_buf[pl.ds(src, nr), :].astype(f32)
        x = _tie(x, after, never)
        mean = jnp.sum(x, axis=-1, keepdims=True) * (1.0 / D)
        mean_b = _bf16_round(mean)
        e = x - mean_b
        off = mean - mean_b
        var = jnp.sum(e * e, axis=-1, keepdims=True) * (1.0 / D) - off * off
        sd = _bf16_round(jnp.sqrt(_bf16_round(_bf16_round(var) + _LN_EPS)))
        rs = pl.reciprocal(sd, approx=True)
        rs = jnp.where(sd == jnp.inf, 0.0, rs * (2.0 - sd * rs))
        xf = _bf16_round(e) * rs
        xn = xf.astype(bf16)
        xn_buf[pl.ds(dst, nr), :] = xn
        if best is not None:
            route(xn, src, best)
        dep = None
        for g in range(0, nr, 8):
            dg = xf[g:g + 8, D - 128:]
            dep = dg if dep is None else dep + dg
        return dep, sd

    def ln_work(src, dst, nr, plan, best, never):
        sub, counts = plan
        assert sub * sum(counts) == nr
        o = 0
        for n in counts:
            dep = None
            for _ in range(n):
                dep = layernorm(src + o, dst + o, sub, best, dep, never)[0]
                o += sub
            yield dep

    def rows_of(r0, nr):
        got = []

        def get():
            if not got:
                got.append(xn_buf[pl.ds(r0, nr), :])
            return got[0]
        return get

    def kg_steps(jobs, work, never):
        def tied(val):
            return _tie(val, next(work, None), never, True)

        def k_part(xn, c0, cw, init):
            cols = slice(c0, c0 + cw)
            xn = xn()
            pk = _phi(tied(jnp.dot(xn, wk_buf[:, cols], preferred_element_type=f32)))
            zc = jnp.sum(pk.reshape(xn.shape[0] // 8, 8, cw), axis=0)
            z_acc[:, cols] = zc if init else z_acc[:, cols] + zc
            return pk.astype(bf16)

        def g_part(pk, xn, c0, cw, init):
            rows = slice(c0, c0 + cw)
            g = tied(lax.dot_general(pk, xn(), _TN, preferred_element_type=f32))
            g_acc[rows, :] = g if init else g_acc[rows, :] + g

        prev = None
        for job in jobs:
            if job is None:
                g_part(prev[0], *prev[1])
                prev = None
                continue
            pk = k_part(*job)
            if prev is not None:
                g_part(prev[0], *prev[1])
            prev = (pk, job)
        g_part(prev[0], *prev[1])
        assert next(work, None) is None

    best = [jnp.full((8, 128), -jnp.inf, f32), jnp.zeros((8, 128), jnp.int32)]
    x_copy(0).wait()
    sd0 = layernorm(0, 0, T0 // 2, None)[1]
    x_copy(1).wait()
    layernorm(T0 // 2, T0 // 2, T0 // 2, None)
    wk_copy(0).wait()
    never = jnp.min(sd0[0:8, :]) < 0.0
    kg_steps([(rows_of(0, T0 // 2), 0, 128, True), (rows_of(T0 // 2, T0 // 2), 0, 128, False)],
             iter(()), never)

    def route_first():
        yield None
        for r in range(0, T0, T0 // 2):
            route(xn_buf[r:r + T0 // 2, :], r, best)
            yield best[0]

    wr_copy.wait()
    wk_copy(1).wait()
    xa = rows_of(0, T0)
    kg_steps([(xa, 128, 128, True), (xa, 256, 128, True)], route_first(), never)

    x_copy(2).wait()
    wk_copy(2).wait()
    xa, xb = rows_of(0, T0), rows_of(T0, T0)
    kg_steps([(xa, 384, 128, True), (xa, 512, 128, True), None,
              (xb, 0, 128, False), (xb, 128, 128, False)],
             ln_work(T0, T0, T0, LN_C, best, never), never)

    wk_copy(3).wait()
    x_copy(3).wait()
    xa, xb = rows_of(0, TS), rows_of(T0, T0)
    kg_steps([(xb, 256, 256, False), (xb, 512, 128, False),
              (xa, 640, 128, True), (xa, 768, 256, True)],
             ln_work(TS, TS, TS, LN_D, best, never), never)
    for c in range(NC):
        wq_copy(c).wait()

    def phase1(i, carry):
        @pl.when(i + 1 < NT)
        def _():
            x_copy(i + 3).wait()

        best = list(carry)
        r0 = pl.multiple_of(i * TS, TS)
        src = pl.multiple_of(jnp.minimum(r0 + TS, S - TS), TS)
        dst = pl.multiple_of(r0 + TS, TS)
        wqt_buf[pl.ds(pl.multiple_of((i - 1) * CW, CW), CW), :] = wq_buf[i - 1].T
        xa = rows_of(r0, TS)
        kg_steps([(xa, c * CW, CW, False) for c in range(NC)],
                 ln_work(src, dst, TS, LN_LOOP, best, never), never)
        return tuple(best)

    best = lax.fori_loop(1, NT, phase1, tuple(best))

    wv_copy.wait()
    wo_copy.wait()
    rr = lax.broadcasted_iota(jnp.int32, (128, 128), 0) // DH
    cc = lax.broadcasted_iota(jnp.int32, (128, 128), 1) // DH
    same_head = rr == cc

    def kv_part(g):
        sl = slice(g * 128, (g + 1) * 128)
        kv = jnp.dot(g_acc[sl, :].astype(bf16), wv_buf[:, sl], preferred_element_type=f32)
        return jnp.where(same_head, kv, 0.0).astype(bf16)

    def m_part(g, kv):
        sl = slice(g * 128, (g + 1) * 128)
        m_buf[sl, :] = jnp.dot(kv, wo_buf[sl, :], preferred_element_type=f32).astype(bf16)

    rmax = jnp.max(best[0], axis=0, keepdims=True)
    idx = jnp.clip(jnp.min(jnp.where(best[0] == rmax, best[1], S)), 0, S - 1)
    gate = 1.0 / (1.0 + jnp.exp(-rmax[:, :1]))
    wqt_buf[D - CW:D, :] = wq_buf[NC - 1].T
    z = jnp.sum(z_acc[...], axis=0, keepdims=True)
    zb_buf[...] = jnp.broadcast_to(z, (128, D)).T
    r16 = pl.multiple_of((idx // 16) * 16, 16)
    blk = xn_buf[pl.ds(r16, 16), :].astype(f32)
    sel = lax.broadcasted_iota(jnp.int32, (16, D), 0) == (idx - r16)
    x_sel = jnp.sum(jnp.where(sel, blk, 0.0), axis=0, keepdims=True)
    xb_buf[...] = jnp.broadcast_to(x_sel, (128, D)).T

    for t in range(NT):
        xt_buf[t] = xn_buf[t * TS:t * TS + 128, :].T

    kv_prev = kv_part(0)
    for g in range(1, G128):
        kv = kv_part(g)
        m_part(g - 1, kv_prev)
        kv_prev = kv
    m_part(G128 - 1, kv_prev)

    def phase2(j, t_prev):
        @pl.when(j < NT - 1)
        def _():
            for c in ffn_copies(j):
                c.wait()

        t = (t_prev + 1) & (NT - 1)
        xn = xn_buf[pl.ds(pl.multiple_of(t * TS, TS), TS), :]
        j_up = jnp.minimum(j, NT - 2)
        j_dn = jnp.maximum(j - 1, 0)
        n_dup = FPC * (NT - 1) - NFU
        keep_dup = jnp.where(j >= NT - 2, 0.0, 1.0)
        late = []

        def matvec(w_ref, slot, nrows, cols, col_ref):
            acc = None
            for r in range(0, nrows, FFN_STEP):
                w = w_ref[slot, r:r + FFN_STEP, cols].astype(f32)
                p = w * jnp.concatenate([col_ref[r:r + FFN_STEP, :]] * (FW // 128), axis=1)
                for g in range(0, FFN_STEP, 8):
                    acc = p[g:g + 8, :] if acc is None else acc + p[g:g + 8, :]
                yield acc[:, :128] + acc[:, 128:]
            return acc

        def ffn_work():
            for e in range(D // FW):
                ec = slice(e * FW, (e + 1) * FW)
                acc = yield from matvec(wd_buf, j_dn, FPC * FW, ec, hb_buf)
                y_acc[:, ec] += acc
            for u in range(FPC):
                fs = slice(u * FW, (u + 1) * FW)
                g = yield from matvec(wg_buf, j_up, D, fs, xb_buf)
                a = yield from matvec(wu_buf, j_up, D, fs, xb_buf)
                g = jnp.sum(g, axis=0, keepdims=True)
                h = g * (1.0 / (1.0 + jnp.exp(-g))) * jnp.sum(a, axis=0, keepdims=True)
                if u < n_dup:
                    h = h * keep_dup
                hb = jnp.broadcast_to(h, (128, FW)).T
                hb_buf[fs, :] = hb
                late.append([FFN_LAG, hb[120:128, :] + hb[FW - 8:, :]])

        def with_late(gen):
            while True:
                dep = next(gen, None)
                if dep is None and not late:
                    return
                for e in late:
                    e[0] -= 1
                if late and late[0][0] <= 0:
                    d = late.pop(0)[1]
                    dep = d if dep is None else dep + d
                yield dep

        work = with_late(ffn_work())

        ps = []
        for c in range(NC):
            rows = slice(c * CW, (c + 1) * CW)
            if c == 0:
                q0 = jnp.dot(wqt_buf[rows, :], xt_buf[t], preferred_element_type=f32)
                qt = lax.dot_general(wqt_buf[rows, :], xn[128:], _NT, preferred_element_type=f32)
                qt = jnp.concatenate([q0, qt], axis=1)
            else:
                qt = lax.dot_general(wqt_buf[rows, :], xn, _NT, preferred_element_type=f32)
            pqt = _phi(_tie_tiles(qt, work, never, FFN_RB))
            zfull = jnp.concatenate([zb_buf[rows, :]] * (TS // 128), axis=1)
            hc = CW // DH
            den = jnp.sum((pqt * zfull).reshape(hc, DH, TS), axis=1, keepdims=True) + _EPS
            pt = pqt.reshape(hc, DH, TS) * pl.reciprocal(den, approx=True)
            ps.append(pt.reshape(CW, TS).astype(bf16).T)
        p = jnp.concatenate(ps, axis=1)
        assert NC * (CW // FFN_RB) * (TS // 128) > (D // FW) * (FPC * FW // FFN_STEP)
        y = jnp.sum(y_acc[...], axis=0, keepdims=True) * gate
        for n, (r0, nr, c0, nc) in enumerate(_OUT_PIECES):
            cols = slice(c0, c0 + nc)
            rows = pl.ds(pl.multiple_of(t * TS + r0, 128), nr)
            o = jnp.dot(p[r0:r0 + nr, :], m_buf[:, cols], preferred_element_type=f32)
            o = _tie_tiles(o, work, never, FFN_RB)
            o = o + x_buf[rows, cols].astype(f32) + xn_buf[rows, cols].astype(f32)
            hit = lax.broadcasted_iota(jnp.int32, (nr, nc), 0) == idx - (t * TS + r0)
            out_buf[rows, cols] = (o + jnp.where(hit, y[:, cols], 0.0)).astype(bf16)
            out_copy(t, n).start()
        assert next(work, 0) == 0
        return t

    lax.fori_loop(0, NT, phase2, idx // TS)
    for t in range(NT):
        for n in range(len(_OUT_PIECES)):
            out_copy(t, n).wait()


@jax.jit
def pallas_parallel_sum__linear_attn_block__moe_arch_mod__prompt_kernel(
    A_x: jax.Array,
    A_wqkv: jax.Array,
    A_wo: jax.Array,
    B_x: jax.Array,
    B_w_r: jax.Array,
    B_w_gate: jax.Array,
    B_w_up: jax.Array,
    B_w_down: jax.Array,
):
    any_spec = pl.BlockSpec(memory_space=pl.ANY)
    out = pl.pallas_call(
        _kernel,
        out_shape=jax.ShapeDtypeStruct((S, D), bf16),
        in_specs=[any_spec] * 7,
        out_specs=any_spec,
        scratch_shapes=[
            pltpu.VMEM((S, D), bf16),
            pltpu.VMEM((S + TS, D), bf16),
            pltpu.VMEM((NC, D, CW), bf16),
            pltpu.VMEM((D, D + 128), bf16),
            pltpu.VMEM((D, D + 128), bf16),
            pltpu.VMEM((D, D), bf16),
            pltpu.VMEM((D, D), bf16),
            pltpu.VMEM((D, D), bf16),
            pltpu.VMEM((D,), bf16),
            pltpu.VMEM((D, D), f32),
            pltpu.VMEM((8, D), f32),
            pltpu.VMEM((D, 128), f32),
            pltpu.VMEM((NT, D, 128), bf16),
            pltpu.VMEM((NT - 1, D, FPC * FW), bf16),
            pltpu.VMEM((NT - 1, D, FPC * FW), bf16),
            pltpu.VMEM((NT - 1, FPC * FW, D), bf16),
            pltpu.VMEM((D, 128), f32),
            pltpu.VMEM((FPC * FW, 128), f32),
            pltpu.VMEM((8, D), f32),
            pltpu.VMEM((S, D), bf16),
            pltpu.SemaphoreType.DMA((_N_SEM,)),
            pltpu.SemaphoreType.DMA((NT * len(_OUT_PIECES),)),
        ],
        compiler_params=pltpu.CompilerParams(vmem_limit_bytes=100 * 1024 * 1024,
                                             disable_semaphore_checks=True),
        name="linattn_mod",
    )(A_x.reshape(S, D), A_wqkv, A_wo, B_w_r, B_w_gate, B_w_up, B_w_down)
    return out.reshape(1, S, D)
```

```python
import jax
import jax.numpy as jnp
from jax import lax
import jax.experimental.pallas as pl
import jax.experimental.pallas.tpu as pltpu

S = 2048
D = 1024
F = 3584
H = 32
DH = D // H
G128 = D // 128
CW = 256
NC = D // CW
T0 = 256
TS = 512
NT = S // TS
FW = 256
NFU = F // FW
FPC = -(-NFU // (NT - 1))

FFN_STEP = 64
FFN_RB = 32
FFN_LAG = 8
LN_C = (32, (0, 0, 6, 2))
LN_D = (16, (0, 0, 8, 0, 0, 17, 7))
LN_LOOP = (16, (9, 8, 0, 8, 0, 7))

_LN_EPS = 1.0013580322265625e-05
_EPS = 1e-6

f32 = jnp.float32
bf16 = jnp.bfloat16

_OUT_PIECES = [(0, TS, c * CW, CW) for c in range(NC - 1)] + [
    (0, 384, D - CW, CW), (384, 128, D - CW, CW)]

_X_ROWS = [(0, T0 // 2), (T0 // 2, T0 // 2), (T0, T0)] + [(i * TS, TS) for i in range(1, NT)]
_WK_COLS = ((0, 128), (128, 384), (384, 640), (640, 1024))
_SEM_X = 0
_SEM_WK = _SEM_X + len(_X_ROWS)
_SEM_WQ = _SEM_WK + len(_WK_COLS)
_SEM_WV = _SEM_WQ + NC
_SEM_WO = _SEM_WV + 1
_SEM_WR = _SEM_WO + 1
_SEM_F = _SEM_WR + 1
_N_SEM = _SEM_F + 3 * (NT - 1)

_TN = (((0,), (0,)), ((), ()))
_NT = (((1,), (1,)), ((), ()))


def _bf16_round(v):
    return v.astype(bf16).astype(f32)


def _phi(t):
    return jnp.where(t > 0, t + 1.0, jnp.exp(t)) + _EPS


def _tie(val, dep, never, last=False):
    if dep is None:
        return val
    if last:
        tail = jnp.where(never, dep, val[-8:, -128:])
        if val.shape[1] > 128:
            tail = jnp.concatenate([val[-8:, :-128], tail], axis=1)
        return jnp.concatenate([val[:-8, :], tail], axis=0)
    head = jnp.where(never, dep, val[:8, :128])
    head = jnp.concatenate([head, val[:8, 128:]], axis=1)
    return jnp.concatenate([head, val[8:, :]], axis=0)


def _tie_tiles(val, deps, never, rb):
    cols = []
    for n in range(val.shape[1] // 128):
        blocks = [_tie(val[r:r + rb, n * 128:(n + 1) * 128], next(deps, None), never, True)
                  for r in range(0, val.shape[0], rb)]
        cols.append(jnp.concatenate(blocks, axis=0))
    return jnp.concatenate(cols, axis=1)


def _kernel(*refs):
    pl.when(pl.program_id(0) == 0)(lambda: _body(*refs))


def _body(x_hbm, wqkv_hbm, wo_hbm, wr_hbm, wg_hbm, wu_hbm, wd_hbm, out_hbm,
          x_buf, xn_buf, wq_buf, wk_buf, wv_buf, wqt_buf, wo_buf, m_buf, wr_buf,
          g_acc, z_acc, zb_buf, xt_buf,
          wg_buf, wu_buf, wd_buf, xb_buf, hb_buf, y_acc, out_buf,
          sem, o_sem):

    def x_copy(i):
        if isinstance(i, int):
            rows = pl.ds(*_X_ROWS[i])
        else:
            rows = pl.ds(pl.multiple_of((i - 2) * TS, TS), TS)
        return pltpu.make_async_copy(x_hbm.at[rows, :], x_buf.at[rows, :], sem.at[_SEM_X + i])

    def wk_copy(s):
        c0, c1 = _WK_COLS[s]
        return pltpu.make_async_copy(wqkv_hbm.at[:, pl.ds(D + c0, c1 - c0)],
                                     wk_buf.at[:, pl.ds(c0, c1 - c0)], sem.at[_SEM_WK + s])

    def wq_copy(c):
        return pltpu.make_async_copy(wqkv_hbm.at[:, pl.ds(c * CW, CW)], wq_buf.at[c],
                                     sem.at[_SEM_WQ + c])

    wv_copy = pltpu.make_async_copy(wqkv_hbm.at[:, pl.ds(2 * D, D)], wv_buf.at[:, pl.ds(0, D)],
                                    sem.at[_SEM_WV])
    wo_copy = pltpu.make_async_copy(wo_hbm, wo_buf, sem.at[_SEM_WO])
    wr_copy = pltpu.make_async_copy(wr_hbm, wr_buf, sem.at[_SEM_WR])

    def ffn_copies(j):
        s = _SEM_F + 3 * j
        if isinstance(j, int):
            f0 = min(j * FPC, NFU - FPC) * FW
        else:
            f0 = pl.multiple_of(jnp.minimum(j * FPC, NFU - FPC) * FW, FW)
        fs = pl.ds(f0, FPC * FW)
        return (pltpu.make_async_copy(wg_hbm.at[:, fs], wg_buf.at[j], sem.at[s]),
                pltpu.make_async_copy(wu_hbm.at[:, fs], wu_buf.at[j], sem.at[s + 1]),
                pltpu.make_async_copy(wd_hbm.at[fs, :], wd_buf.at[j], sem.at[s + 2]))

    def out_copy(t, p):
        r0, nr, c0, nc = _OUT_PIECES[p]
        row = t * TS + r0
        rows = pl.ds(row if isinstance(t, int) else pl.multiple_of(row, 128), nr)
        cols = pl.ds(c0, nc)
        return pltpu.make_async_copy(out_buf.at[rows, cols], out_hbm.at[rows, cols],
                                     o_sem.at[t * len(_OUT_PIECES) + p])

    x_copy(0).start()
    x_copy(1).start()
    wk_copy(0).start()
    wr_copy.start()
    wk_copy(1).start()
    x_copy(2).start()
    wk_copy(2).start()
    wk_copy(3).start()
    for i in range(3, len(_X_ROWS)):
        x_copy(i).start()
    for c in range(NC):
        wq_copy(c).start()
    wv_copy.start()
    wo_copy.start()
    for j in range(NT - 1):
        for c in ffn_copies(j):
            c.start(priority=1)

    y_acc[...] = jnp.zeros_like(y_acc)
    hb_buf[...] = jnp.zeros_like(hb_buf)

    sub_iota = lax.broadcasted_iota(jnp.int32, (8, 128), 0)

    def route(xn, row0, best):
        nr = xn.shape[0]
        wr = wr_buf[...].reshape(1, D).astype(f32)
        r = _bf16_round(jnp.sum(xn.astype(f32) * wr, axis=-1, keepdims=True))
        r = jnp.broadcast_to(r, (nr, 128))
        for g in range(0, nr, 8):
            rg = r[g:g + 8, :]
            better = rg > best[0]
            best[0] = jnp.where(better, rg, best[0])
            best[1] = jnp.where(better, sub_iota + (row0 + g), best[1])

    def layernorm(src, dst, nr, best, after=None, never=None):
        x = x_buf[pl.ds(src, nr), :].astype(f32)
        x = _tie(x, after, never)
        mean = jnp.sum(x, axis=-1, keepdims=True) * (1.0 / D)
        mean_b = _bf16_round(mean)
        e = x - mean_b
        off = mean - mean_b
        var = jnp.sum(e * e, axis=-1, keepdims=True) * (1.0 / D) - off * off
        sd = _bf16_round(jnp.sqrt(_bf16_round(_bf16_round(var) + _LN_EPS)))
        rs = pl.reciprocal(sd, approx=True)
        rs = jnp.where(sd == jnp.inf, 0.0, rs * (2.0 - sd * rs))
        xf = _bf16_round(e) * rs
        xn = xf.astype(bf16)
        xn_buf[pl.ds(dst, nr), :] = xn
        if best is not None:
            route(xn, src, best)
        dep = None
        for g in range(0, nr, 8):
            dg = xf[g:g + 8, D - 128:]
            dep = dg if dep is None else dep + dg
        return dep, sd

    def ln_work(src, dst, nr, plan, best, never):
        sub, counts = plan
        assert sub * sum(counts) == nr
        o = 0
        for n in counts:
            dep = None
            for _ in range(n):
                dep = layernorm(src + o, dst + o, sub, best, dep, never)[0]
                o += sub
            yield dep

    def rows_of(r0, nr):
        got = []

        def get():
            if not got:
                got.append(xn_buf[pl.ds(r0, nr), :])
            return got[0]
        return get

    def kg_steps(jobs, work, never):
        def tied(val):
            return _tie(val, next(work, None), never, True)

        def k_part(xn, c0, cw, init):
            cols = slice(c0, c0 + cw)
            xn = xn()
            pk = _phi(tied(jnp.dot(xn, wk_buf[:, cols], preferred_element_type=f32)))
            zc = jnp.sum(pk.reshape(xn.shape[0] // 8, 8, cw), axis=0)
            z_acc[:, cols] = zc if init else z_acc[:, cols] + zc
            return pk.astype(bf16)

        def g_part(pk, xn, c0, cw, init):
            rows = slice(c0, c0 + cw)
            g = tied(lax.dot_general(pk, xn(), _TN, preferred_element_type=f32))
            g_acc[rows, :] = g if init else g_acc[rows, :] + g

        prev = None
        for job in jobs:
            if job is None:
                g_part(prev[0], *prev[1])
                prev = None
                continue
            pk = k_part(*job)
            if prev is not None:
                g_part(prev[0], *prev[1])
            prev = (pk, job)
        g_part(prev[0], *prev[1])
        assert next(work, None) is None

    best = [jnp.full((8, 128), -jnp.inf, f32), jnp.zeros((8, 128), jnp.int32)]
    x_copy(0).wait()
    sd0 = layernorm(0, 0, T0 // 2, None)[1]
    x_copy(1).wait()
    layernorm(T0 // 2, T0 // 2, T0 // 2, None)
    wk_copy(0).wait()
    never = jnp.min(sd0[0:8, :]) < 0.0
    kg_steps([(rows_of(0, T0 // 2), 0, 128, True), (rows_of(T0 // 2, T0 // 2), 0, 128, False)],
             iter(()), never)

    def route_first():
        yield None
        for r in range(0, T0, T0 // 2):
            route(xn_buf[r:r + T0 // 2, :], r, best)
            yield best[0]

    wr_copy.wait()
    wk_copy(1).wait()
    xa = rows_of(0, T0)
    kg_steps([(xa, 128, 128, True), (xa, 256, 128, True)], route_first(), never)

    x_copy(2).wait()
    wk_copy(2).wait()
    xa, xb = rows_of(0, T0), rows_of(T0, T0)
    kg_steps([(xa, 384, 128, True), (xa, 512, 128, True), None,
              (xb, 0, 128, False), (xb, 128, 128, False)],
             ln_work(T0, T0, T0, LN_C, best, never), never)

    wk_copy(3).wait()
    x_copy(3).wait()
    xa, xb = rows_of(0, TS), rows_of(T0, T0)
    kg_steps([(xb, 256, 256, False), (xb, 512, 128, False),
              (xa, 640, 128, True), (xa, 768, 256, True)],
             ln_work(TS, TS, TS, LN_D, best, never), never)
    for c in range(NC):
        wq_copy(c).wait()

    def phase1(i, carry):
        @pl.when(i + 1 < NT)
        def _():
            x_copy(i + 3).wait()

        best = list(carry)
        r0 = pl.multiple_of(i * TS, TS)
        src = pl.multiple_of(jnp.minimum(r0 + TS, S - TS), TS)
        dst = pl.multiple_of(r0 + TS, TS)
        wqt_buf[pl.ds(pl.multiple_of((i - 1) * CW, CW), CW), :] = wq_buf[i - 1].T
        xa = rows_of(r0, TS)
        kg_steps([(xa, c * CW, CW, False) for c in range(NC)],
                 ln_work(src, dst, TS, LN_LOOP, best, never), never)
        return tuple(best)

    best = lax.fori_loop(1, NT, phase1, tuple(best))

    wv_copy.wait()
    wo_copy.wait()
    rr = lax.broadcasted_iota(jnp.int32, (128, 128), 0) // DH
    cc = lax.broadcasted_iota(jnp.int32, (128, 128), 1) // DH
    same_head = rr == cc

    def kv_part(g):
        sl = slice(g * 128, (g + 1) * 128)
        kv = jnp.dot(g_acc[sl, :].astype(bf16), wv_buf[:, sl], preferred_element_type=f32)
        return jnp.where(same_head, kv, 0.0).astype(bf16)

    def m_part(g, kv):
        sl = slice(g * 128, (g + 1) * 128)
        m_buf[sl, :] = jnp.dot(kv, wo_buf[sl, :], preferred_element_type=f32).astype(bf16)

    rmax = jnp.max(best[0], axis=0, keepdims=True)
    idx = jnp.clip(jnp.min(jnp.where(best[0] == rmax, best[1], S)), 0, S - 1)
    gate = 1.0 / (1.0 + jnp.exp(-rmax[:, :1]))
    wqt_buf[D - CW:D, :] = wq_buf[NC - 1].T
    z = jnp.sum(z_acc[...], axis=0, keepdims=True)
    zb_buf[...] = jnp.broadcast_to(z, (128, D)).T
    r16 = pl.multiple_of((idx // 16) * 16, 16)
    blk = xn_buf[pl.ds(r16, 16), :].astype(f32)
    sel = lax.broadcasted_iota(jnp.int32, (16, D), 0) == (idx - r16)
    x_sel = jnp.sum(jnp.where(sel, blk, 0.0), axis=0, keepdims=True)
    xb_buf[...] = jnp.broadcast_to(x_sel, (128, D)).T

    for t in range(NT):
        xt_buf[t] = xn_buf[t * TS:t * TS + 128, :].T

    kv_prev = kv_part(0)
    for g in range(1, G128):
        kv = kv_part(g)
        m_part(g - 1, kv_prev)
        kv_prev = kv
    m_part(G128 - 1, kv_prev)

    def phase2(j, t_prev):
        @pl.when(j < NT - 1)
        def _():
            for c in ffn_copies(j):
                c.wait()

        t = (t_prev + 1) & (NT - 1)
        xn = xn_buf[pl.ds(pl.multiple_of(t * TS, TS), TS), :]
        j_up = jnp.minimum(j, NT - 2)
        j_dn = jnp.maximum(j - 1, 0)
        n_dup = FPC * (NT - 1) - NFU
        keep_dup = jnp.where(j >= NT - 2, 0.0, 1.0)
        late = []

        def matvec(w_ref, slot, nrows, cols, col_ref):
            acc = None
            for r in range(0, nrows, FFN_STEP):
                w = w_ref[slot, r:r + FFN_STEP, cols].astype(f32)
                p = w * jnp.concatenate([col_ref[r:r + FFN_STEP, :]] * (FW // 128), axis=1)
                for g in range(0, FFN_STEP, 8):
                    acc = p[g:g + 8, :] if acc is None else acc + p[g:g + 8, :]
                yield acc[:, :128] + acc[:, 128:]
            return acc

        def ffn_work():
            for e in range(D // FW):
                ec = slice(e * FW, (e + 1) * FW)
                acc = yield from matvec(wd_buf, j_dn, FPC * FW, ec, hb_buf)
                y_acc[:, ec] += acc
            for u in range(FPC):
                fs = slice(u * FW, (u + 1) * FW)
                g = yield from matvec(wg_buf, j_up, D, fs, xb_buf)
                a = yield from matvec(wu_buf, j_up, D, fs, xb_buf)
                g = jnp.sum(g, axis=0, keepdims=True)
                h = g * (1.0 / (1.0 + jnp.exp(-g))) * jnp.sum(a, axis=0, keepdims=True)
                if u < n_dup:
                    h = h * keep_dup
                hb = jnp.broadcast_to(h, (128, FW)).T
                hb_buf[fs, :] = hb
                late.append([FFN_LAG, hb[120:128, :] + hb[FW - 8:, :]])

        def with_late(gen):
            while True:
                dep = next(gen, None)
                if dep is None and not late:
                    return
                for e in late:
                    e[0] -= 1
                if late and late[0][0] <= 0:
                    d = late.pop(0)[1]
                    dep = d if dep is None else dep + d
                yield dep

        work = with_late(ffn_work())

        ps = []
        for c in range(NC):
            rows = slice(c * CW, (c + 1) * CW)
            if c == 0:
                q0 = jnp.dot(wqt_buf[rows, :], xt_buf[t], preferred_element_type=f32)
                qt = lax.dot_general(wqt_buf[rows, :], xn[128:], _NT, preferred_element_type=f32)
                qt = jnp.concatenate([q0, qt], axis=1)
            else:
                qt = lax.dot_general(wqt_buf[rows, :], xn, _NT, preferred_element_type=f32)
            pqt = _phi(_tie_tiles(qt, work, never, FFN_RB))
            zfull = jnp.concatenate([zb_buf[rows, :]] * (TS // 128), axis=1)
            hc = CW // DH
            den = jnp.sum((pqt * zfull).reshape(hc, DH, TS), axis=1, keepdims=True) + _EPS
            pt = pqt.reshape(hc, DH, TS) * pl.reciprocal(den, approx=True)
            ps.append(pt.reshape(CW, TS).astype(bf16).T)
        p = jnp.concatenate(ps, axis=1)
        assert NC * (CW // FFN_RB) * (TS // 128) > (D // FW) * (FPC * FW // FFN_STEP)
        y = jnp.sum(y_acc[...], axis=0, keepdims=True) * gate
        for n, (r0, nr, c0, nc) in enumerate(_OUT_PIECES):
            cols = slice(c0, c0 + nc)
            rows = pl.ds(pl.multiple_of(t * TS + r0, 128), nr)
            o = jnp.dot(p[r0:r0 + nr, :], m_buf[:, cols], preferred_element_type=f32)
            o = _tie_tiles(o, work, never, FFN_RB)
            o = o + x_buf[rows, cols].astype(f32) + xn_buf[rows, cols].astype(f32)
            hit = lax.broadcasted_iota(jnp.int32, (nr, nc), 0) == idx - (t * TS + r0)
            out_buf[rows, cols] = (o + jnp.where(hit, y[:, cols], 0.0)).astype(bf16)
            out_copy(t, n).start()
        assert next(work, 0) == 0
        return t

    lax.fori_loop(0, NT, phase2, idx // TS)
    for t in range(NT):
        for n in range(len(_OUT_PIECES)):
            out_copy(t, n).wait()


@jax.jit
def pallas_parallel_sum__linear_attn_block__moe_arch_mod__prompt_kernel(
    A_x: jax.Array,
    A_wqkv: jax.Array,
    A_wo: jax.Array,
    B_x: jax.Array,
    B_w_r: jax.Array,
    B_w_gate: jax.Array,
    B_w_up: jax.Array,
    B_w_down: jax.Array,
):
    any_spec = pl.BlockSpec(memory_space=pl.ANY)
    out = pl.pallas_call(
        _kernel,
        out_shape=jax.ShapeDtypeStruct((S, D), bf16),
        grid=(2,),
        in_specs=[any_spec] * 7,
        out_specs=any_spec,
        scratch_shapes=[
            pltpu.VMEM((S, D), bf16),
            pltpu.VMEM((S + TS, D), bf16),
            pltpu.VMEM((NC, D, CW), bf16),
            pltpu.VMEM((D, D + 128), bf16),
            pltpu.VMEM((D, D + 128), bf16),
            pltpu.VMEM((D, D), bf16),
            pltpu.VMEM((D, D), bf16),
            pltpu.VMEM((D, D), bf16),
            pltpu.VMEM((D,), bf16),
            pltpu.VMEM((D, D), f32),
            pltpu.VMEM((8, D), f32),
            pltpu.VMEM((D, 128), f32),
            pltpu.VMEM((NT, D, 128), bf16),
            pltpu.VMEM((NT - 1, D, FPC * FW), bf16),
            pltpu.VMEM((NT - 1, D, FPC * FW), bf16),
            pltpu.VMEM((NT - 1, FPC * FW, D), bf16),
            pltpu.VMEM((D, 128), f32),
            pltpu.VMEM((FPC * FW, 128), f32),
            pltpu.VMEM((8, D), f32),
            pltpu.VMEM((S, D), bf16),
            pltpu.SemaphoreType.DMA((_N_SEM,)),
            pltpu.SemaphoreType.DMA((NT * len(_OUT_PIECES),)),
        ],
        compiler_params=pltpu.CompilerParams(dimension_semantics=("arbitrary",),
                                             vmem_limit_bytes=100 * 1024 * 1024,
                                             disable_semaphore_checks=True),
        name="linattn_mod",
    )(A_x.reshape(S, D), A_wqkv, A_wo, B_w_r, B_w_gate, B_w_up, B_w_down)
    return out.reshape(1, S, D)
```

```python
import itertools

import jax
import jax.numpy as jnp
from jax import lax
import jax.experimental.pallas as pl
import jax.experimental.pallas.tpu as pltpu

S = 2048
D = 1024
F = 3584
H = 32
DH = D // H
G128 = D // 128
CW = 256
NC = D // CW
T0 = 256
TS = 512
NT = S // TS
T1 = TS + T0
N1 = (S - TS) // T1
FW = 256
NFU = F // FW
FPC = -(-NFU // (NT - 1))

FFN_STEP = 64
FFN_RB = 32
FFN_LAG = 8
LN_C = (32, (0, 0, 6, 2))
LN_D = (16, (0, 0, 8, 0, 0, 17, 7))
LN_OWN = (16, (8, 8, 0))
LN_NEXT = (16, (0, 0, 17, 0, 15))

_LN_EPS = 1.0013580322265625e-05
_EPS = 1e-6

f32 = jnp.float32
bf16 = jnp.bfloat16

_OUT_PIECES = [(0, TS, c * CW, CW) for c in range(NC - 1)] + [
    (0, 384, D - CW, CW), (384, 128, D - CW, CW)]

_X_ROWS = [(0, T0 // 2), (T0 // 2, T0 // 2), (T0, T0), (TS, TS),
           (2 * TS, T0), (2 * TS + T0, TS), (S - T0, T0)]
_WK_COLS = ((0, 128), (128, 384), (384, 640), (640, 1024))
_SEM_X = 0
_SEM_WK = _SEM_X + len(_X_ROWS)
_SEM_WQ = _SEM_WK + len(_WK_COLS)
_SEM_WV = _SEM_WQ + NC
_SEM_WO = _SEM_WV + 1
_SEM_WR = _SEM_WO + 1
_SEM_F = _SEM_WR + 1
_N_SEM = _SEM_F + 3 * (NT - 1)

_TN = (((0,), (0,)), ((), ()))
_NT = (((1,), (1,)), ((), ()))


def _bf16_round(v):
    return v.astype(bf16).astype(f32)


def _phi(t):
    return jnp.where(t > 0, t + 1.0, jnp.exp(t)) + _EPS


def _tie(val, dep, never, last=False):
    if dep is None:
        return val
    if last:
        tail = jnp.where(never, dep, val[-8:, -128:])
        if val.shape[1] > 128:
            tail = jnp.concatenate([val[-8:, :-128], tail], axis=1)
        return jnp.concatenate([val[:-8, :], tail], axis=0)
    head = jnp.where(never, dep, val[:8, :128])
    head = jnp.concatenate([head, val[:8, 128:]], axis=1)
    return jnp.concatenate([head, val[8:, :]], axis=0)


def _tie_tiles(val, deps, never, rb):
    cols = []
    for n in range(val.shape[1] // 128):
        blocks = [_tie(val[r:r + rb, n * 128:(n + 1) * 128], next(deps, None), never, True)
                  for r in range(0, val.shape[0], rb)]
        cols.append(jnp.concatenate(blocks, axis=0))
    return jnp.concatenate(cols, axis=1)


def _kernel(*refs):
    pl.when(pl.program_id(0) == 0)(lambda: _body(*refs))


def _body(x_hbm, wqkv_hbm, wo_hbm, wr_hbm, wg_hbm, wu_hbm, wd_hbm, out_hbm,
          x_buf, xn_buf, wq_buf, wk_buf, wv_buf, wqt_buf, wo_buf, m_buf, wr_buf,
          g_acc, z_acc, zb_buf, xt_buf,
          wg_buf, wu_buf, wd_buf, xb_buf, hb_buf, y_acc, out_buf,
          sem, o_sem):

    def x_copy(i):
        if isinstance(i, int):
            rows = pl.ds(*_X_ROWS[i])
        else:
            rows = pl.ds(pl.multiple_of(2 * TS + (i - 4) // 2 * T1, 128), T0)
        return pltpu.make_async_copy(x_hbm.at[rows, :], x_buf.at[rows, :], sem.at[_SEM_X + i])

    def wk_copy(s):
        c0, c1 = _WK_COLS[s]
        return pltpu.make_async_copy(wqkv_hbm.at[:, pl.ds(D + c0, c1 - c0)],
                                     wk_buf.at[:, pl.ds(c0, c1 - c0)], sem.at[_SEM_WK + s])

    def wq_copy(c):
        return pltpu.make_async_copy(wqkv_hbm.at[:, pl.ds(c * CW, CW)], wq_buf.at[c],
                                     sem.at[_SEM_WQ + c])

    wv_copy = pltpu.make_async_copy(wqkv_hbm.at[:, pl.ds(2 * D, D)], wv_buf.at[:, pl.ds(0, D)],
                                    sem.at[_SEM_WV])
    wo_copy = pltpu.make_async_copy(wo_hbm, wo_buf, sem.at[_SEM_WO])
    wr_copy = pltpu.make_async_copy(wr_hbm, wr_buf, sem.at[_SEM_WR])

    def ffn_copies(j):
        s = _SEM_F + 3 * j
        if isinstance(j, int):
            f0 = min(j * FPC, NFU - FPC) * FW
        else:
            f0 = pl.multiple_of(jnp.minimum(j * FPC, NFU - FPC) * FW, FW)
        fs = pl.ds(f0, FPC * FW)
        return (pltpu.make_async_copy(wg_hbm.at[:, fs], wg_buf.at[j], sem.at[s]),
                pltpu.make_async_copy(wu_hbm.at[:, fs], wu_buf.at[j], sem.at[s + 1]),
                pltpu.make_async_copy(wd_hbm.at[fs, :], wd_buf.at[j], sem.at[s + 2]))

    def out_copy(t, p):
        r0, nr, c0, nc = _OUT_PIECES[p]
        row = t * TS + r0
        rows = pl.ds(row if isinstance(t, int) else pl.multiple_of(row, 128), nr)
        cols = pl.ds(c0, nc)
        return pltpu.make_async_copy(out_buf.at[rows, cols], out_hbm.at[rows, cols],
                                     o_sem.at[t * len(_OUT_PIECES) + p])

    x_copy(0).start()
    x_copy(1).start()
    wk_copy(0).start()
    wr_copy.start()
    wk_copy(1).start()
    x_copy(2).start()
    wk_copy(2).start()
    wk_copy(3).start()
    for i in range(3, len(_X_ROWS)):
        x_copy(i).start()
    for c in range(NC):
        wq_copy(c).start()
    wv_copy.start()
    wo_copy.start()
    for j in range(NT - 1):
        for c in ffn_copies(j):
            c.start(priority=1)

    y_acc[...] = jnp.zeros_like(y_acc)
    hb_buf[...] = jnp.zeros_like(hb_buf)

    sub_iota = lax.broadcasted_iota(jnp.int32, (8, 128), 0)

    def route(xn, row0, best):
        nr = xn.shape[0]
        wr = wr_buf[...].reshape(1, D).astype(f32)
        r = _bf16_round(jnp.sum(xn.astype(f32) * wr, axis=-1, keepdims=True))
        r = jnp.broadcast_to(r, (nr, 128))
        for g in range(0, nr, 8):
            rg = r[g:g + 8, :]
            better = rg > best[0]
            best[0] = jnp.where(better, rg, best[0])
            best[1] = jnp.where(better, sub_iota + (row0 + g), best[1])

    def layernorm(src, dst, nr, best, after=None, never=None):
        x = x_buf[pl.ds(src, nr), :].astype(f32)
        x = _tie(x, after, never)
        mean = jnp.sum(x, axis=-1, keepdims=True) * (1.0 / D)
        mean_b = _bf16_round(mean)
        e = x - mean_b
        off = mean - mean_b
        var = jnp.sum(e * e, axis=-1, keepdims=True) * (1.0 / D) - off * off
        sd = _bf16_round(jnp.sqrt(_bf16_round(_bf16_round(var) + _LN_EPS)))
        rs = pl.reciprocal(sd, approx=True)
        rs = jnp.where(sd == jnp.inf, 0.0, rs * (2.0 - sd * rs))
        xf = _bf16_round(e) * rs
        xn = xf.astype(bf16)
        xn_buf[pl.ds(dst, nr), :] = xn
        if best is not None:
            route(xn, src, best)
        dep = None
        for g in range(0, nr, 8):
            dg = xf[g:g + 8, D - 128:]
            dep = dg if dep is None else dep + dg
        return dep, sd

    def ln_work(src, dst, nr, plan, best, never):
        sub, counts = plan
        assert sub * sum(counts) == nr
        o = 0
        for n in counts:
            dep = None
            for _ in range(n):
                dep = layernorm(src + o, dst + o, sub, best, dep, never)[0]
                o += sub
            yield dep

    def rows_of(r0, nr):
        got = []

        def get():
            if not got:
                got.append(xn_buf[pl.ds(r0, nr), :])
            return got[0]
        return get

    def kg_steps(jobs, work, never):
        def tied(val):
            return _tie(val, next(work, None), never, True)

        def k_part(xn, c0, cw, init):
            cols = slice(c0, c0 + cw)
            xn = xn()
            pk = _phi(tied(jnp.dot(xn, wk_buf[:, cols], preferred_element_type=f32)))
            zc = jnp.sum(pk.reshape(xn.shape[0] // 8, 8, cw), axis=0)
            z_acc[:, cols] = zc if init else z_acc[:, cols] + zc
            return pk.astype(bf16)

        def g_part(pk, xn, c0, cw, init):
            rows = slice(c0, c0 + cw)
            g = tied(lax.dot_general(pk, xn(), _TN, preferred_element_type=f32))
            g_acc[rows, :] = g if init else g_acc[rows, :] + g

        prev = None
        for job in jobs:
            if job is None:
                g_part(prev[0], *prev[1])
                prev = None
                continue
            pk = k_part(*job)
            if prev is not None:
                g_part(prev[0], *prev[1])
            prev = (pk, job)
        g_part(prev[0], *prev[1])
        assert next(work, None) is None

    best = [jnp.full((8, 128), -jnp.inf, f32), jnp.zeros((8, 128), jnp.int32)]
    x_copy(0).wait()
    sd0 = layernorm(0, 0, T0 // 2, None)[1]
    x_copy(1).wait()
    layernorm(T0 // 2, T0 // 2, T0 // 2, None)
    wk_copy(0).wait()
    never = jnp.min(sd0[0:8, :]) < 0.0
    kg_steps([(rows_of(0, T0 // 2), 0, 128, True), (rows_of(T0 // 2, T0 // 2), 0, 128, False)],
             iter(()), never)

    def route_first():
        yield None
        for r in range(0, T0, T0 // 2):
            route(xn_buf[r:r + T0 // 2, :], r, best)
            yield best[0]

    wr_copy.wait()
    wk_copy(1).wait()
    xa = rows_of(0, T0)
    kg_steps([(xa, 128, 128, True), (xa, 256, 128, True)], route_first(), never)

    x_copy(2).wait()
    wk_copy(2).wait()
    xa, xb = rows_of(0, T0), rows_of(T0, T0)
    kg_steps([(xa, 384, 128, True), (xa, 512, 128, True), None,
              (xb, 0, 128, False), (xb, 128, 128, False)],
             ln_work(T0, T0, T0, LN_C, best, never), never)

    wk_copy(3).wait()
    x_copy(3).wait()
    xa, xb = rows_of(0, TS), rows_of(T0, T0)
    kg_steps([(xb, 256, 256, False), (xb, 512, 128, False),
              (xa, 640, 128, True), (xa, 768, 256, True)],
             ln_work(TS, TS, TS, LN_D, best, never), never)
    for c in range(NC):
        wq_copy(c).wait()

    def phase1(i, carry):
        x_copy(2 * i + 4).wait()

        @pl.when(i == 0)
        def _():
            x_copy(5).wait()

        best = list(carry)
        r0 = pl.multiple_of(TS + i * T1, 128)
        src = pl.multiple_of(jnp.minimum(r0 + T1, S - TS), 128)
        for c in range(NC // N1):
            cq = i * (NC // N1) + c
            wqt_buf[pl.ds(pl.multiple_of(cq * CW, CW), CW), :] = wq_buf[cq].T
        xa, xb = rows_of(r0, TS), rows_of(r0 + TS, T0)

        def xc():
            return jnp.concatenate([xa(), xb()], axis=0)

        kg_steps([(xa, 0, CW, False), (xa, CW, CW, False), (xb, 0, 2 * CW, False),
                  (xc, 2 * CW, CW, False), (xc, 3 * CW, CW, False)],
                 itertools.chain(ln_work(r0 + TS, r0 + TS, T0, LN_OWN, best, never),
                                 ln_work(src, r0 + T1, TS, LN_NEXT, best, never)), never)
        return tuple(best)

    assert N1 == 2
    best = lax.fori_loop(0, N1, phase1, tuple(best))

    wv_copy.wait()
    wo_copy.wait()
    rr = lax.broadcasted_iota(jnp.int32, (128, 128), 0) // DH
    cc = lax.broadcasted_iota(jnp.int32, (128, 128), 1) // DH
    same_head = rr == cc

    def kv_part(g):
        sl = slice(g * 128, (g + 1) * 128)
        kv = jnp.dot(g_acc[sl, :].astype(bf16), wv_buf[:, sl], preferred_element_type=f32)
        return jnp.where(same_head, kv, 0.0).astype(bf16)

    def m_part(g, kv):
        sl = slice(g * 128, (g + 1) * 128)
        m_buf[sl, :] = jnp.dot(kv, wo_buf[sl, :], preferred_element_type=f32).astype(bf16)

    rmax = jnp.max(best[0], axis=0, keepdims=True)
    idx = jnp.clip(jnp.min(jnp.where(best[0] == rmax, best[1], S)), 0, S - 1)
    gate = 1.0 / (1.0 + jnp.exp(-rmax[:, :1]))
    z = jnp.sum(z_acc[...], axis=0, keepdims=True)
    zb_buf[...] = jnp.broadcast_to(z, (128, D)).T
    r16 = pl.multiple_of((idx // 16) * 16, 16)
    blk = xn_buf[pl.ds(r16, 16), :].astype(f32)
    sel = lax.broadcasted_iota(jnp.int32, (16, D), 0) == (idx - r16)
    x_sel = jnp.sum(jnp.where(sel, blk, 0.0), axis=0, keepdims=True)
    xb_buf[...] = jnp.broadcast_to(x_sel, (128, D)).T

    for t in range(NT):
        xt_buf[t] = xn_buf[t * TS:t * TS + 128, :].T

    kv_prev = kv_part(0)
    for g in range(1, G128):
        kv = kv_part(g)
        m_part(g - 1, kv_prev)
        kv_prev = kv
    m_part(G128 - 1, kv_prev)

    def phase2(j, t_prev):
        @pl.when(j < NT - 1)
        def _():
            for c in ffn_copies(j):
                c.wait()

        t = (t_prev + 1) & (NT - 1)
        xn = xn_buf[pl.ds(pl.multiple_of(t * TS, TS), TS), :]
        j_up = jnp.minimum(j, NT - 2)
        j_dn = jnp.maximum(j - 1, 0)
        n_dup = FPC * (NT - 1) - NFU
        keep_dup = jnp.where(j >= NT - 2, 0.0, 1.0)
        late = []

        def matvec(w_ref, slot, nrows, cols, col_ref):
            acc = None
            for r in range(0, nrows, FFN_STEP):
                w = w_ref[slot, r:r + FFN_STEP, cols].astype(f32)
                p = w * jnp.concatenate([col_ref[r:r + FFN_STEP, :]] * (FW // 128), axis=1)
                for g in range(0, FFN_STEP, 8):
                    acc = p[g:g + 8, :] if acc is None else acc + p[g:g + 8, :]
                yield acc[:, :128] + acc[:, 128:]
            return acc

        def ffn_work():
            for e in range(D // FW):
                ec = slice(e * FW, (e + 1) * FW)
                acc = yield from matvec(wd_buf, j_dn, FPC * FW, ec, hb_buf)
                y_acc[:, ec] += acc
            for u in range(FPC):
                fs = slice(u * FW, (u + 1) * FW)
                g = yield from matvec(wg_buf, j_up, D, fs, xb_buf)
                a = yield from matvec(wu_buf, j_up, D, fs, xb_buf)
                g = jnp.sum(g, axis=0, keepdims=True)
                h = g * (1.0 / (1.0 + jnp.exp(-g))) * jnp.sum(a, axis=0, keepdims=True)
                if u < n_dup:
                    h = h * keep_dup
                hb = jnp.broadcast_to(h, (128, FW)).T
                hb_buf[fs, :] = hb
                late.append([FFN_LAG, hb[120:128, :] + hb[FW - 8:, :]])

        def with_late(gen):
            while True:
                dep = next(gen, None)
                if dep is None and not late:
                    return
                for e in late:
                    e[0] -= 1
                if late and late[0][0] <= 0:
                    d = late.pop(0)[1]
                    dep = d if dep is None else dep + d
                yield dep

        work = with_late(ffn_work())

        ps = []
        for c in range(NC):
            rows = slice(c * CW, (c + 1) * CW)
            if c == 0:
                q0 = jnp.dot(wqt_buf[rows, :], xt_buf[t], preferred_element_type=f32)
                qt = lax.dot_general(wqt_buf[rows, :], xn[128:], _NT, preferred_element_type=f32)
                qt = jnp.concatenate([q0, qt], axis=1)
            else:
                qt = lax.dot_general(wqt_buf[rows, :], xn, _NT, preferred_element_type=f32)
            pqt = _phi(_tie_tiles(qt, work, never, FFN_RB))
            zfull = jnp.concatenate([zb_buf[rows, :]] * (TS // 128), axis=1)
            hc = CW // DH
            den = jnp.sum((pqt * zfull).reshape(hc, DH, TS), axis=1, keepdims=True) + _EPS
            pt = pqt.reshape(hc, DH, TS) * pl.reciprocal(den, approx=True)
            ps.append(pt.reshape(CW, TS).astype(bf16).T)
        p = jnp.concatenate(ps, axis=1)
        assert NC * (CW // FFN_RB) * (TS // 128) > (D // FW) * (FPC * FW // FFN_STEP)
        y = jnp.sum(y_acc[...], axis=0, keepdims=True) * gate
        for n, (r0, nr, c0, nc) in enumerate(_OUT_PIECES):
            cols = slice(c0, c0 + nc)
            rows = pl.ds(pl.multiple_of(t * TS + r0, 128), nr)
            o = jnp.dot(p[r0:r0 + nr, :], m_buf[:, cols], preferred_element_type=f32)
            o = _tie_tiles(o, work, never, FFN_RB)
            o = o + x_buf[rows, cols].astype(f32) + xn_buf[rows, cols].astype(f32)
            hit = lax.broadcasted_iota(jnp.int32, (nr, nc), 0) == idx - (t * TS + r0)
            out_buf[rows, cols] = (o + jnp.where(hit, y[:, cols], 0.0)).astype(bf16)
            out_copy(t, n).start()
        assert next(work, 0) == 0
        return t

    lax.fori_loop(0, NT, phase2, idx // TS)
    for t in range(NT):
        for n in range(len(_OUT_PIECES)):
            out_copy(t, n).wait()


@jax.jit
def pallas_parallel_sum__linear_attn_block__moe_arch_mod__prompt_kernel(
    A_x: jax.Array,
    A_wqkv: jax.Array,
    A_wo: jax.Array,
    B_x: jax.Array,
    B_w_r: jax.Array,
    B_w_gate: jax.Array,
    B_w_up: jax.Array,
    B_w_down: jax.Array,
):
    any_spec = pl.BlockSpec(memory_space=pl.ANY)
    out = pl.pallas_call(
        _kernel,
        out_shape=jax.ShapeDtypeStruct((S, D), bf16),
        grid=(2,),
        in_specs=[any_spec] * 7,
        out_specs=any_spec,
        scratch_shapes=[
            pltpu.VMEM((S, D), bf16),
            pltpu.VMEM((S + TS, D), bf16),
            pltpu.VMEM((NC, D, CW), bf16),
            pltpu.VMEM((D, D + 128), bf16),
            pltpu.VMEM((D, D + 128), bf16),
            pltpu.VMEM((D, D), bf16),
            pltpu.VMEM((D, D), bf16),
            pltpu.VMEM((D, D), bf16),
            pltpu.VMEM((D,), bf16),
            pltpu.VMEM((D, D), f32),
            pltpu.VMEM((8, D), f32),
            pltpu.VMEM((D, 128), f32),
            pltpu.VMEM((NT, D, 128), bf16),
            pltpu.VMEM((NT - 1, D, FPC * FW), bf16),
            pltpu.VMEM((NT - 1, D, FPC * FW), bf16),
            pltpu.VMEM((NT - 1, FPC * FW, D), bf16),
            pltpu.VMEM((D, 128), f32),
            pltpu.VMEM((FPC * FW, 128), f32),
            pltpu.VMEM((8, D), f32),
            pltpu.VMEM((S, D), bf16),
            pltpu.SemaphoreType.DMA((_N_SEM,)),
            pltpu.SemaphoreType.DMA((NT * len(_OUT_PIECES),)),
        ],
        compiler_params=pltpu.CompilerParams(dimension_semantics=("arbitrary",),
                                             vmem_limit_bytes=100 * 1024 * 1024,
                                             disable_semaphore_checks=True),
        name="linattn_mod",
    )(A_x.reshape(S, D), A_wqkv, A_wo, B_w_r, B_w_gate, B_w_up, B_w_down)
    return out.reshape(1, S, D)
```

```python
import itertools

import jax
import jax.numpy as jnp
from jax import lax
import jax.experimental.pallas as pl
import jax.experimental.pallas.tpu as pltpu

S = 2048
D = 1024
F = 3584
H = 32
DH = D // H
G128 = D // 128
CW = 256
NC = D // CW
T0 = 256
TS = 512
NT = S // TS
T1 = TS + T0
N1 = (S - TS) // T1
FW = 256
NFU = F // FW
FPC = -(-NFU // (NT - 1))

FFN_STEP = 64
FFN_RB = 32
FFN_LAG = 8
LN_C = (32, (0, 0, 6, 2))
LN_D = (16, (0, 0, 8, 0, 0, 17, 7))
LN_OWN = (16, (5, 11, 0))
LN_NEXT = (16, (0, 0, 15, 0, 17))

_LN_EPS = 1.0013580322265625e-05
_EPS = 1e-6

f32 = jnp.float32
bf16 = jnp.bfloat16

_OUT_PIECES = [(0, TS, c * CW, CW) for c in range(NC - 1)] + [
    (0, 384, D - CW, CW), (384, 128, D - CW, CW)]

_X_ROWS = [(0, T0 // 2), (T0 // 2, T0 // 2), (T0, T0), (TS, TS), (2 * TS, S - 2 * TS)]
_WK_COLS = ((0, 128), (128, 384), (384, 640), (640, 1024))
_SEM_X = 0
_SEM_WK = _SEM_X + len(_X_ROWS)
_SEM_WQ = _SEM_WK + len(_WK_COLS)
_SEM_WV = _SEM_WQ + NC
_SEM_WO = _SEM_WV + 1
_SEM_WR = _SEM_WO + 1
_SEM_F = _SEM_WR + 1
_N_SEM = _SEM_F + 3 * (NT - 1)

_TN = (((0,), (0,)), ((), ()))
_NT = (((1,), (1,)), ((), ()))


def _bf16_round(v):
    return v.astype(bf16).astype(f32)


def _phi(t):
    return jnp.where(t > 0, t + 1.0, jnp.exp(t)) + _EPS


def _tie(val, dep, never, last=False):
    if dep is None:
        return val
    if last:
        tail = jnp.where(never, dep, val[-8:, -128:])
        if val.shape[1] > 128:
            tail = jnp.concatenate([val[-8:, :-128], tail], axis=1)
        return jnp.concatenate([val[:-8, :], tail], axis=0)
    head = jnp.where(never, dep, val[:8, :128])
    head = jnp.concatenate([head, val[:8, 128:]], axis=1)
    return jnp.concatenate([head, val[8:, :]], axis=0)


def _tie_tiles(val, deps, never, rb):
    cols = []
    for n in range(val.shape[1] // 128):
        blocks = [_tie(val[r:r + rb, n * 128:(n + 1) * 128], next(deps, None), never, True)
                  for r in range(0, val.shape[0], rb)]
        cols.append(jnp.concatenate(blocks, axis=0))
    return jnp.concatenate(cols, axis=1)


def _kernel(*refs):
    pl.when(pl.program_id(0) == 0)(lambda: _body(*refs))


def _body(x_hbm, wqkv_hbm, wo_hbm, wr_hbm, wg_hbm, wu_hbm, wd_hbm, out_hbm,
          x_buf, xn_buf, wq_buf, wk_buf, wv_buf, wqt_buf, wo_buf, m_buf, wr_buf,
          g_acc, z_acc, zb_buf, xt_buf,
          wg_buf, wu_buf, wd_buf, xb_buf, hb_buf, y_acc, out_buf,
          sem, o_sem):

    def x_copy(i):
        rows = pl.ds(*_X_ROWS[i])
        return pltpu.make_async_copy(x_hbm.at[rows, :], x_buf.at[rows, :], sem.at[_SEM_X + i])

    def wk_copy(s):
        c0, c1 = _WK_COLS[s]
        return pltpu.make_async_copy(wqkv_hbm.at[:, pl.ds(D + c0, c1 - c0)],
                                     wk_buf.at[:, pl.ds(c0, c1 - c0)], sem.at[_SEM_WK + s])

    def wq_copy(c):
        return pltpu.make_async_copy(wqkv_hbm.at[:, pl.ds(c * CW, CW)], wq_buf.at[c],
                                     sem.at[_SEM_WQ + c])

    wv_copy = pltpu.make_async_copy(wqkv_hbm.at[:, pl.ds(2 * D, D)], wv_buf.at[:, pl.ds(0, D)],
                                    sem.at[_SEM_WV])
    wo_copy = pltpu.make_async_copy(wo_hbm, wo_buf, sem.at[_SEM_WO])
    wr_copy = pltpu.make_async_copy(wr_hbm, wr_buf, sem.at[_SEM_WR])

    def ffn_copies(j):
        s = _SEM_F + 3 * j
        if isinstance(j, int):
            f0 = min(j * FPC, NFU - FPC) * FW
        else:
            f0 = pl.multiple_of(jnp.minimum(j * FPC, NFU - FPC) * FW, FW)
        fs = pl.ds(f0, FPC * FW)
        return (pltpu.make_async_copy(wg_hbm.at[:, fs], wg_buf.at[j], sem.at[s]),
                pltpu.make_async_copy(wu_hbm.at[:, fs], wu_buf.at[j], sem.at[s + 1]),
                pltpu.make_async_copy(wd_hbm.at[fs, :], wd_buf.at[j], sem.at[s + 2]))

    def out_copy(t, p):
        r0, nr, c0, nc = _OUT_PIECES[p]
        row = t * TS + r0
        rows = pl.ds(row if isinstance(t, int) else pl.multiple_of(row, 128), nr)
        cols = pl.ds(c0, nc)
        return pltpu.make_async_copy(out_buf.at[rows, cols], out_hbm.at[rows, cols],
                                     o_sem.at[t * len(_OUT_PIECES) + p])

    x_copy(0).start()
    x_copy(1).start()
    wk_copy(0).start()
    wr_copy.start()
    wk_copy(1).start()
    x_copy(2).start()
    wk_copy(2).start()
    wk_copy(3).start()
    for i in range(3, len(_X_ROWS)):
        x_copy(i).start()
    for c in range(NC):
        wq_copy(c).start()
    wv_copy.start()
    wo_copy.start()
    for j in range(NT - 1):
        for c in ffn_copies(j):
            c.start(priority=1)

    y_acc[...] = jnp.zeros_like(y_acc)
    hb_buf[...] = jnp.zeros_like(hb_buf)

    sub_iota = lax.broadcasted_iota(jnp.int32, (8, 128), 0)

    def route(xn, row0, best):
        nr = xn.shape[0]
        wr = wr_buf[...].reshape(1, D).astype(f32)
        r = _bf16_round(jnp.sum(xn.astype(f32) * wr, axis=-1, keepdims=True))
        r = jnp.broadcast_to(r, (nr, 128))
        for g in range(0, nr, 8):
            rg = r[g:g + 8, :]
            better = rg > best[0]
            best[0] = jnp.where(better, rg, best[0])
            best[1] = jnp.where(better, sub_iota + (row0 + g), best[1])

    def layernorm(src, dst, nr, best, after=None, never=None):
        x = x_buf[pl.ds(src, nr), :].astype(f32)
        x = _tie(x, after, never)
        mean = jnp.sum(x, axis=-1, keepdims=True) * (1.0 / D)
        mean_b = _bf16_round(mean)
        e = x - mean_b
        off = mean - mean_b
        var = jnp.sum(e * e, axis=-1, keepdims=True) * (1.0 / D) - off * off
        sd = _bf16_round(jnp.sqrt(_bf16_round(_bf16_round(var) + _LN_EPS)))
        rs = pl.reciprocal(sd, approx=True)
        rs = jnp.where(sd == jnp.inf, 0.0, rs * (2.0 - sd * rs))
        xf = _bf16_round(e) * rs
        xn = xf.astype(bf16)
        xn_buf[pl.ds(dst, nr), :] = xn
        if best is not None:
            route(xn, src, best)
        dep = None
        for g in range(0, nr, 8):
            dg = xf[g:g + 8, D - 128:]
            dep = dg if dep is None else dep + dg
        return dep, sd

    def ln_work(src, dst, nr, plan, best, never):
        sub, counts = plan
        assert sub * sum(counts) == nr
        o = 0
        for n in counts:
            dep = None
            for _ in range(n):
                dep = layernorm(src + o, dst + o, sub, best, dep, never)[0]
                o += sub
            yield dep

    def rows_of(r0, nr):
        got = []

        def get():
            if not got:
                got.append(xn_buf[pl.ds(r0, nr), :])
            return got[0]
        return get

    def kg_steps(jobs, work, never):
        def tied(val):
            return _tie(val, next(work, None), never, True)

        def k_part(xn, c0, cw, init):
            cols = slice(c0, c0 + cw)
            xn = xn()
            pk = _phi(tied(jnp.dot(xn, wk_buf[:, cols], preferred_element_type=f32)))
            zc = jnp.sum(pk.reshape(xn.shape[0] // 8, 8, cw), axis=0)
            z_acc[:, cols] = zc if init else z_acc[:, cols] + zc
            return pk.astype(bf16)

        def g_part(pk, xn, c0, cw, init):
            rows = slice(c0, c0 + cw)
            g = tied(lax.dot_general(pk, xn(), _TN, preferred_element_type=f32))
            g_acc[rows, :] = g if init else g_acc[rows, :] + g

        prev = None
        for job in jobs:
            if job is None:
                g_part(prev[0], *prev[1])
                prev = None
                continue
            pk = k_part(*job)
            if prev is not None:
                g_part(prev[0], *prev[1])
            prev = (pk, job)
        g_part(prev[0], *prev[1])
        assert next(work, None) is None

    best = [jnp.full((8, 128), -jnp.inf, f32), jnp.zeros((8, 128), jnp.int32)]
    x_copy(0).wait()
    sd0 = layernorm(0, 0, T0 // 2, None)[1]
    x_copy(1).wait()
    layernorm(T0 // 2, T0 // 2, T0 // 2, None)
    wk_copy(0).wait()
    never = jnp.min(sd0[0:8, :]) < 0.0
    kg_steps([(rows_of(0, T0 // 2), 0, 128, True), (rows_of(T0 // 2, T0 // 2), 0, 128, False)],
             iter(()), never)

    def route_first():
        yield None
        for r in range(0, T0, T0 // 2):
            route(xn_buf[r:r + T0 // 2, :], r, best)
            yield best[0]

    wr_copy.wait()
    wk_copy(1).wait()
    xa = rows_of(0, T0)
    kg_steps([(xa, 128, 128, True), (xa, 256, 128, True)], route_first(), never)

    x_copy(2).wait()
    wk_copy(2).wait()
    xa, xb = rows_of(0, T0), rows_of(T0, T0)
    kg_steps([(xa, 384, 128, True), (xa, 512, 128, True), None,
              (xb, 0, 128, False), (xb, 128, 128, False)],
             ln_work(T0, T0, T0, LN_C, best, never), never)

    wk_copy(3).wait()
    x_copy(3).wait()
    xa, xb = rows_of(0, TS), rows_of(T0, T0)
    kg_steps([(xb, 256, 256, False), (xb, 512, 128, False),
              (xa, 640, 128, True), (xa, 768, 256, True)],
             ln_work(TS, TS, TS, LN_D, best, never), never)
    x_copy(4).wait()
    for c in range(NC):
        wq_copy(c).wait()

    def phase1(i, carry):
        best = list(carry)
        r0 = pl.multiple_of(TS + i * T1, 128)
        src = pl.multiple_of(jnp.minimum(r0 + T1, S - TS), 128)
        for c in range(NC // N1):
            cq = i * (NC // N1) + c
            wqt_buf[pl.ds(pl.multiple_of(cq * CW, CW), CW), :] = wq_buf[cq].T
        xa, xb = rows_of(r0, TS), rows_of(r0 + TS, T0)

        def xc():
            return jnp.concatenate([xa(), xb()], axis=0)

        kg_steps([(xa, 0, CW, False), (xa, CW, CW, False), (xb, 0, 2 * CW, False),
                  (xc, 2 * CW, CW, False), (xc, 3 * CW, CW, False)],
                 itertools.chain(ln_work(r0 + TS, r0 + TS, T0, LN_OWN, best, never),
                                 ln_work(src, r0 + T1, TS, LN_NEXT, best, never)), never)
        return tuple(best)

    best = lax.fori_loop(0, N1, phase1, tuple(best))

    wv_copy.wait()
    wo_copy.wait()
    rr = lax.broadcasted_iota(jnp.int32, (128, 128), 0) // DH
    cc = lax.broadcasted_iota(jnp.int32, (128, 128), 1) // DH
    same_head = rr == cc

    def kv_part(g):
        sl = slice(g * 128, (g + 1) * 128)
        kv = jnp.dot(g_acc[sl, :].astype(bf16), wv_buf[:, sl], preferred_element_type=f32)
        return jnp.where(same_head, kv, 0.0).astype(bf16)

    def m_part(g, kv):
        sl = slice(g * 128, (g + 1) * 128)
        m_buf[sl, :] = jnp.dot(kv, wo_buf[sl, :], preferred_element_type=f32).astype(bf16)

    rmax = jnp.max(best[0], axis=0, keepdims=True)
    idx = jnp.clip(jnp.min(jnp.where(best[0] == rmax, best[1], S)), 0, S - 1)
    gate = 1.0 / (1.0 + jnp.exp(-rmax[:, :1]))
    z = jnp.sum(z_acc[...], axis=0, keepdims=True)
    zb_buf[...] = jnp.broadcast_to(z, (128, D)).T
    r16 = pl.multiple_of((idx // 16) * 16, 16)
    blk = xn_buf[pl.ds(r16, 16), :].astype(f32)
    sel = lax.broadcasted_iota(jnp.int32, (16, D), 0) == (idx - r16)
    x_sel = jnp.sum(jnp.where(sel, blk, 0.0), axis=0, keepdims=True)
    xb_buf[...] = jnp.broadcast_to(x_sel, (128, D)).T

    for t in range(NT):
        xt_buf[t] = xn_buf[t * TS:t * TS + 128, :].T

    kv_prev = kv_part(0)
    for g in range(1, G128):
        kv = kv_part(g)
        m_part(g - 1, kv_prev)
        kv_prev = kv
    m_part(G128 - 1, kv_prev)

    def phase2(j, t_prev):
        @pl.when(j < NT - 1)
        def _():
            for c in ffn_copies(j):
                c.wait()

        t = (t_prev + 1) & (NT - 1)
        xn = xn_buf[pl.ds(pl.multiple_of(t * TS, TS), TS), :]
        j_up = jnp.minimum(j, NT - 2)
        j_dn = jnp.maximum(j - 1, 0)
        n_dup = FPC * (NT - 1) - NFU
        keep_dup = jnp.where(j >= NT - 2, 0.0, 1.0)
        late = []

        def matvec(w_ref, slot, nrows, cols, col_ref):
            acc = None
            for r in range(0, nrows, FFN_STEP):
                w = w_ref[slot, r:r + FFN_STEP, cols].astype(f32)
                p = w * jnp.concatenate([col_ref[r:r + FFN_STEP, :]] * (FW // 128), axis=1)
                for g in range(0, FFN_STEP, 8):
                    acc = p[g:g + 8, :] if acc is None else acc + p[g:g + 8, :]
                yield acc[:, :128] + acc[:, 128:]
            return acc

        def ffn_work():
            for e in range(D // FW):
                ec = slice(e * FW, (e + 1) * FW)
                acc = yield from matvec(wd_buf, j_dn, FPC * FW, ec, hb_buf)
                y_acc[:, ec] += acc
            for u in range(FPC):
                fs = slice(u * FW, (u + 1) * FW)
                g = yield from matvec(wg_buf, j_up, D, fs, xb_buf)
                a = yield from matvec(wu_buf, j_up, D, fs, xb_buf)
                g = jnp.sum(g, axis=0, keepdims=True)
                h = g * (1.0 / (1.0 + jnp.exp(-g))) * jnp.sum(a, axis=0, keepdims=True)
                if u < n_dup:
                    h = h * keep_dup
                hb = jnp.broadcast_to(h, (128, FW)).T
                hb_buf[fs, :] = hb
                late.append([FFN_LAG, hb[120:128, :] + hb[FW - 8:, :]])

        def with_late(gen):
            while True:
                dep = next(gen, None)
                if dep is None and not late:
                    return
                for e in late:
                    e[0] -= 1
                if late and late[0][0] <= 0:
                    d = late.pop(0)[1]
                    dep = d if dep is None else dep + d
                yield dep

        work = with_late(ffn_work())

        ps = []
        for c in range(NC):
            rows = slice(c * CW, (c + 1) * CW)
            if c == 0:
                q0 = jnp.dot(wqt_buf[rows, :], xt_buf[t], preferred_element_type=f32)
                qt = lax.dot_general(wqt_buf[rows, :], xn[128:], _NT, preferred_element_type=f32)
                qt = jnp.concatenate([q0, qt], axis=1)
            else:
                qt = lax.dot_general(wqt_buf[rows, :], xn, _NT, preferred_element_type=f32)
            pqt = _phi(_tie_tiles(qt, work, never, FFN_RB))
            zfull = jnp.concatenate([zb_buf[rows, :]] * (TS // 128), axis=1)
            hc = CW // DH
            den = jnp.sum((pqt * zfull).reshape(hc, DH, TS), axis=1, keepdims=True) + _EPS
            pt = pqt.reshape(hc, DH, TS) * pl.reciprocal(den, approx=True)
            ps.append(pt.reshape(CW, TS).astype(bf16).T)
        p = jnp.concatenate(ps, axis=1)
        assert NC * (CW // FFN_RB) * (TS // 128) > (D // FW) * (FPC * FW // FFN_STEP)
        y = jnp.sum(y_acc[...], axis=0, keepdims=True) * gate
        for n, (r0, nr, c0, nc) in enumerate(_OUT_PIECES):
            cols = slice(c0, c0 + nc)
            rows = pl.ds(pl.multiple_of(t * TS + r0, 128), nr)
            o = jnp.dot(p[r0:r0 + nr, :], m_buf[:, cols], preferred_element_type=f32)
            o = _tie_tiles(o, work, never, FFN_RB)
            o = o + x_buf[rows, cols].astype(f32) + xn_buf[rows, cols].astype(f32)
            hit = lax.broadcasted_iota(jnp.int32, (nr, nc), 0) == idx - (t * TS + r0)
            out_buf[rows, cols] = (o + jnp.where(hit, y[:, cols], 0.0)).astype(bf16)
            out_copy(t, n).start()
        assert next(work, 0) == 0
        return t

    lax.fori_loop(0, NT, phase2, idx // TS)
    for t in range(NT):
        for n in range(len(_OUT_PIECES)):
            out_copy(t, n).wait()


@jax.jit
def pallas_parallel_sum__linear_attn_block__moe_arch_mod__prompt_kernel(
    A_x: jax.Array,
    A_wqkv: jax.Array,
    A_wo: jax.Array,
    B_x: jax.Array,
    B_w_r: jax.Array,
    B_w_gate: jax.Array,
    B_w_up: jax.Array,
    B_w_down: jax.Array,
):
    any_spec = pl.BlockSpec(memory_space=pl.ANY)
    out = pl.pallas_call(
        _kernel,
        out_shape=jax.ShapeDtypeStruct((S, D), bf16),
        grid=(2,),
        in_specs=[any_spec] * 7,
        out_specs=any_spec,
        scratch_shapes=[
            pltpu.VMEM((S, D), bf16),
            pltpu.VMEM((S + TS, D), bf16),
            pltpu.VMEM((NC, D, CW), bf16),
            pltpu.VMEM((D, D + 128), bf16),
            pltpu.VMEM((D, D + 128), bf16),
            pltpu.VMEM((D, D), bf16),
            pltpu.VMEM((D, D), bf16),
            pltpu.VMEM((D, D), bf16),
            pltpu.VMEM((D,), bf16),
            pltpu.VMEM((D, D), f32),
            pltpu.VMEM((8, D), f32),
            pltpu.VMEM((D, 128), f32),
            pltpu.VMEM((NT, D, 128), bf16),
            pltpu.VMEM((NT - 1, D, FPC * FW), bf16),
            pltpu.VMEM((NT - 1, D, FPC * FW), bf16),
            pltpu.VMEM((NT - 1, FPC * FW, D), bf16),
            pltpu.VMEM((D, 128), f32),
            pltpu.VMEM((FPC * FW, 128), f32),
            pltpu.VMEM((8, D), f32),
            pltpu.VMEM((S, D), bf16),
            pltpu.SemaphoreType.DMA((_N_SEM,)),
            pltpu.SemaphoreType.DMA((NT * len(_OUT_PIECES),)),
        ],
        compiler_params=pltpu.CompilerParams(dimension_semantics=("arbitrary",),
                                             vmem_limit_bytes=100 * 1024 * 1024,
                                             disable_semaphore_checks=True),
        name="linattn_mod",
    )(A_x.reshape(S, D), A_wqkv, A_wo, B_w_r, B_w_gate, B_w_up, B_w_down)
    return out.reshape(1, S, D)
```

```python
import itertools

import jax
import jax.numpy as jnp
from jax import lax
import jax.experimental.pallas as pl
import jax.experimental.pallas.tpu as pltpu

S = 2048
D = 1024
F = 3584
H = 32
DH = D // H
G128 = D // 128
CW = 256
NC = D // CW
T0 = 256
TS = 512
NT = S // TS
T1 = TS + T0
N1 = (S - TS) // T1
FW = 256
NFU = F // FW
FPC = -(-NFU // NT)
FP0 = NFU - (NT - 1) * FPC

FFN_STEP = 64
FFN_RB = 16
FFN_THIN = (2, 5)
FFN_LAG = 8
LN_C = (32, (0, 0, 6, 2))
LN_D = (16, (0, 0, 8, 0, 0, 17, 7))
LN_OWN = (16, (5, 11, 0))
LN_NEXT = (16, (0, 0, 15, 0, 17))

_LN_EPS = 1.0013580322265625e-05
_EPS = 1e-6

f32 = jnp.float32
bf16 = jnp.bfloat16

_OUT_PIECES = [(0, TS, c * CW, CW) for c in range(NC - 1)] + [
    (0, 384, D - CW, CW), (384, 128, D - CW, CW)]

_X_ROWS = [(0, T0 // 2), (T0 // 2, T0 // 2), (T0, T0), (TS, TS), (2 * TS, S - 2 * TS)]
_WK_COLS = ((0, 128), (128, 384), (384, 640), (640, 1024))
_SEM_X = 0
_SEM_WK = _SEM_X + len(_X_ROWS)
_SEM_WQ = _SEM_WK + len(_WK_COLS)
_SEM_WV = _SEM_WQ + NC
_SEM_WO = _SEM_WV + 1
_SEM_WR = _SEM_WO + 1
_SEM_F = _SEM_WR + 1
_N_SEM = _SEM_F + 3 * NT

_TN = (((0,), (0,)), ((), ()))
_NT = (((1,), (1,)), ((), ()))


def _bf16_round(v):
    return v.astype(bf16).astype(f32)


def _phi(t):
    return jnp.where(t > 0, t + 1.0, jnp.exp(t)) + _EPS


def _tie(val, dep, never, last=False):
    if dep is None:
        return val
    if last:
        tail = jnp.where(never, dep, val[-8:, -128:])
        if val.shape[1] > 128:
            tail = jnp.concatenate([val[-8:, :-128], tail], axis=1)
        return jnp.concatenate([val[:-8, :], tail], axis=0)
    head = jnp.where(never, dep, val[:8, :128])
    head = jnp.concatenate([head, val[:8, 128:]], axis=1)
    return jnp.concatenate([head, val[8:, :]], axis=0)


def _tie_tiles(val, deps, never, rb):
    cols = []
    for n in range(val.shape[1] // 128):
        blocks = [_tie(val[r:r + rb, n * 128:(n + 1) * 128], next(deps, None), never, True)
                  for r in range(0, val.shape[0], rb)]
        cols.append(jnp.concatenate(blocks, axis=0))
    return jnp.concatenate(cols, axis=1)


def _thin(it, num, den):
    i = 0
    while True:
        take = ((i + 1) * num) // den > (i * num) // den
        yield next(it, None) if take else None
        i += 1


def _kernel(*refs):
    pl.when(pl.program_id(0) == 0)(lambda: _body(*refs))


def _body(x_hbm, wqkv_hbm, wo_hbm, wr_hbm, wg_hbm, wu_hbm, wd_hbm, out_hbm,
          x_buf, xn_buf, wq_buf, wk_buf, wv_buf, wqt_buf, wo_buf, m_buf, wr_buf,
          g_acc, z_acc, zb_buf, xt_buf,
          wg_buf, wu_buf, wd_buf, xb_buf, hb_buf, y_acc, out_buf,
          sem, o_sem):

    def x_copy(i):
        rows = pl.ds(*_X_ROWS[i])
        return pltpu.make_async_copy(x_hbm.at[rows, :], x_buf.at[rows, :], sem.at[_SEM_X + i])

    def wk_copy(s):
        c0, c1 = _WK_COLS[s]
        return pltpu.make_async_copy(wqkv_hbm.at[:, pl.ds(D + c0, c1 - c0)],
                                     wk_buf.at[:, pl.ds(c0, c1 - c0)], sem.at[_SEM_WK + s])

    def wq_copy(c):
        return pltpu.make_async_copy(wqkv_hbm.at[:, pl.ds(c * CW, CW)], wq_buf.at[c],
                                     sem.at[_SEM_WQ + c])

    wv_copy = pltpu.make_async_copy(wqkv_hbm.at[:, pl.ds(2 * D, D)], wv_buf.at[:, pl.ds(0, D)],
                                    sem.at[_SEM_WV])
    wo_copy = pltpu.make_async_copy(wo_hbm, wo_buf, sem.at[_SEM_WO])
    wr_copy = pltpu.make_async_copy(wr_hbm, wr_buf, sem.at[_SEM_WR])

    def ffn_copy(j, which):
        n = (FP0 if isinstance(j, int) and j == 0 and which < 2 else FPC) * FW
        if isinstance(j, int):
            f0 = max(FP0 + (j - 1) * FPC, 0) * FW
        else:
            f0 = pl.multiple_of(jnp.maximum(FP0 + (j - 1) * FPC, 0) * FW, FW)
        s = sem.at[_SEM_F + 3 * j + which]
        if which == 2:
            return pltpu.make_async_copy(wd_hbm.at[pl.ds(f0, n), :],
                                         wd_buf.at[j, :, pl.ds(0, D)], s)
        src, dst = ((wg_hbm, wg_buf), (wu_hbm, wu_buf))[which]
        return pltpu.make_async_copy(src.at[:, pl.ds(f0, n)], dst.at[j, :, pl.ds(0, n)], s)

    def out_copy(t, p):
        r0, nr, c0, nc = _OUT_PIECES[p]
        row = t * TS + r0
        rows = pl.ds(row if isinstance(t, int) else pl.multiple_of(row, 128), nr)
        cols = pl.ds(c0, nc)
        return pltpu.make_async_copy(out_buf.at[rows, cols], out_hbm.at[rows, cols],
                                     o_sem.at[t * len(_OUT_PIECES) + p])

    x_copy(0).start()
    x_copy(1).start()
    wk_copy(0).start()
    wr_copy.start()
    wk_copy(1).start()
    x_copy(2).start()
    wk_copy(2).start()
    wk_copy(3).start()
    for i in range(3, len(_X_ROWS)):
        x_copy(i).start()
    for c in range(NC):
        wq_copy(c).start()
    wv_copy.start()
    wo_copy.start()
    for j in range(NT):
        for which in range(3):
            ffn_copy(j, which).start(priority=1)

    y_acc[...] = jnp.zeros_like(y_acc)
    hb_buf[...] = jnp.zeros_like(hb_buf)

    sub_iota = lax.broadcasted_iota(jnp.int32, (8, 128), 0)

    def route(xn, row0, best):
        nr = xn.shape[0]
        wr = wr_buf[...].reshape(1, D).astype(f32)
        r = _bf16_round(jnp.sum(xn.astype(f32) * wr, axis=-1, keepdims=True))
        r = jnp.broadcast_to(r, (nr, 128))
        for g in range(0, nr, 8):
            rg = r[g:g + 8, :]
            better = rg > best[0]
            best[0] = jnp.where(better, rg, best[0])
            best[1] = jnp.where(better, sub_iota + (row0 + g), best[1])

    def layernorm(src, dst, nr, best, after=None, never=None):
        x = x_buf[pl.ds(src, nr), :].astype(f32)
        x = _tie(x, after, never)
        mean = jnp.sum(x, axis=-1, keepdims=True) * (1.0 / D)
        mean_b = _bf16_round(mean)
        e = x - mean_b
        off = mean - mean_b
        var = jnp.sum(e * e, axis=-1, keepdims=True) * (1.0 / D) - off * off
        sd = _bf16_round(jnp.sqrt(_bf16_round(_bf16_round(var) + _LN_EPS)))
        rs = pl.reciprocal(sd, approx=True)
        rs = jnp.where(sd == jnp.inf, 0.0, rs * (2.0 - sd * rs))
        xf = _bf16_round(e) * rs
        xn = xf.astype(bf16)
        xn_buf[pl.ds(dst, nr), :] = xn
        if best is not None:
            route(xn, src, best)
        dep = None
        for g in range(0, nr, 8):
            dg = xf[g:g + 8, D - 128:]
            dep = dg if dep is None else dep + dg
        return dep, sd

    def ln_work(src, dst, nr, plan, best, never):
        sub, counts = plan
        assert sub * sum(counts) == nr
        o = 0
        for n in counts:
            dep = None
            for _ in range(n):
                dep = layernorm(src + o, dst + o, sub, best, dep, never)[0]
                o += sub
            yield dep

    def rows_of(r0, nr):
        got = []

        def get():
            if not got:
                got.append(xn_buf[pl.ds(r0, nr), :])
            return got[0]
        return get

    def kg_steps(jobs, work, never):
        def tied(val):
            return _tie(val, next(work, None), never, True)

        def k_part(xn, c0, cw, init):
            cols = slice(c0, c0 + cw)
            xn = xn()
            pk = _phi(tied(jnp.dot(xn, wk_buf[:, cols], preferred_element_type=f32)))
            zc = jnp.sum(pk.reshape(xn.shape[0] // 8, 8, cw), axis=0)
            z_acc[:, cols] = zc if init else z_acc[:, cols] + zc
            return pk.astype(bf16)

        def g_part(pk, xn, c0, cw, init):
            rows = slice(c0, c0 + cw)
            g = tied(lax.dot_general(pk, xn(), _TN, preferred_element_type=f32))
            g_acc[rows, :] = g if init else g_acc[rows, :] + g

        prev = None
        for job in jobs:
            if job is None:
                g_part(prev[0], *prev[1])
                prev = None
                continue
            pk = k_part(*job)
            if prev is not None:
                g_part(prev[0], *prev[1])
            prev = (pk, job)
        g_part(prev[0], *prev[1])
        assert next(work, None) is None

    best = [jnp.full((8, 128), -jnp.inf, f32), jnp.zeros((8, 128), jnp.int32)]
    x_copy(0).wait()
    sd0 = layernorm(0, 0, T0 // 2, None)[1]
    x_copy(1).wait()
    layernorm(T0 // 2, T0 // 2, T0 // 2, None)
    wk_copy(0).wait()
    never = jnp.min(sd0[0:8, :]) < 0.0
    kg_steps([(rows_of(0, T0 // 2), 0, 128, True), (rows_of(T0 // 2, T0 // 2), 0, 128, False)],
             iter(()), never)

    def route_first():
        yield None
        for r in range(0, T0, T0 // 2):
            route(xn_buf[r:r + T0 // 2, :], r, best)
            yield best[0]

    wr_copy.wait()
    wk_copy(1).wait()
    xa = rows_of(0, T0)
    kg_steps([(xa, 128, 128, True), (xa, 256, 128, True)], route_first(), never)

    x_copy(2).wait()
    wk_copy(2).wait()
    xa, xb = rows_of(0, T0), rows_of(T0, T0)
    kg_steps([(xa, 384, 128, True), (xa, 512, 128, True), None,
              (xb, 0, 128, False), (xb, 128, 128, False)],
             ln_work(T0, T0, T0, LN_C, best, never), never)

    wk_copy(3).wait()
    x_copy(3).wait()
    xa, xb = rows_of(0, TS), rows_of(T0, T0)
    kg_steps([(xb, 256, 256, False), (xb, 512, 128, False),
              (xa, 640, 128, True), (xa, 768, 256, True)],
             ln_work(TS, TS, TS, LN_D, best, never), never)
    x_copy(4).wait()
    for c in range(NC):
        wq_copy(c).wait()

    def phase1(i, carry):
        best = list(carry)
        r0 = pl.multiple_of(TS + i * T1, 128)
        src = pl.multiple_of(jnp.minimum(r0 + T1, S - TS), 128)
        for c in range(NC // N1):
            cq = i * (NC // N1) + c
            wqt_buf[pl.ds(pl.multiple_of(cq * CW, CW), CW), :] = wq_buf[cq].T
        xa, xb = rows_of(r0, TS), rows_of(r0 + TS, T0)

        def xc():
            return jnp.concatenate([xa(), xb()], axis=0)

        kg_steps([(xa, 0, CW, False), (xa, CW, CW, False), (xb, 0, 2 * CW, False),
                  (xc, 2 * CW, CW, False), (xc, 3 * CW, CW, False)],
                 itertools.chain(ln_work(r0 + TS, r0 + TS, T0, LN_OWN, best, never),
                                 ln_work(src, r0 + T1, TS, LN_NEXT, best, never)), never)
        return tuple(best)

    best = lax.fori_loop(0, N1, phase1, tuple(best))

    wv_copy.wait()
    wo_copy.wait()
    ffn_copy(0, 0).wait()
    ffn_copy(0, 1).wait()
    rr = lax.broadcasted_iota(jnp.int32, (128, 128), 0) // DH
    cc = lax.broadcasted_iota(jnp.int32, (128, 128), 1) // DH
    same_head = rr == cc

    def kv_part(g):
        sl = slice(g * 128, (g + 1) * 128)
        kv = jnp.dot(g_acc[sl, :].astype(bf16), wv_buf[:, sl], preferred_element_type=f32)
        return jnp.where(same_head, kv, 0.0).astype(bf16)

    def m_part(g, kv, work):
        sl = slice(g * 128, (g + 1) * 128)
        m = jnp.dot(kv, wo_buf[sl, :], preferred_element_type=f32)
        m_buf[sl, :] = _tie_tiles(m, work, never, 64).astype(bf16)

    def ffn_items(j_dn, j_up, n_up, down_done):
        late = []

        def matvec(w_ref, slot, nrows, cols, col_ref):
            acc = None
            for r in range(0, nrows, FFN_STEP):
                w = w_ref[slot, r:r + FFN_STEP, cols].astype(f32)
                p = w * jnp.concatenate([col_ref[r:r + FFN_STEP, :]] * (FW // 128), axis=1)
                for g in range(0, FFN_STEP, 8):
                    acc = p[g:g + 8, :] if acc is None else acc + p[g:g + 8, :]
                yield acc[:, :128] + acc[:, 128:]
            return acc

        def work():
            if j_dn is not None:
                for e in range(D // FW):
                    ec = slice(e * FW, (e + 1) * FW)
                    acc = yield from matvec(wd_buf, j_dn, FPC * FW, ec, hb_buf)
                    y_acc[:, ec] += acc
                down_done.append(True)
            for u in range(n_up):
                fs = slice(u * FW, (u + 1) * FW)
                g = yield from matvec(wg_buf, j_up, D, fs, xb_buf)
                a = yield from matvec(wu_buf, j_up, D, fs, xb_buf)
                g = jnp.sum(g, axis=0, keepdims=True)
                h = g * (1.0 / (1.0 + jnp.exp(-g))) * jnp.sum(a, axis=0, keepdims=True)
                hb = jnp.broadcast_to(h, (128, FW)).T
                hb_buf[fs, :] = hb
                late.append([FFN_LAG, hb[120:128, :] + hb[FW - 8:, :]])

        gen = work()
        while True:
            dep = next(gen, None)
            if dep is None and not late:
                return
            for e in late:
                e[0] -= 1
            if late and late[0][0] <= 0:
                d = late.pop(0)[1]
                dep = d if dep is None else dep + d
            yield dep


    rmax = jnp.max(best[0], axis=0, keepdims=True)
    idx = jnp.clip(jnp.min(jnp.where(best[0] == rmax, best[1], S)), 0, S - 1)
    gate = 1.0 / (1.0 + jnp.exp(-rmax[:, :1]))
    r16 = pl.multiple_of((idx // 16) * 16, 16)
    blk = xn_buf[pl.ds(r16, 16), :].astype(f32)
    sel = lax.broadcasted_iota(jnp.int32, (16, D), 0) == (idx - r16)
    x_sel = jnp.sum(jnp.where(sel, blk, 0.0), axis=0, keepdims=True)
    xb_buf[...] = jnp.broadcast_to(x_sel, (128, D)).T

    items = ffn_items(None, 0, FP0, None)
    kv_prev = kv_part(0)
    for g in range(1, G128):
        kv = kv_part(g)
        m_part(g - 1, kv_prev, items)
        kv_prev = kv
    m_part(G128 - 1, kv_prev, items)
    assert next(items, 0) == 0
    z = jnp.sum(z_acc[...], axis=0, keepdims=True)
    zb_buf[...] = jnp.broadcast_to(z, (128, D)).T
    for t in range(NT):
        xt_buf[t] = xn_buf[t * TS:t * TS + 128, :].T

    def phase2(j, t_prev):
        ffn_copy(j, 2).wait()

        @pl.when(j < NT - 1)
        def _():
            ffn_copy(j + 1, 0).wait()
            ffn_copy(j + 1, 1).wait()

        t = (t_prev + 1) & (NT - 1)
        xn = xn_buf[pl.ds(pl.multiple_of(t * TS, TS), TS), :]
        down_done = []
        items = ffn_items(j, jnp.minimum(j + 1, NT - 1), FPC, down_done)
        work = _thin(items, *FFN_THIN)

        ps = []
        for c in range(NC):
            rows = slice(c * CW, (c + 1) * CW)
            if c == 0:
                q0 = jnp.dot(wqt_buf[rows, :], xt_buf[t], preferred_element_type=f32)
                qt = lax.dot_general(wqt_buf[rows, :], xn[128:], _NT, preferred_element_type=f32)
                qt = jnp.concatenate([q0, qt], axis=1)
            else:
                qt = lax.dot_general(wqt_buf[rows, :], xn, _NT, preferred_element_type=f32)
            pqt = _phi(_tie_tiles(qt, work, never, FFN_RB))
            zfull = jnp.concatenate([zb_buf[rows, :]] * (TS // 128), axis=1)
            hc = CW // DH
            den = jnp.sum((pqt * zfull).reshape(hc, DH, TS), axis=1, keepdims=True) + _EPS
            pt = pqt.reshape(hc, DH, TS) * pl.reciprocal(den, approx=True)
            ps.append(pt.reshape(CW, TS).astype(bf16).T)
        p = jnp.concatenate(ps, axis=1)
        assert down_done
        y = jnp.sum(y_acc[...], axis=0, keepdims=True) * gate
        for n, (r0, nr, c0, nc) in enumerate(_OUT_PIECES):
            cols = slice(c0, c0 + nc)
            rows = pl.ds(pl.multiple_of(t * TS + r0, 128), nr)
            o = jnp.dot(p[r0:r0 + nr, :], m_buf[:, cols], preferred_element_type=f32)
            o = _tie_tiles(o, work, never, FFN_RB)
            o = o + x_buf[rows, cols].astype(f32) + xn_buf[rows, cols].astype(f32)
            hit = lax.broadcasted_iota(jnp.int32, (nr, nc), 0) == idx - (t * TS + r0)
            out_buf[rows, cols] = (o + jnp.where(hit, y[:, cols], 0.0)).astype(bf16)
            out_copy(t, n).start()
        assert next(items, 0) == 0
        return t

    lax.fori_loop(0, NT, phase2, idx // TS)
    for t in range(NT):
        for n in range(len(_OUT_PIECES)):
            out_copy(t, n).wait()


@jax.jit
def pallas_parallel_sum__linear_attn_block__moe_arch_mod__prompt_kernel(
    A_x: jax.Array,
    A_wqkv: jax.Array,
    A_wo: jax.Array,
    B_x: jax.Array,
    B_w_r: jax.Array,
    B_w_gate: jax.Array,
    B_w_up: jax.Array,
    B_w_down: jax.Array,
):
    any_spec = pl.BlockSpec(memory_space=pl.ANY)
    out = pl.pallas_call(
        _kernel,
        out_shape=jax.ShapeDtypeStruct((S, D), bf16),
        grid=(2,),
        in_specs=[any_spec] * 7,
        out_specs=any_spec,
        scratch_shapes=[
            pltpu.VMEM((S, D), bf16),
            pltpu.VMEM((S + TS, D), bf16),
            pltpu.VMEM((NC, D, CW), bf16),
            pltpu.VMEM((D, D + 128), bf16),
            pltpu.VMEM((D, D + 128), bf16),
            pltpu.VMEM((D, D), bf16),
            pltpu.VMEM((D, D), bf16),
            pltpu.VMEM((D, D), bf16),
            pltpu.VMEM((D,), bf16),
            pltpu.VMEM((D, D), f32),
            pltpu.VMEM((8, D), f32),
            pltpu.VMEM((D, 128), f32),
            pltpu.VMEM((NT, D, 128), bf16),
            pltpu.VMEM((NT, D, FPC * FW + 256), bf16),
            pltpu.VMEM((NT, D, FPC * FW + 256), bf16),
            pltpu.VMEM((NT, FPC * FW, D + 256), bf16),
            pltpu.VMEM((D, 128), f32),
            pltpu.VMEM((FPC * FW, 128), f32),
            pltpu.VMEM((8, D), f32),
            pltpu.VMEM((S, D), bf16),
            pltpu.SemaphoreType.DMA((_N_SEM,)),
            pltpu.SemaphoreType.DMA((NT * len(_OUT_PIECES),)),
        ],
        compiler_params=pltpu.CompilerParams(dimension_semantics=("arbitrary",),
                                             vmem_limit_bytes=100 * 1024 * 1024,
                                             disable_semaphore_checks=True),
        name="linattn_mod",
    )(A_x.reshape(S, D), A_wqkv, A_wo, B_w_r, B_w_gate, B_w_up, B_w_down)
    return out.reshape(1, S, D)
```

```python
import itertools

import jax
import jax.numpy as jnp
from jax import lax
import jax.experimental.pallas as pl
import jax.experimental.pallas.tpu as pltpu

S = 2048
D = 1024
F = 3584
H = 32
DH = D // H
G128 = D // 128
CW = 256
NC = D // CW
T0 = 256
TS = 512
NT = S // TS
T1 = TS + T0
N1 = (S - TS) // T1
FW = 256
NFU = F // FW
FPC = -(-NFU // NT)
FP0 = NFU - (NT - 1) * FPC

FFN_STEP = 64
FFN_RB = 16
FFN_THIN = (2, 5)
FFN_LAG = 8
LN_C = (32, (0, 0, 6, 2))
LN_D = (16, (0, 0, 8, 0, 0, 17, 7))
LN_OWN = (16, (5, 11, 0))
LN_NEXT = (16, (0, 0, 15, 0, 17))

_LN_EPS = 1.0013580322265625e-05
_EPS = 1e-6

f32 = jnp.float32
bf16 = jnp.bfloat16

_OUT_DOTS = [(0, TS, c * CW, CW) for c in range(NC - 1)] + [
    (0, 384, D - CW, CW), (384, 128, D - CW, CW)]
_OUT_PIECES = _OUT_DOTS[:NC] + [(r, n, D - CW, CW) for r, n in ((384, 64), (448, 48), (496, 16))]

_X_ROWS = [(0, T0 // 2), (T0 // 2, T0 // 2), (T0, T0), (TS, TS), (2 * TS, S - 2 * TS)]
_WK_COLS = ((0, 128), (128, 384), (384, 640), (640, 1024))
_SEM_X = 0
_SEM_WK = _SEM_X + len(_X_ROWS)
_SEM_WQ = _SEM_WK + len(_WK_COLS)
_SEM_WV = _SEM_WQ + NC
_SEM_WO = _SEM_WV + 1
_SEM_WR = _SEM_WO + 1
_SEM_F = _SEM_WR + 1
_N_SEM = _SEM_F + 3 * NT

_TN = (((0,), (0,)), ((), ()))
_NT = (((1,), (1,)), ((), ()))


def _bf16_round(v):
    return v.astype(bf16).astype(f32)


def _phi(t):
    return jnp.where(t > 0, t + 1.0, jnp.exp(t)) + _EPS


def _tie(val, dep, never, last=False):
    if dep is None:
        return val
    if last:
        tail = jnp.where(never, dep, val[-8:, -128:])
        if val.shape[1] > 128:
            tail = jnp.concatenate([val[-8:, :-128], tail], axis=1)
        return jnp.concatenate([val[:-8, :], tail], axis=0)
    head = jnp.where(never, dep, val[:8, :128])
    head = jnp.concatenate([head, val[:8, 128:]], axis=1)
    return jnp.concatenate([head, val[8:, :]], axis=0)


def _tie_tiles(val, deps, never, rb):
    cols = []
    for n in range(val.shape[1] // 128):
        blocks = [_tie(val[r:r + rb, n * 128:(n + 1) * 128], next(deps, None), never, True)
                  for r in range(0, val.shape[0], rb)]
        cols.append(jnp.concatenate(blocks, axis=0))
    return jnp.concatenate(cols, axis=1)


def _thin(it, num, den):
    i = 0
    while True:
        take = ((i + 1) * num) // den > (i * num) // den
        yield next(it, None) if take else None
        i += 1


def _kernel(*refs):
    pl.when(pl.program_id(0) == 0)(lambda: _body(*refs))


def _body(x_hbm, wqkv_hbm, wo_hbm, wr_hbm, wg_hbm, wu_hbm, wd_hbm, out_hbm,
          x_buf, xn_buf, wq_buf, wk_buf, wv_buf, wqt_buf, wo_buf, m_buf, wr_buf,
          g_acc, z_acc, zb_buf, xt_buf,
          wg_buf, wu_buf, wd_buf, xb_buf, hb_buf, y_acc, out_buf,
          sem, o_sem):

    def x_copy(i):
        rows = pl.ds(*_X_ROWS[i])
        return pltpu.make_async_copy(x_hbm.at[rows, :], x_buf.at[rows, :], sem.at[_SEM_X + i])

    def wk_copy(s):
        c0, c1 = _WK_COLS[s]
        return pltpu.make_async_copy(wqkv_hbm.at[:, pl.ds(D + c0, c1 - c0)],
                                     wk_buf.at[:, pl.ds(c0, c1 - c0)], sem.at[_SEM_WK + s])

    def wq_copy(c):
        return pltpu.make_async_copy(wqkv_hbm.at[:, pl.ds(c * CW, CW)], wq_buf.at[c],
                                     sem.at[_SEM_WQ + c])

    wv_copy = pltpu.make_async_copy(wqkv_hbm.at[:, pl.ds(2 * D, D)], wv_buf.at[:, pl.ds(0, D)],
                                    sem.at[_SEM_WV])
    wo_copy = pltpu.make_async_copy(wo_hbm, wo_buf, sem.at[_SEM_WO])
    wr_copy = pltpu.make_async_copy(wr_hbm, wr_buf, sem.at[_SEM_WR])

    def ffn_copy(j, which):
        n = (FP0 if isinstance(j, int) and j == 0 and which < 2 else FPC) * FW
        if isinstance(j, int):
            f0 = max(FP0 + (j - 1) * FPC, 0) * FW
        else:
            f0 = pl.multiple_of(jnp.maximum(FP0 + (j - 1) * FPC, 0) * FW, FW)
        s = sem.at[_SEM_F + 3 * j + which]
        if which == 2:
            return pltpu.make_async_copy(wd_hbm.at[pl.ds(f0, n), :],
                                         wd_buf.at[j, :, pl.ds(0, D)], s)
        src, dst = ((wg_hbm, wg_buf), (wu_hbm, wu_buf))[which]
        return pltpu.make_async_copy(src.at[:, pl.ds(f0, n)], dst.at[j, :, pl.ds(0, n)], s)

    def out_copy(t, p):
        r0, nr, c0, nc = _OUT_PIECES[p]
        row = t * TS + r0
        rows = pl.ds(row if isinstance(t, int) else pl.multiple_of(row, 16), nr)
        cols = pl.ds(c0, nc)
        return pltpu.make_async_copy(out_buf.at[rows, cols], out_hbm.at[rows, cols],
                                     o_sem.at[t * len(_OUT_PIECES) + p])

    x_copy(0).start()
    x_copy(1).start()
    wk_copy(0).start()
    wr_copy.start()
    wk_copy(1).start()
    x_copy(2).start()
    wk_copy(2).start()
    wk_copy(3).start()
    for i in range(3, len(_X_ROWS)):
        x_copy(i).start()
    for c in range(NC):
        wq_copy(c).start()
    wv_copy.start()
    wo_copy.start()
    for j in range(NT):
        for which in range(3):
            ffn_copy(j, which).start(priority=1)

    y_acc[...] = jnp.zeros_like(y_acc)
    hb_buf[...] = jnp.zeros_like(hb_buf)

    sub_iota = lax.broadcasted_iota(jnp.int32, (8, 128), 0)

    def route(xn, row0, best):
        nr = xn.shape[0]
        wr = wr_buf[...].reshape(1, D).astype(f32)
        r = _bf16_round(jnp.sum(xn.astype(f32) * wr, axis=-1, keepdims=True))
        r = jnp.broadcast_to(r, (nr, 128))
        for g in range(0, nr, 8):
            rg = r[g:g + 8, :]
            better = rg > best[0]
            best[0] = jnp.where(better, rg, best[0])
            best[1] = jnp.where(better, sub_iota + (row0 + g), best[1])

    def layernorm(src, dst, nr, best, after=None, never=None):
        x = x_buf[pl.ds(src, nr), :].astype(f32)
        x = _tie(x, after, never)
        mean = jnp.sum(x, axis=-1, keepdims=True) * (1.0 / D)
        mean_b = _bf16_round(mean)
        e = x - mean_b
        off = mean - mean_b
        var = jnp.sum(e * e, axis=-1, keepdims=True) * (1.0 / D) - off * off
        sd = _bf16_round(jnp.sqrt(_bf16_round(_bf16_round(var) + _LN_EPS)))
        rs = pl.reciprocal(sd, approx=True)
        rs = jnp.where(sd == jnp.inf, 0.0, rs * (2.0 - sd * rs))
        xf = _bf16_round(e) * rs
        xn = xf.astype(bf16)
        xn_buf[pl.ds(dst, nr), :] = xn
        if best is not None:
            route(xn, src, best)
        dep = None
        for g in range(0, nr, 8):
            dg = xf[g:g + 8, D - 128:]
            dep = dg if dep is None else dep + dg
        return dep, sd

    def ln_work(src, dst, nr, plan, best, never):
        sub, counts = plan
        assert sub * sum(counts) == nr
        o = 0
        for n in counts:
            dep = None
            for _ in range(n):
                dep = layernorm(src + o, dst + o, sub, best, dep, never)[0]
                o += sub
            yield dep

    def rows_of(r0, nr):
        got = []

        def get():
            if not got:
                got.append(xn_buf[pl.ds(r0, nr), :])
            return got[0]
        return get

    def kg_steps(jobs, work, never):
        def tied(val):
            return _tie(val, next(work, None), never, True)

        def k_part(xn, c0, cw, init):
            cols = slice(c0, c0 + cw)
            xn = xn()
            pk = _phi(tied(jnp.dot(xn, wk_buf[:, cols], preferred_element_type=f32)))
            zc = jnp.sum(pk.reshape(xn.shape[0] // 8, 8, cw), axis=0)
            z_acc[:, cols] = zc if init else z_acc[:, cols] + zc
            return pk.astype(bf16)

        def g_part(pk, xn, c0, cw, init):
            rows = slice(c0, c0 + cw)
            g = tied(lax.dot_general(pk, xn(), _TN, preferred_element_type=f32))
            g_acc[rows, :] = g if init else g_acc[rows, :] + g

        prev = None
        for job in jobs:
            if job is None:
                g_part(prev[0], *prev[1])
                prev = None
                continue
            pk = k_part(*job)
            if prev is not None:
                g_part(prev[0], *prev[1])
            prev = (pk, job)
        g_part(prev[0], *prev[1])
        assert next(work, None) is None

    best = [jnp.full((8, 128), -jnp.inf, f32), jnp.zeros((8, 128), jnp.int32)]
    x_copy(0).wait()
    sd0 = layernorm(0, 0, T0 // 2, None)[1]
    x_copy(1).wait()
    layernorm(T0 // 2, T0 // 2, T0 // 2, None)
    wk_copy(0).wait()
    never = jnp.min(sd0[0:8, :]) < 0.0
    kg_steps([(rows_of(0, T0 // 2), 0, 128, True), (rows_of(T0 // 2, T0 // 2), 0, 128, False)],
             iter(()), never)

    def route_first():
        yield None
        for r in range(0, T0, T0 // 2):
            route(xn_buf[r:r + T0 // 2, :], r, best)
            yield best[0]

    wr_copy.wait()
    wk_copy(1).wait()
    xa = rows_of(0, T0)
    kg_steps([(xa, 128, 128, True), (xa, 256, 128, True)], route_first(), never)

    x_copy(2).wait()
    wk_copy(2).wait()
    xa, xb = rows_of(0, T0), rows_of(T0, T0)
    kg_steps([(xa, 384, 128, True), (xa, 512, 128, True), None,
              (xb, 0, 128, False), (xb, 128, 128, False)],
             ln_work(T0, T0, T0, LN_C, best, never), never)

    wk_copy(3).wait()
    x_copy(3).wait()
    xa, xb = rows_of(0, TS), rows_of(T0, T0)
    kg_steps([(xb, 256, 256, False), (xb, 512, 128, False),
              (xa, 640, 128, True), (xa, 768, 256, True)],
             ln_work(TS, TS, TS, LN_D, best, never), never)
    x_copy(4).wait()
    for c in range(NC):
        wq_copy(c).wait()

    def phase1(i, carry):
        best = list(carry)
        r0 = pl.multiple_of(TS + i * T1, 128)
        src = pl.multiple_of(jnp.minimum(r0 + T1, S - TS), 128)
        for c in range(NC // N1):
            cq = i * (NC // N1) + c
            wqt_buf[pl.ds(pl.multiple_of(cq * CW, CW), CW), :] = wq_buf[cq].T
        xa, xb = rows_of(r0, TS), rows_of(r0 + TS, T0)

        def xc():
            return jnp.concatenate([xa(), xb()], axis=0)

        kg_steps([(xa, 0, CW, False), (xa, CW, CW, False), (xb, 0, 2 * CW, False),
                  (xc, 2 * CW, CW, False), (xc, 3 * CW, CW, False)],
                 itertools.chain(ln_work(r0 + TS, r0 + TS, T0, LN_OWN, best, never),
                                 ln_work(src, r0 + T1, TS, LN_NEXT, best, never)), never)
        return tuple(best)

    best = lax.fori_loop(0, N1, phase1, tuple(best))

    wv_copy.wait()
    wo_copy.wait()
    ffn_copy(0, 0).wait()
    ffn_copy(0, 1).wait()
    rr = lax.broadcasted_iota(jnp.int32, (128, 128), 0) // DH
    cc = lax.broadcasted_iota(jnp.int32, (128, 128), 1) // DH
    same_head = rr == cc

    def kv_part(g):
        sl = slice(g * 128, (g + 1) * 128)
        kv = jnp.dot(g_acc[sl, :].astype(bf16), wv_buf[:, sl], preferred_element_type=f32)
        return jnp.where(same_head, kv, 0.0).astype(bf16)

    def m_part(g, kv, work):
        sl = slice(g * 128, (g + 1) * 128)
        m = jnp.dot(kv, wo_buf[sl, :], preferred_element_type=f32)
        m_buf[sl, :] = _tie_tiles(m, work, never, 64).astype(bf16)

    def ffn_items(j_dn, j_up, n_up, down_done):
        late = []

        def matvec(w_ref, slot, nrows, cols, col_ref):
            acc = None
            for r in range(0, nrows, FFN_STEP):
                w = w_ref[slot, r:r + FFN_STEP, cols].astype(f32)
                p = w * jnp.concatenate([col_ref[r:r + FFN_STEP, :]] * (FW // 128), axis=1)
                for g in range(0, FFN_STEP, 8):
                    acc = p[g:g + 8, :] if acc is None else acc + p[g:g + 8, :]
                yield acc[:, :128] + acc[:, 128:]
            return acc

        def work():
            if j_dn is not None:
                for e in range(D // FW):
                    ec = slice(e * FW, (e + 1) * FW)
                    acc = yield from matvec(wd_buf, j_dn, FPC * FW, ec, hb_buf)
                    y_acc[:, ec] += acc
                down_done.append(True)
            for u in range(n_up):
                fs = slice(u * FW, (u + 1) * FW)
                g = yield from matvec(wg_buf, j_up, D, fs, xb_buf)
                a = yield from matvec(wu_buf, j_up, D, fs, xb_buf)
                g = jnp.sum(g, axis=0, keepdims=True)
                h = g * (1.0 / (1.0 + jnp.exp(-g))) * jnp.sum(a, axis=0, keepdims=True)
                hb = jnp.broadcast_to(h, (128, FW)).T
                hb_buf[fs, :] = hb
                late.append([FFN_LAG, hb[120:128, :] + hb[FW - 8:, :]])

        gen = work()
        while True:
            dep = next(gen, None)
            if dep is None and not late:
                return
            for e in late:
                e[0] -= 1
            if late and late[0][0] <= 0:
                d = late.pop(0)[1]
                dep = d if dep is None else dep + d
            yield dep

    rmax = jnp.max(best[0], axis=0, keepdims=True)
    idx = jnp.clip(jnp.min(jnp.where(best[0] == rmax, best[1], S)), 0, S - 1)
    gate = 1.0 / (1.0 + jnp.exp(-rmax[:, :1]))
    r16 = pl.multiple_of((idx // 16) * 16, 16)
    blk = xn_buf[pl.ds(r16, 16), :].astype(f32)
    sel = lax.broadcasted_iota(jnp.int32, (16, D), 0) == (idx - r16)
    x_sel = jnp.sum(jnp.where(sel, blk, 0.0), axis=0, keepdims=True)
    xb_buf[...] = jnp.broadcast_to(x_sel, (128, D)).T

    items = ffn_items(None, 0, FP0, None)
    kv_prev = kv_part(0)
    for g in range(1, G128):
        kv = kv_part(g)
        m_part(g - 1, kv_prev, items)
        kv_prev = kv
    m_part(G128 - 1, kv_prev, items)
    assert next(items, 0) == 0
    z = jnp.sum(z_acc[...], axis=0, keepdims=True)
    zb_buf[...] = jnp.broadcast_to(z, (128, D)).T
    for t in range(NT):
        xt_buf[t] = xn_buf[t * TS:t * TS + 128, :].T

    def phase2(j, t_prev):
        ffn_copy(j, 2).wait()

        @pl.when(j < NT - 1)
        def _():
            ffn_copy(j + 1, 0).wait()
            ffn_copy(j + 1, 1).wait()

        t = (t_prev + 1) & (NT - 1)
        xn = xn_buf[pl.ds(pl.multiple_of(t * TS, TS), TS), :]
        down_done = []
        items = ffn_items(j, jnp.minimum(j + 1, NT - 1), FPC, down_done)
        work = _thin(items, *FFN_THIN)

        ps = []
        for c in range(NC):
            rows = slice(c * CW, (c + 1) * CW)
            if c == 0:
                q0 = jnp.dot(wqt_buf[rows, :], xt_buf[t], preferred_element_type=f32)
                qt = lax.dot_general(wqt_buf[rows, :], xn[128:], _NT, preferred_element_type=f32)
                qt = jnp.concatenate([q0, qt], axis=1)
            else:
                qt = lax.dot_general(wqt_buf[rows, :], xn, _NT, preferred_element_type=f32)
            pqt = _phi(_tie_tiles(qt, work, never, FFN_RB))
            zfull = jnp.concatenate([zb_buf[rows, :]] * (TS // 128), axis=1)
            hc = CW // DH
            den = jnp.sum((pqt * zfull).reshape(hc, DH, TS), axis=1, keepdims=True) + _EPS
            pt = pqt.reshape(hc, DH, TS) * pl.reciprocal(den, approx=True)
            ps.append(pt.reshape(CW, TS).astype(bf16).T)
        p = jnp.concatenate(ps, axis=1)
        assert down_done
        y = jnp.sum(y_acc[...], axis=0, keepdims=True) * gate
        for r0, nr, c0, nc in _OUT_DOTS:
            cols = slice(c0, c0 + nc)
            rows = pl.ds(pl.multiple_of(t * TS + r0, 128), nr)
            o = jnp.dot(p[r0:r0 + nr, :], m_buf[:, cols], preferred_element_type=f32)
            o = _tie_tiles(o, work, never, FFN_RB)
            o = o + x_buf[rows, cols].astype(f32) + xn_buf[rows, cols].astype(f32)
            hit = lax.broadcasted_iota(jnp.int32, (nr, nc), 0) == idx - (t * TS + r0)
            o = (o + jnp.where(hit, y[:, cols], 0.0)).astype(bf16)
            for n, (p0, pr, pc, _) in enumerate(_OUT_PIECES):
                if pc == c0 and r0 <= p0 < r0 + nr:
                    dst = pl.ds(pl.multiple_of(t * TS + p0, 16), pr)
                    out_buf[dst, cols] = o[p0 - r0:p0 - r0 + pr]
                    out_copy(t, n).start()
        assert next(items, 0) == 0
        return t

    lax.fori_loop(0, NT, phase2, idx // TS)
    for t in range(NT):
        for n in range(len(_OUT_PIECES)):
            out_copy(t, n).wait()


@jax.jit
def pallas_parallel_sum__linear_attn_block__moe_arch_mod__prompt_kernel(
    A_x: jax.Array,
    A_wqkv: jax.Array,
    A_wo: jax.Array,
    B_x: jax.Array,
    B_w_r: jax.Array,
    B_w_gate: jax.Array,
    B_w_up: jax.Array,
    B_w_down: jax.Array,
):
    any_spec = pl.BlockSpec(memory_space=pl.ANY)
    out = pl.pallas_call(
        _kernel,
        out_shape=jax.ShapeDtypeStruct((S, D), bf16),
        grid=(2,),
        in_specs=[any_spec] * 7,
        out_specs=any_spec,
        scratch_shapes=[
            pltpu.VMEM((S, D), bf16),
            pltpu.VMEM((S + TS, D), bf16),
            pltpu.VMEM((NC, D, CW), bf16),
            pltpu.VMEM((D, D + 128), bf16),
            pltpu.VMEM((D, D + 128), bf16),
            pltpu.VMEM((D, D), bf16),
            pltpu.VMEM((D, D), bf16),
            pltpu.VMEM((D, D), bf16),
            pltpu.VMEM((D,), bf16),
            pltpu.VMEM((D, D), f32),
            pltpu.VMEM((8, D), f32),
            pltpu.VMEM((D, 128), f32),
            pltpu.VMEM((NT, D, 128), bf16),
            pltpu.VMEM((NT, D, FPC * FW + 256), bf16),
            pltpu.VMEM((NT, D, FPC * FW + 256), bf16),
            pltpu.VMEM((NT, FPC * FW, D + 256), bf16),
            pltpu.VMEM((D, 128), f32),
            pltpu.VMEM((FPC * FW, 128), f32),
            pltpu.VMEM((8, D), f32),
            pltpu.VMEM((S, D), bf16),
            pltpu.SemaphoreType.DMA((_N_SEM,)),
            pltpu.SemaphoreType.DMA((NT * len(_OUT_PIECES),)),
        ],
        compiler_params=pltpu.CompilerParams(dimension_semantics=("arbitrary",),
                                             vmem_limit_bytes=100 * 1024 * 1024,
                                             disable_semaphore_checks=True),
        name="linattn_mod",
    )(A_x.reshape(S, D), A_wqkv, A_wo, B_w_r, B_w_gate, B_w_up, B_w_down)
    return out.reshape(1, S, D)
```
